```python
import jax
import jax.numpy as jnp

def _softmax(x, axis=-1):
    return jax.nn.softmax(x, axis=axis)

def _gelu(x):
    return jax.nn.gelu(x, approximate=True)

def _silu(x):
    return jax.nn.silu(x)

def _sigmoid(x):
    return jax.nn.sigmoid(x)

def _layernorm(x, axis=-1, eps=1e-05):
    m = jnp.mean(x, axis=axis, keepdims=True)
    v = jnp.var(x, axis=axis, keepdims=True)
    return (x - m) / jnp.sqrt(v + eps)

def _scatter_add(tgt, idx, src, axis=0):
    return tgt.at[idx].add(src)

def _segment_sum(src, seg, n):
    return jax.ops.segment_sum(src, seg, n)

class _Rng:

    def __init__(self, key):
        self._k = key

    def _next(self):
        self._k, sub = jax.random.split(self._k)
        return sub

    def normal(self, shape):
        return jax.random.normal(self._next(), shape, dtype=jnp.bfloat16)

    def randint(self, lo, hi, shape):
        return jax.random.randint(self._next(), shape, lo, hi, dtype=jnp.int32)

    def uniform(self, shape, lo=0.0, hi=1.0):
        return jax.random.uniform(self._next(), shape, jnp.bfloat16, lo, hi)

    def permutation(self, n):
        return jax.random.permutation(self._next(), n)
kernel_name = 'concat_heads__sliding_local_dilated__memory_aug_recurrent_mem_tr__prompt'

def setup_inputs():
    _rng = _Rng(jax.random.key(int.from_bytes(__import__("os").urandom(4), "little")))
    _w = lambda a: (lambda t: t.astype(jnp.bfloat16) if jnp.issubdtype(t.dtype, jnp.floating) else t)(jnp.asarray(a))

    def _A_setup():
        B, S, D = (1, 2048, 640)
        return {'x': _w((lambda *s: _rng.normal(s) * 0.05)(B, S, D)), 'wqkv': _w((lambda *s: _rng.normal(s) * 0.05)(D, 3 * D)), 'wo': _w((lambda *s: _rng.normal(s) * 0.05)(D, D))}
    _A_in = _A_setup()

    def _B_setup():
        B, S, Dm = (1, 2048, 640)
        H, Dh = (32, 192)
        M, seg = (8, 32)
        seg = min(seg, S)
        S = S // seg * seg
        return {'x': _w((lambda *s: _rng.normal(s) * 0.05)(B, S, Dm)), 'mem0': _w((lambda *s: _rng.normal(s) * 0.05)(B, M, Dm)), 'Wq': _w((lambda *s: _rng.normal(s) * 0.05)(Dm, H, Dh) * Dm ** (-0.5)), 'Wk': _w((lambda *s: _rng.normal(s) * 0.05)(Dm, H, Dh) * Dm ** (-0.5)), 'Wv': _w((lambda *s: _rng.normal(s) * 0.05)(Dm, H, Dh) * Dm ** (-0.5)), 'Wo': _w((lambda *s: _rng.normal(s) * 0.05)(H, Dh, Dm) * (H * Dh) ** (-0.5)), 'seg_len': seg}
    _B_in = _B_setup()
    return {'A_x': _A_in['x'], 'A_wqkv': _A_in['wqkv'], 'A_wo': _A_in['wo'], 'B_x': _B_in['x'], 'B_mem0': _B_in['mem0'], 'B_Wq': _B_in['Wq'], 'B_Wk': _B_in['Wk'], 'B_Wv': _B_in['Wv'], 'B_Wo': _B_in['Wo'], 'B_seg_len': _B_in['seg_len']}

def reference(A_x, A_wqkv, A_wo, B_x, B_mem0, B_Wq, B_Wk, B_Wv, B_Wo, B_seg_len):

    def _A_ref(x, wqkv, wo):
        B, S, D = x.shape
        H = 32
        Dh = D // H
        W, dil = (8, 2)
        qkv = (lambda x, *d: x.transpose(*d))((x @ wqkv).reshape(B, S, 3, H, Dh), 2, 0, 3, 1, 4)
        q, k, v = (qkv[0], qkv[1], qkv[2])
        scale = Dh ** (-0.5)
        pos = jnp.arange(S)
        off = jnp.arange(W) * dil
        idx = pos[:, None] - off[None, :]
        mask = idx >= 0
        idx_c = jnp.where(mask, idx, 0).reshape(-1)
        kg = k[:, :, idx_c, :].reshape(B, H, S, W, Dh)
        vg = v[:, :, idx_c, :].reshape(B, H, S, W, Dh)
        logits = jnp.einsum('bhsd,bhswd->bhsw', q, kg) * scale
        logits = jnp.where(mask[None, None, :, :], logits, -1000000000.0)
        attn = _softmax(logits, axis=-1)
        o = jnp.einsum('bhsw,bhswd->bhsd', attn, vg)
        return (lambda x, *d: x.transpose(*d))(o, 0, 2, 1, 3).reshape(B, S, D) @ wo

    def _B_ref(x, mem0, Wq, Wk, Wv, Wo, seg_len):
        B, S, Dm = x.shape
        H, Dh = (Wq.shape[1], Wq.shape[2])
        M = mem0.shape[1]
        scale = Dh ** (-0.5)
        n_seg = S // seg_len
        L = M + seg_len
        idx = jnp.arange(L)
        mask = (idx[:, None] < M) | (idx[:, None] >= idx[None, :])
        mem = mem0
        outs = []
        for s in range(n_seg):
            xs = x[:, s * seg_len:(s + 1) * seg_len, :].copy()
            h = jnp.concatenate([mem, xs], axis=1)
            q = jnp.einsum('btd,dhe->bhte', h, Wq)
            k = jnp.einsum('btd,dhe->bhte', h, Wk)
            v = jnp.einsum('btd,dhe->bhte', h, Wv)
            scores = jnp.einsum('bhqe,bhke->bhqk', q, k) * scale
            scores = jnp.where(mask[None, None], scores, -1000000000.0)
            p = _softmax(scores, axis=-1)
            o = jnp.einsum('bhqk,bhke->bhqe', p, v)
            o = jnp.einsum('bhte,hed->btd', o, Wo)
            mem = o[:, :M, :].copy()
            outs.append(o[:, M:, :])
        return jnp.concatenate(outs, axis=1)
    a = _A_ref(A_x, A_wqkv, A_wo)
    b = _B_ref(B_x, B_mem0, B_Wq, B_Wk, B_Wv, B_Wo, B_seg_len)
    return jnp.concatenate([a, b], axis=-1)
```

```python
import functools

import jax
import jax.numpy as jnp
from jax import lax
from jax.experimental import pallas as pl
from jax.experimental.pallas import tpu as pltpu

F32, BF16, U32 = jnp.float32, jnp.bfloat16, jnp.uint32
NN = (((1,), (0,)), ((), ()))
NT = (((1,), (1,)), ((), ()))
MASKED = -1000000000.0
CFG = dict(UN=4, UT=1, AHEAD=2, cuts=[2, 3, 4, 6, 7, 8, 10, 11, 12, 14, 15, 16, 17, 18, 19], vlag=2, kc=3, lat=120, ties=[1, 2, 3, 4, 5], d_step=24, d_norm=280,
           rounds="LPssssLssssLssssLssssLQsssLssssLssssLQssssLsPssssLssssLssssVQsssLssssLssssLsWsWssssLssssVsWQssWsWsWssVQssssLsPssssLssssLssssVQssWssLssWPsWsssLsWsssLssWsssVQsssLssWsWsWsWsssVsWQsWsssLssssLssWWssssLsWsWssWWssssLssWQsssVsWssWsWWsWssWQsWssVsWsWssWWssssVQssWssWWWQssWWssWsWVsWPWWWVWWVWWWWWWWWWWW",
           rounds0="LPssssLssssLssssLssssLQsssLssssLssssLQssssLsPssssLssssLssssVQsssLssssLssssLsWsWssssLssssVsWQssWsWsWssVQssssLsPssssLssssLssssVQssWssLssWPsWsssLsWsssLssWsssVQsssLssWsWsWsWsssVsWQsWsssLssssLssWWssssLsWsWssWWssssLssWQsssVsWssWsWWsWssWQsWssVsWsWssWWssssVQssWssWWWQssWWssWsWVsWPWWWVWWLVWWWWWWWWWWW",
           last_rounds="PsssssssssssssPsssssssssssssssssssssssPQQssssssssssssssssssPQsssVPssssssWWWssssssVsssWQssVsssssssWssssssssWQssWssssWQWsssssssVWssWssWssWQsssssssVssssWQWssWWsWssWWsssVsWWsssssWsWQsWssssVssWssWsWWsssssWsssWsWsWssVsWQsssssVssWQsssWssWsWQWsWsWsWsVsWWWWWVWVWWWWWWWWWWWW")

S, D = 2048, 640
LT = D // 128

AH, AD, AW, ADIL = 32, 20, 8, 2
HALO = 16
TB = 128
NB = S // TB
RC = 8

H, DH, M, SEG = 32, 192, 8, 32
L = M + SEG
HALF = SEG // 2
NP = H // 2
FT = 3 * NP
NSEG = S // SEG
LAM = (0.0, 0.625, -0.625, 1.875, -1.875)
PAIRS = [(i, j) for i in range(LT) for j in range(i + 1, LT)]
NZ = LT + len(PAIRS)
NG = 28
ZB = 4
GS = NG // ZB
ZS = (GS * LT + 1) * HALF
AHEAD = CFG["AHEAD"]
UN, UT = CFG["UN"], CFG["UT"]
NBUF = max(UN, UT)
CG = 2
NCH = NG // CG
WOC = 4
KC = CFG["kc"]


def _tile_order():
    order = []
    for p in range(NP + CFG["vlag"]):
        if p < NP:
            order += [(j, 3 * p + t) for j in (0, 1) for t in range(3)]
        if p >= CFG["vlag"]:
            order += [(2, 3 * (p - CFG["vlag"]) + t) for t in range(3)]
    return order


TILES = _tile_order()
NPL = len(TILES) - NG * LT

R_LHS = 0
R_H = R_LHS + NBUF * LT * LT * (M + HALF)
R_QKV = R_H + NBUF * LT * L
R_O = R_QKV + 3 * FT * L
R_P = R_O + FT * L
R_ACC = R_P + NP * 2 * L
R_S = R_ACC + LT * L
R_END = (R_S + NP * L + 31) // 32 * 32


def _make_plan(rounds, longs):
    shell = []
    for k in range(LT):
        for n in range(k + 1, LT):
            shell += [(k, n), (n, k)]
        shell += [(k, k)]
    todo = dict(
        L=longs,
        s=[("short", g, i, j) for g in range(NG) for (i, j) in shell],
        W=[("out", k0 + k, n) for k0 in range(0, FT, KC) for n in range(LT) for k in range(KC)],
        P=[("plain", n, k) for k in range(LT) for n in range(NPL)],
        Q=[("score", t) for t in range(FT)],
        V=[("pv", t) for t in range(FT)])
    plan, timed, now = [], [], 0

    def later(time, *task):
        timed.append((time, task))

    def flush(time):
        timed.sort(key=lambda x: x[0])
        while timed and timed[0][0] <= time:
            plan.append(timed.pop(0)[1])

    def needs(task):
        if task[0] == "out":
            return [("pv_end", task[1])]
        if task[0] not in ("score", "pv"):
            return []
        need = [("softmax", task[1] // 3, 5)] if task[0] == "pv" else []
        for j in (2,) if task[0] == "pv" else (0, 1):
            n = TILES.index((j, task[1]))
            need.append(("take", n // LT, n % LT, n % LT) if n < NG * LT else ("plain_end", n - NG * LT, LT - 1))
        return need

    for n, kind in enumerate(rounds):
        four = todo[kind][:4]
        del todo[kind][:4]
        need = [x for task in four for x in needs(task)]
        now = max([now] + [time for time, task in timed if task in need])
        flush(now)
        assert all(x in plan for x in need)
        plan += four
        now += dict(s=M + HALF if longs is not None else 30, L=ZB * HALF).get(kind, L)
        end = now + CFG["lat"]
        for name, *args in four:
            if name == "short":
                later(end, "take", *args)
            elif name == "out" and args[0] % KC == KC - 1:
                later(end, "out_end", *args)
            elif name in ("plain", "long", "pv"):
                later(end, name + "_end", *args)
            elif name == "score" and args[0] % 3 == 2:
                for step in range(6):
                    later(now + CFG["d_step"] * sum(x <= step for x in CFG["ties"]), "softmax", args[0] // 3, step)
        if kind not in rounds[n + 1:] and kind in "sL":
            plan.append(("token_lhs",) if kind == "s" else ("z_lhs",))
    assert not any(todo[kind] for kind in "sWPQV")
    return plan, [task for _, task in sorted(timed, key=lambda x: x[0])]


def _ds(i, n):
    return pl.ds(i * n if isinstance(i, int) else pl.multiple_of(i * n, n), n)


def _dot(a, b, dims=NN):
    r = lax.dot_general(a, b, dims, preferred_element_type=F32)
    return jnp.concatenate([r[0:8], r[8:]], axis=0)


def _share(tasks, k, n):
    return tasks[k * len(tasks) // n:(k + 1) * len(tasks) // n]


def _run(tasks):
    for task in tasks:
        task()


def _inverse(x):
    r = pltpu.reciprocal(x, approx=True)
    return r + r * (1.0 - x * r)


def _pack(x):
    return pltpu.bitcast(x.astype(BF16), U32)


def _kernel(ax_hbm, awqkv_hbm, awo_hbm, bx_hbm, mem_hbm, wq_hbm, wk_hbm, wv_hbm, wo_hbm,
            out_hbm,
            ax, awqkv, awo, tmp, wqkv_p, wo_p, q_s, kv_s, oa_s, outa,
            bx, mem, raw, wb, wz, wo, lz, z, buf, outb,
            sem_a, sem_x, sem_w, sem_b, sem_wo, sem_o):
    cp = pltpu.make_async_copy

    def rows_copy(src, dst, r0, r1, sem):
        return cp(src.at[pl.ds(r0, r1 - r0), :], dst.at[pl.ds(r0, r1 - r0), :], sem)

    c_wqkv = [cp(awqkv_hbm.at[:, pl.ds(j * D, D)], awqkv.at[j], sem_a.at[j]) for j in range(3)]
    c_awo = cp(awo_hbm, awo, sem_a.at[3])
    c_ax = [rows_copy(ax_hbm, ax, TB * c, TB * (c + 1), sem_x.at[c]) for c in range(NB)]
    c_mem = cp(mem_hbm, mem.at[pl.ds(0, M), :], sem_b.at[0])
    first_rows = (AHEAD + 2) * ZB * SEG
    c_bx0 = rows_copy(bx_hbm, bx, 0, first_rows, sem_b.at[1])
    c_bx1 = rows_copy(bx_hbm, bx, first_rows, S, sem_b.at[2])
    wo_rows = H * DH // WOC
    c_wo = [rows_copy(wo_hbm, wo, c * wo_rows, (c + 1) * wo_rows, sem_wo.at[c]) for c in range(WOC)]
    c_outa = cp(outa, out_hbm.at[:, pl.ds(0, D)], sem_o.at[0])

    def c_w(c):
        if c > NCH:
            return [c_wo[c - NCH - 1]]
        copies, n, end = [c_mem if c == NCH else c_ax[c + 2]], c * CG * LT, min((c + 1) * CG * LT, len(TILES))
        while n < end:
            j, t = TILES[n]
            k = min(3 - t % 3, end - n)
            copies.append(cp((wq_hbm, wk_hbm, wv_hbm)[j].at[pl.ds(t * 128, k * 128), :],
                             raw.at[pl.ds(n * 128, k * 128), :], sem_w.at[c]))
            n += k
        return copies

    def wait_w(c):
        chunk = raw.at[_ds(c, CG * LT * 128), :]
        cp(chunk, chunk, sem_w.at[c]).wait()
        block = ax.at[_ds(c + 2, TB), :]
        cp(block, block, sem_x.at[c + 2]).wait()

    def c_outb(r0, n):
        return cp(outb.at[pl.ds(r0, n), :], out_hbm.at[pl.ds(r0, n), pl.ds(D, D)], sem_o.at[1])

    def start(copies):
        for c in copies:
            c.start()

    def wait(copies):
        for c in copies:
            c.wait()

    def permute_rows(dst, base):
        for d in range(AD):
            for t in range(LT):
                dst[pl.ds((base + d * AH) // 2, AH // 2), t * 128:(t + 1) * 128] = _pack(
                    tmp[t, pl.ds(d, AH, stride=AD), :])

    def prep_wqkv(j):
        for t in range(LT):
            tmp[t] = awqkv[j, t * 128:(t + 1) * 128, :].astype(F32).T
        permute_rows(wqkv_p, j * D)

    def prep_wo():
        for t in range(LT):
            tmp[t] = awo[:, t * 128:(t + 1) * 128].astype(F32)
        permute_rows(wo_p, 0)

    def a_proj(i, j):
        w = pltpu.bitcast(wqkv_p[j * D // 2:(j + 1) * D // 2, :], BF16)
        r = lax.dot_general(ax[_ds(i, TB), :], w, NT, preferred_element_type=F32)
        for t in range(LT):
            rt = r[:, t * 128:(t + 1) * 128]
            if j == 0:
                q_s[t] = rt
                continue
            c = (j - 1) * LT + t
            if isinstance(i, int) and i == 0:
                kv_s[c, 0:HALO, :] = jnp.broadcast_to(rt[0:1, :], (HALO, 128))
            else:
                kv_s[c, 0:HALO, :] = kv_s[c, TB:TB + HALO, :]
            kv_s[c, HALO:HALO + TB, :] = rt

    def a_attention(first_block=False):
        state = {}

        def window(c, r0, w):
            lo = HALO + r0 - ADIL * w
            return kv_s[c, lo:lo + RC, :]

        def logits(r0):
            q = [q_s[t, r0:r0 + RC, :] for t in range(LT)]
            state[r0] = []
            for w in range(AW):
                a = q[0] * window(0, r0, w)
                for t in range(1, LT):
                    a = a + q[t] * window(t, r0, w)
                state[r0].append(a + pltpu.roll(a, 2 * AH, 1))

        def fold(r0):
            state[r0] = [a + pltpu.roll(a, AH, 1) for a in state[r0]]

        def mix(r0):
            lg = []
            for w, a in enumerate(state.pop(r0)):
                a = a * (AD ** -0.5)
                if first_block and r0 < ADIL * w:
                    pos = lax.broadcasted_iota(jnp.int32, (RC, 128), 0) + r0
                    a = jnp.where(pos >= ADIL * w, a, MASKED)
                lg.append(a)
            m = functools.reduce(jnp.maximum, lg)
            e = [jnp.exp(a - m) for a in lg]
            inv = _inverse(functools.reduce(jnp.add, e))
            for t in range(LT):
                o = e[0] * window(LT + t, r0, 0)
                for w in range(1, AW):
                    o = o + e[w] * window(LT + t, r0, w)
                oa_s[r0:r0 + RC, t * 128:(t + 1) * 128] = o * inv

        n = TB // RC
        for k in range(n + 2):
            for lag, f in enumerate((logits, fold, mix)):
                if 0 <= k - lag < n:
                    f((k - lag) * RC)

    def a_out(i):
        outa[_ds(i, TB), :] = _dot(oa_s[...], pltpu.bitcast(wo_p[...], BF16)).astype(BF16)

    def w_transpose(n):
        wb[n] = pltpu.bitcast(raw[_ds(n, 128), :].T, U32)

    def w_combine(g, r):
        def rows(i):
            return slice(i * 64 + 8 * r, i * 64 + 8 * r + 8)
        b = [[pltpu.bitcast(wb[g * LT + j, rows(i), :], BF16).astype(F32) for j in range(LT)] for i in range(LT)]
        for n, (i, j) in enumerate(PAIRS):
            wz[g, LT + n, rows(0), :] = _pack(b[i][j] - b[j][i])
        for i in range(LT):
            rest = [k for k in range(LT) if k != i]
            wz[g, i, rows(0), :] = _pack(b[i][i] - functools.reduce(jnp.add, [b[i][k] for k in rest]))
            wb[g * LT + i, rows(i), :] = _pack(b[i][i] - functools.reduce(jnp.add, [b[k][i] for k in rest]))

    def w_prep(g):
        return ([functools.partial(w_transpose, g * LT + j) for j in range(LT)]
                + [functools.partial(w_combine, g, r) for r in range(8)])

    def halves(s):
        x = bx[_ds(s, SEG), :].astype(F32)
        return [[x[r:r + HALF, i * 128:(i + 1) * 128] for i in range(LT)] for r in (0, HALF)]

    def z_lhs(s):
        a, b = halves(s)
        p = [a[i] + LAM[i] * b[i] if LAM[i] else a[i] for i in range(LT)]
        for i in range(LT):
            lz[i, _ds(s, HALF // 2), :] = _pack(b[i])
        for n, (i, j) in enumerate(PAIRS):
            lz[LT + n, _ds(s, HALF // 2), :] = _pack((p[i] + p[j]) * (1.0 / (LAM[i] - LAM[j])))

    def z_product(g, n, batch, count=1):
        x = lz[n, _ds(batch, ZB * HALF // 2) if count == 1 else pl.ds(0, count * ZB * HALF // 2), :]
        return _dot(pltpu.bitcast(x, BF16), pltpu.bitcast(wz[g, n], BF16))

    def z_first(g):
        sums = [z_product(g, i, 0, AHEAD) for i in range(LT)]
        for n, pair in enumerate(PAIRS):
            r = z_product(g, LT + n, 0, AHEAD)
            for i in pair:
                sums[i] = sums[i] + r
        for i in range(LT):
            for u in range(AHEAD * ZB):
                z[u // ZB, u % ZB, g, i * HALF:(i + 1) * HALF, :] = sums[i][u * HALF:(u + 1) * HALF]

    if not CFG.get('onlyB'):
        start([c_wqkv[0], c_ax[0], c_wqkv[1]])
        c_wqkv[0].wait()
        c_wqkv[2].start()
        prep_wqkv(0)
        wait([c_ax[0], c_wqkv[1]])
        start([c_awo, c_ax[1], c_bx0])
        a_proj(0, 0)
        prep_wqkv(1)
        c_wqkv[2].wait()
        start(c_w(0))
        a_proj(0, 1)
        prep_wqkv(2)
        a_proj(0, 2)
        wait([c_awo, c_ax[1], c_bx0])
        start(c_w(1))
        a_attention(True)
        prep_wo()
        for s in range((AHEAD + 1) * ZB):
            z_lhs(s)
        for j in range(3):
            a_proj(1, j)
        a_out(0)

        def a_step(c, carry):
            wait_w(c)
            for k in range(NCH):
                @pl.when(c == k)
                def _():
                    for n in range(CFG["cuts"][k], CFG["cuts"][k + 1]):
                        start(c_w(n))
            g = jnp.where(c == 0, NG - CG, (c - 1) * CG)
            for u in range(CG):
                z_first(g + u)
            a_attention()
            for u in range(CG):
                _run(w_prep(c * CG + u))
            for j in range(3):
                a_proj(c + 2, j)
            a_out(c + 1)
            return carry

        lax.fori_loop(0, NCH, a_step, 0)
        wait(c_w(NCH))
        for g in range(NG - CG, NG):
            z_first(g)
        a_attention()
        for n in range(NG * LT, len(TILES)):
            w_transpose(n)
        a_out(NB - 1)

    def rows(r0, n):
        return slice(r0, r0 + n)

    def r_lhs(hb, i, j):
        return R_LHS + ((hb * LT + i) * LT + j) * (M + HALF)

    def r_qkv(j, t):
        return rows(R_QKV + (j * FT + t) * L, L)

    def token_lhs(s, hb):
        a, b = halves(s)
        for j in range(LT):
            buf[rows(R_H + (hb * LT + j) * L + M, SEG)] = jnp.concatenate([a[j], b[j]], axis=0)
            p = [a[i] + LAM[j] * b[i] if LAM[j] else a[i] for i in range(LT)]
            for i in range(LT):
                buf[rows(r_lhs(hb, i, j) + M, HALF)] = (
                    p[j] if i == j else (p[i] + p[j]) * (1.0 / (LAM[j] - LAM[i])))

    def memory_lhs(m, n, hb):
        buf[rows(R_H + (hb * LT + n) * L, M)] = m[n]
        buf[rows(r_lhs(hb, n, n), M)] = m[n]
        for k in range(n):
            buf[rows(r_lhs(hb, n, k), M)] = buf[rows(r_lhs(hb, k, n), M)] = m[n] + m[k]

    def segment(plan, batch, part, hb, nh, before=()):
        s = batch * ZB + part
        key = lax.broadcasted_iota(jnp.int32, (L, 128), 0)
        col = lax.broadcasted_iota(jnp.int32, (L, 128), 1)
        head0 = col < L
        query = jnp.where(head0, col, col - L)
        visible = (query < M) | (query >= key)
        low = lax.broadcasted_iota(jnp.int32, (L, 128), 1) < 64
        val = {}
        new_mem = []

        def add(name, x):
            val[name] = val[name] + x if name in val else x

        def product(*args):
            r = _dot(*args)
            val["latest"] = r[-8:]
            return r

        def short(g, i, j):
            w = pltpu.bitcast(wb[g * LT + j, rows(i * 64, 64), :], BF16)
            val[g, i, j] = product(buf[rows(r_lhs(hb, i, j), M + HALF)], w)

        def take(g, i, j):
            r = val.pop((g, i, j))
            add(("m", g, j), r[0:M])
            if i != j:
                add(("y", g, i), r[M:])
                add(("d", g, j), r[M:])
                if LAM[i]:
                    add(("c", g, j), r[M:] * -LAM[i])
                return
            y = z[batch % (AHEAD + 1), part, g, rows(j * HALF, HALF), :] + val.pop(("y", g, j))
            c = val.pop(("c", g, j)) + r[M:]
            if LAM[j]:
                c = c - LAM[j] * y
            buf[r_qkv(*TILES[g * LT + j])] = jnp.concatenate(
                [val.pop(("m", g, j)), c, val.pop(("d", g, j)) + y], axis=0)

        def plain(n, k):
            w = pltpu.bitcast(wb[NG * LT + n, rows(k * 64, 64), :], BF16)
            val["plain", n, k] = product(buf[rows(R_H + (hb * LT + k) * L, L)], w)

        def plain_end(n, k):
            dst = r_qkv(*TILES[NG * LT + n])
            r = val.pop(("plain", n, k))
            buf[dst] = r + buf[dst] if k else r

        def long(g, n):
            val["long", g, n] = z_product(g, n, batch + AHEAD)
            val["latest"] = val["long", g, n][24:32]

        def long_end(g, n):
            r = val.pop(("long", g, n))
            res = []
            for i in ((n,) if n < LT else PAIRS[n - LT]):
                for u in range(ZB):
                    dst = ((batch + AHEAD) % (AHEAD + 1), u, g, rows(i * HALF, HALF))
                    x = r[u * HALF:(u + 1) * HALF]
                    res.append((dst, x if n < LT else x + z[dst]))
            for dst, x in res:
                z[dst] = x

        def score(t):
            q = buf[r_qkv(0, t)]
            none = jnp.zeros((L, 128), F32)
            q = ((q, none), (jnp.where(low, q, 0.0), jnp.where(low, 0.0, q)), (none, q))[t % 3]
            q = jnp.concatenate(q + (jnp.zeros((128 - 2 * L, 128), F32),), axis=0)
            add(("s", t // 3), product(buf[r_qkv(1, t)], q.astype(BF16), NT))

        def softmax(p, step):
            def late(x):
                return jnp.where(col[0:8] < 2 * L, x, val["latest"]) if step in CFG["ties"] else x

            def groups(x):
                return [x[r:r + 8] for r in range(0, L, 8)]

            def spread(x):
                return jnp.concatenate([x] * (L // 8), axis=0)
            x, y = val["s", p], val.get(("t", p))
            if step == 0:
                x = jnp.where(visible, x * (DH ** -0.5), MASKED)
                y = functools.reduce(jnp.maximum, groups(x))
            elif step == 1:
                y = jnp.broadcast_to(jnp.max(late(y), axis=0, keepdims=True), (8, 128))
            elif step == 2:
                x = jnp.exp(x - spread(late(y)))
                y = functools.reduce(jnp.add, groups(x))
            elif step == 3:
                y = jnp.broadcast_to(jnp.sum(late(y), axis=0, keepdims=True), (8, 128))
            elif step == 4:
                y = _inverse(late(y))
            else:
                x = x * spread(late(y))
                x = jnp.concatenate([x, x], axis=0)[:, 0:2 * L]
                buf[rows(R_P + p * 2 * L, 2 * L), 0:2 * L] = x.astype(BF16).T.astype(F32) if CFG.get("xp16", 1) else x.T
            val["s", p], val["t", p] = x, y

        def pv(t):
            pa, pb = [buf[rows(R_P + (2 * (t // 3) + u) * L, L), 0:2 * L] for u in range(2)]
            v = buf[r_qkv(2, t)]
            if t % 3 == 1:
                v = jnp.concatenate([jnp.where(low, v, 0.0), jnp.where(low, 0.0, v)], axis=0)
            pr = (pa[:, 0:L], jnp.where(head0[:, 0:2 * L], pa, pb), pb[:, 0:L])[t % 3]
            val["o", t] = product(pr, v.astype(BF16))

        def pv_end(t):
            buf[rows(R_O + t * L, L)] = val.pop(("o", t))

        def out(t, n):
            add(("out", t // KC, n), product(buf[rows(R_O + t * L, L)], wo[rows(t * 128, 128), rows(n * 128, 128)]))

        def out_end(t, n):
            r = val.pop(("out", t // KC, n))
            if t >= KC:
                r = r + buf[rows(R_ACC + n * L, L)]
            if t < FT - 1:
                buf[rows(R_ACC + n * L, L)] = r
                return
            new_mem.append(r[0:M])
            memory_lhs(new_mem, n, nh)
            outb[_ds(s, SEG), rows(n * 128, 128)] = r[M:L].astype(BF16)

        tasks = dict(short=short, take=take, plain=plain, plain_end=plain_end, long=long, long_end=long_end,
                     score=score, softmax=softmax, pv=pv, pv_end=pv_end,
                     out=out, out_end=out_end,
                     token_lhs=lambda: token_lhs(jnp.minimum(s + 1, NSEG - 1), nh),
                     z_lhs=lambda: z_lhs(jnp.minimum(s + (AHEAD + 1) * ZB, NSEG - 1)))
        before = list(before)
        for name, *args in plan[0]:
            need = max(args[1:]) if name in ("short", "plain") else -1
            while len(before) > LT - 1 - need:
                before.pop(0)()
            tasks[name](*args)
        return [functools.partial(tasks[name], *args) for name, *args in plan[1]]

    if CFG.get('onlyB'):
        start(c_w(0) + c_wo + [c_bx0, c_mem])
        w_transpose(0)
        w_combine(0, 0)
        z_first(0)
    token_lhs(0, 0)
    mem0 = mem[0:M, :].astype(F32)
    for n in range(LT):
        memory_lhs([mem0[:, k * 128:(k + 1) * 128] for k in range(LT)], n, 0)

    longs = [("long", g, n) for g in range(NG) for n in range(NZ)]
    main_plans = [_make_plan(CFG["rounds"] if u else CFG["rounds0"], longs) for u in range(UN)]
    assert not longs or UN < ZB
    last_plan = _make_plan(CFG["last_rounds"], None)
    n_main = NSEG // ZB - AHEAD

    def b_step(it, carry):
        @pl.when(it == 1)
        def _():
            c_bx1.wait()
        rest = ()
        for u in range(UN):
            rest = segment(main_plans[u], it, u, u, (u + 1) % UN, rest)
        _run(rest)
        c_outb(pl.multiple_of(it * ZB * SEG, SEG), ZB * SEG).start()
        return carry

    def last_step(s, carry):
        _run(segment(last_plan, s // ZB, s % ZB, 0, 0))
        c_outb(pl.multiple_of(s * SEG, SEG), SEG).start()
        return carry

    wait(c_wo)
    start([c_bx1, c_outa])
    if CFG.get('onlyB') != 2 and not CFG.get('onlyA'):
        lax.fori_loop(0, n_main, b_step, 0)
    if CFG.get('onlyB') != 1 and not CFG.get('onlyA'):
        lax.fori_loop(n_main * ZB, NSEG, last_step, 0)
    if CFG.get('onlyA'):
        c_bx1.wait()
        outb[0:16, 0:128] = (z[0, 0, 0, 0:16] + pltpu.bitcast(wb[0, 0:16], F32) + buf[0:16] + pltpu.bitcast(lz[0, 32:48], F32)).astype(BF16)
        start([c_outb(0, S)])
    c_outa.wait()
    c_outb(0, S).wait()


def pallas_concat_heads__sliding_local_dilated__memory_aug_recurrent_mem_tr__prompt_kernel(
    A_x, A_wqkv, A_wo, B_x, B_mem0, B_Wq, B_Wk, B_Wv, B_Wo, B_seg_len,
):
    assert B_seg_len == SEG
    assert A_x.shape == B_x.shape == (1, S, D) and B_mem0.shape == (1, M, D)
    assert B_Wq.shape == B_Wk.shape == B_Wv.shape == (D, H, DH) and B_Wo.shape == (H, DH, D)
    vmem, dma = pltpu.VMEM, pltpu.SemaphoreType.DMA
    call = pl.pallas_call(
        _kernel,
        out_shape=jax.ShapeDtypeStruct((S, 2 * D), BF16),
        in_specs=[pl.BlockSpec(memory_space=pl.ANY)] * 9,
        out_specs=pl.BlockSpec(memory_space=pl.ANY),
        scratch_shapes=[
            vmem((S, D), BF16),
            vmem((3, D, D), BF16),
            vmem((D, D), BF16),
            vmem((LT, D, 128), F32),
            vmem((3 * D // 2, D), U32),
            vmem((D // 2, D), U32),
            vmem((LT, TB, 128), F32),
            vmem((2 * LT, HALO + TB, 128), F32),
            vmem((TB, D), F32),
            vmem((S, D), BF16),
            vmem((S, D), BF16),
            vmem((64, D), BF16),
            vmem((len(TILES) * 128, D), BF16),
            vmem((len(TILES), D // 2, 128), U32),
            vmem((NG, NZ, 64, 128), U32),
            vmem((H * DH, D), BF16),
            vmem((NZ, S // 4, 128), U32),
            vmem((AHEAD + 1, ZB, NG, LT * HALF, 128), F32),
            vmem((R_END, 128), F32),
            vmem((S, D), BF16),
            dma((4,)), dma((NB,)), dma((NCH + 1,)), dma((3,)), dma((WOC,)), dma((2,)),
        ],
        compiler_params=pltpu.CompilerParams(vmem_limit_bytes=120 * 1024 * 1024,
                                             internal_scratch_in_bytes=48 * 1024),
        name="sliding_and_memory_attention",
    )

    def by_feature(w):
        return w.transpose(1, 2, 0).reshape(H * DH, D)

    out = call(A_x.reshape(S, D), A_wqkv, A_wo, B_x.reshape(S, D), B_mem0.reshape(M, D),
               by_feature(B_Wq), by_feature(B_Wk), by_feature(B_Wv), B_Wo.reshape(H * DH, D))
    return out.reshape(1, S, 2 * D)
```

```python
import functools

import jax
import jax.numpy as jnp
from jax import lax
from jax.experimental import pallas as pl
from jax.experimental.pallas import tpu as pltpu

F32, BF16, U32 = jnp.float32, jnp.bfloat16, jnp.uint32
NN = (((1,), (0,)), ((), ()))
NT = (((1,), (1,)), ((), ()))
MASKED = -1000000000.0
CFG = dict(UN=4, UT=1, G0=4, f=[1200, 700, 2700, 2400, 4200], lags=[0, 50, 330, 380, 430], cuts=[2, 3, 4, 6, 7, 8, 10, 11, 12, 14, 15, 16, 17, 18, 19], vlag=2, kc=3, lat=120, ties=[1, 2, 3, 4, 5], d_step=24, d_norm=280,
           rounds="LPssssLssssssLssssLssssLssssssLQQssssLssssLssssLssssLssssssLssssLssssVQssssLssssLssPsWsWsWsssLssssLssWsssLssssLssssVsssVsWssWQQsWsWsWssWQsWsPsWsWsssVssWQsWssVsWsWssWsPsssVQsWssWsWssssLssssLsWssssLssssLssssVQsWssWsWWssWsWsWWssWWssWQsssVsssVQssWsPsssWssWsWQWWsWWssWssVWWWWWVWVWWWWWWWWWWWW",
           rounds0="LPssssLssssLsssssLssssLssssLssssLsssssLssssLssssLsssPQQQssPsssLsssssLssssLssssVsssVsWsssVssWssssLssssLssssLssWsssLssWssWQQQssssLssssLsWsWssssLsWssWssVssWWssWsWsWssVssWsWQsWsWsssVQssWWssWQsWsWsWsWsssVsWssPsWsssLssWWssssLsWssssLssPQsssVssWssVsWQssWssWssWWWQsWsWsWWssWVsWWWWWVVWWWWWWWWWWWWW",
           last_rounds="PsssssssssssssPsssssssssssssssssssssssPQQssssssssssssssssssPQsssVPssssssWWWssssssVsssWQssVsssssssWssssssssWQssWssssWQWsssssssVWssWssWssWQsssssssVssssWQWssWWsWssWWsssVsWWsssssWsWQsWssssVssWssWsWWsssssWsssWsWsWssVsWQsssssVssWQsssWssWsWQWsWsWsWsVsWWWWWVWVWWWWWWWWWWWW")

S, D = 2048, 640
LT = D // 128

AH, AD, AW, ADIL = 32, 20, 8, 2
HALO = 16
TB = 128
NB = S // TB
RC = 8

H, DH, M, SEG = 32, 192, 8, 32
L = M + SEG
HALF = SEG // 2
NP = H // 2
FT = 3 * NP
NSEG = S // SEG
LAM = (0.0, 0.625, -0.625, 1.875, -1.875)
PAIRS = [(i, j) for i in range(LT) for j in range(i + 1, LT)]
NZ = LT + len(PAIRS)
NG = 28
ZB = 4
GS = NG // ZB
ZS = (GS * LT + 1) * HALF
G0 = CFG["G0"]
UN, UT = CFG["UN"], CFG["UT"]
NBUF = max(UN, UT)
CG = 2
NCH = NG // CG
STEP = (432, 448, 512)
WO_STEP = 256
KC = CFG["kc"]
VLAG = 2


def _tile_order():
    order = []
    for p in range(NP + VLAG):
        if p < NP:
            order += [(j, 3 * p + t) for j in (0, 1) for t in range(3)]
        if p >= VLAG:
            order += [(2, 3 * (p - VLAG) + t) for t in range(3)]
    return order


TILES = _tile_order()
assert all((t + 1) * 128 <= H * DH - (NG // CG - 2 - n // (CG * LT)) * STEP[j] for n, (j, t) in enumerate(TILES))
NPL = len(TILES) - NG * LT

R_LHS = 0
R_H = R_LHS + NBUF * LT * LT * (M + HALF)
R_QKV = R_H + NBUF * LT * L
R_O = R_QKV + 3 * FT * L
R_P = R_O + FT * L
R_ACC = R_P + NP * 2 * L
R_S = R_ACC + LT * L
R_END = (R_S + NP * L + 31) // 32 * 32


def _make_plan(rounds, longs):
    shell = []
    for k in range(LT):
        for n in range(k + 1, LT):
            shell += [(k, n), (n, k)]
        shell += [(k, k)]
    todo = dict(
        L=longs,
        s=[("short", g, i, j) for g in range(NG) for (i, j) in shell],
        W=[("out", k0 + k, n) for k0 in range(0, FT, KC) for n in range(LT) for k in range(KC)],
        P=[("plain", n, k) for k in range(LT) for n in range(NPL)],
        Q=[("score", t) for t in range(FT)],
        V=[("pv", t) for t in range(FT)])
    plan, timed, now = [], [], 0

    def later(time, *task):
        timed.append((time, task))

    def flush(time):
        timed.sort(key=lambda x: x[0])
        while timed and timed[0][0] <= time:
            plan.append(timed.pop(0)[1])

    def needs(task):
        if task[0] == "out":
            return [("pv_end", task[1])]
        if task[0] not in ("score", "pv"):
            return []
        need = [("softmax", task[1] // 3, 5)] if task[0] == "pv" else []
        for j in (2,) if task[0] == "pv" else (0, 1):
            n = TILES.index((j, task[1]))
            need.append(("take", n // LT, n % LT, n % LT) if n < NG * LT else ("plain_end", n - NG * LT, LT - 1))
        return need

    for n, kind in enumerate(rounds):
        four = todo[kind][:4]
        del todo[kind][:4]
        need = [x for task in four for x in needs(task)]
        now = max([now] + [time for time, task in timed if task in need])
        flush(now)
        assert all(x in plan for x in need)
        plan += four
        now += dict(s=M + HALF if longs is not None else 30, L=ZB * HALF).get(kind, L)
        end = now + CFG["lat"]
        for name, *args in four:
            if name == "short":
                later(end, "take", *args)
            elif name == "out" and args[0] % KC == KC - 1:
                later(end, "out_end", *args)
            elif name in ("plain", "long", "pv"):
                later(end, name + "_end", *args)
            elif name == "score" and args[0] % 3 == 2:
                for step in range(6):
                    later(now + CFG["d_step"] * sum(x <= step for x in CFG["ties"]), "softmax", args[0] // 3, step)
        if kind not in rounds[n + 1:] and kind == "s":
            plan.append(("token_lhs",))
    assert not any(todo[kind] for kind in "sWPQV")
    return plan, [task for _, task in sorted(timed, key=lambda x: x[0])]


def _ds(i, n):
    return pl.ds(i * n if isinstance(i, int) else pl.multiple_of(i * n, n), n)


def _dot(a, b, dims=NN):
    r = lax.dot_general(a, b, dims, preferred_element_type=F32)
    return jnp.concatenate([r[0:8], r[8:]], axis=0)


def _share(tasks, k, n):
    return tasks[k * len(tasks) // n:(k + 1) * len(tasks) // n]


def _run(tasks):
    for task in tasks:
        task()


def _inverse(x):
    r = pltpu.reciprocal(x, approx=True)
    return r + r * (1.0 - x * r)


def _pack(x):
    return pltpu.bitcast(x.astype(BF16), U32)


def _kernel(ax_hbm, awqkv_hbm, awo_hbm, bx_hbm, mem_hbm, wq_hbm, wk_hbm, wv_hbm, wo_hbm,
            out_hbm,
            ax, awqkv, awo, tmp, wqkv_p, wo_p, q_s, kv_s, oa_s, xa, ob, outa,
            bx, mem, raw, wb, wz, wo, lz, z, buf, outb,
            sem_a, sem_w, sem_o):
    cp = pltpu.make_async_copy

    def rows_copy(src, dst, r0, r1, sem):
        return cp(src.at[pl.ds(r0, r1 - r0), :], dst.at[pl.ds(r0, r1 - r0), :], sem)

    c_wqkv = [cp(awqkv_hbm.at[:, pl.ds(j * D, D)], awqkv.at[j], sem_a.at[j]) for j in range(3)]
    c_awo = cp(awo_hbm, awo, sem_a.at[3])
    c_mem = cp(mem_hbm, mem.at[pl.ds(0, M), :], sem_a.at[4])
    c_outa = cp(outa, out_hbm.at[:, pl.ds(0, D)], sem_o.at[0])

    def c_rows(src, dst, first, i, n, sem):
        at = pl.ds(first + i * n if isinstance(i, int) else pl.multiple_of(first + i * n, 16), n)
        return cp(src.at[at, :], dst.at[at, :], sem)

    def c_x(i, sem):
        return [c_rows(ax_hbm, ax, 0, i, TB, sem), c_rows(bx_hbm, bx, 0, i, TB, sem)]

    def c_step(c):
        return c_x(c + 2, sem_w.at[c]) + [
            c_rows(w, raw.at[pl.ds(j * H * DH, H * DH), :], H * DH - (NCH - 2) * n, c - 1, n, sem_w.at[c])
            for j, (w, n) in enumerate(zip((wq_hbm, wk_hbm, wv_hbm), STEP))]

    c_first = c_x(2, sem_w.at[0]) + [
        c_rows(w, raw.at[pl.ds(j * H * DH, H * DH), :], 0, 0, H * DH - (NCH - 2) * STEP[j], sem_w.at[0]) for j, w in enumerate((wq_hbm, wk_hbm))]
    c_last = c_x(NB - 1, sem_w.at[NCH - 1]) + [c_mem]
    c_ax0, c_bx0 = c_x(0, sem_a.at[6])[0], c_x(0, sem_a.at[3])[1]

    def c_outb(r0, n):
        return cp(outb.at[pl.ds(r0, n), :], out_hbm.at[pl.ds(r0, n), pl.ds(D, D)], sem_o.at[1])

    def start(copies):
        for c in copies:
            c.start()

    def wait(copies):
        for c in copies:
            c.wait()

    def permute_rows(dst, base):
        for d in range(AD):
            for t in range(LT):
                dst[pl.ds((base + d * AH) // 2, AH // 2), t * 128:(t + 1) * 128] = _pack(
                    tmp[t, pl.ds(d, AH, stride=AD), :])

    def prep_wqkv(j):
        for t in range(LT):
            tmp[t] = awqkv[j, t * 128:(t + 1) * 128, :].astype(F32).T
        permute_rows(wqkv_p, j * D)

    def prep_wo():
        for t in range(LT):
            tmp[t] = awo[:, t * 128:(t + 1) * 128].astype(F32)
        permute_rows(wo_p, 0)

    def a_proj(i, j):
        acc = {}

        def tile(t, k):
            w = pltpu.bitcast(wqkv_p[(j * D + t * 128) // 2:(j * D + t * 128 + 128) // 2, k * 128:(k + 1) * 128], BF16)
            r = _dot(pltpu.bitcast(xa[k], BF16), w, NT)
            acc[t] = acc[t] + r if k else r
            return r

        def end(t):
            if j == 0:
                q_s[t] = acc[t]
                return
            c = (j - 1) * LT + t
            if isinstance(i, int) and i == 0:
                kv_s[c, 0:HALO, :] = jnp.broadcast_to(acc[t][0:1, :], (HALO, 128))
            else:
                kv_s[c, 0:HALO, :] = kv_s[c, TB:TB + HALO, :]
            kv_s[c, HALO:HALO + TB, :] = acc[t]
        return [(TB, functools.partial(tile, t, k), functools.partial(end, t) if k == LT - 1 else None)
                for t in range(LT) for k in range(LT)]

    def a_input(i):
        for k in range(LT):
            xa[k] = pltpu.bitcast(ax[_ds(i, TB), k * 128:(k + 1) * 128], U32)

    def a_attention(i):
        state = {}

        def window(c, r0, w):
            lo = HALO + r0 - ADIL * w
            return kv_s[c, lo:lo + RC, :]

        def logits(r0, half, late):
            q = [q_s[t, r0:r0 + RC, :] for t in range(LT)]
            q[0] = late(q[0])
            for w in range(half * AW // 2, (half + 1) * AW // 2):
                a = q[0] * window(0, r0, w)
                for t in range(1, LT):
                    a = a + q[t] * window(t, r0, w)
                a = a + pltpu.roll(a, 2 * AH, 1)
                a = (a + pltpu.roll(a, AH, 1)) * (AD ** -0.5)
                if isinstance(i, int) and i == 0 and r0 < ADIL * w:
                    pos = lax.broadcasted_iota(jnp.int32, (RC, 128), 0) + r0
                    a = jnp.where(pos >= ADIL * w, a, MASKED)
                state.setdefault(r0, []).append(a)

        def weights(r0, late):
            m = late(functools.reduce(jnp.maximum, state[r0]))
            state[r0] = [jnp.exp(a - m) for a in state[r0]]

        def mix(r0, tiles, late):
            e = [late(state[r0][0])] + state[r0][1:]
            if 0 in tiles:
                state[r0, "inv"] = _inverse(functools.reduce(jnp.add, e))
            for t in tiles:
                o = e[0] * window(LT + t, r0, 0)
                for w in range(1, AW):
                    o = o + e[w] * window(LT + t, r0, w)
                oa_s[t, r0:r0 + RC, :] = o * state[r0, "inv"]

        stages = ((logits, 0), (logits, 1), (weights,), (mix, (0, 1)), (mix, (2, 3, 4)))
        return [[functools.partial(f, r0, *args) for r0 in range(0, TB, RC)] for f, *args in stages]

    def a_attention_now(i):
        for tasks in zip(*a_attention(i)):
            for task in tasks:
                task(lambda x: x)

    def a_pack():
        def pack(k):
            ob[k] = _pack(oa_s[k])
        return [functools.partial(pack, k) for k in range(LT)]

    def a_out(i):
        acc = {}

        def tile(t, k):
            r = _dot(pltpu.bitcast(ob[k], BF16), pltpu.bitcast(wo_p[k * 64:(k + 1) * 64, t * 128:(t + 1) * 128], BF16))
            acc[t] = acc[t] + r if k else r
            return r

        def end(t):
            outa[_ds(i, TB), t * 128:(t + 1) * 128] = acc[t].astype(BF16)
        return [(TB, functools.partial(tile, t, k), functools.partial(end, t) if k == LT - 1 else None)
                for t in range(LT) for k in range(LT)]

    def overlap(tiles, side=(), zero=None):
        due = sorted((lo + (hi - lo) * n / len(tasks), m, n, task, ref)
                     for m, (lo, hi, tasks, ref) in enumerate(side) for n, task in enumerate(tasks))
        free = [0] * 4
        for count, tile, end in tiles:
            now = min(free)
            free[free.index(now)] += count
            r = tile()
            while due and due[0][0] < min(free):
                time, _, _, task, ref = due.pop(0)
                row = max(0, int(time - now)) // 8 * 8
                if isinstance(ref, str):
                    task(lambda x: jnp.where(zero == 0, x, r[row:row + 8]))
                    continue
                if ref is bx:
                    ref[pl.ds(pl.multiple_of(S + 16 * zero, 16), 16), 0:128] = r[row // 16 * 16:row // 16 * 16 + 16].astype(BF16)
                elif ref is not None:
                    ref[(ref.shape[0] - 1 - zero,) + (0,) * (len(ref.shape) - 3) + (slice(0, 8),)] = (
                        pltpu.bitcast(r[row:row + 8], ref.dtype))
                task()
            if end:
                end()
        assert not due

    def w_transpose(c, n):
        size = CG * LT if not isinstance(c, int) else NPL
        first = c * CG * LT
        at = [FT * j + t for j, t in TILES[n::CG * LT]]
        if isinstance(c, int):
            at = at[c]
        else:
            words = [sum(x << 8 * k for k, x in enumerate(at[m::5])) for m in range(5)]
            word = functools.reduce(lambda x, m: jnp.where(lax.rem(c, 5) == m, words[m], x), range(1, 5), words[0])
            at = lax.shift_right_logical(word, lax.div(c, 5) * 8) & 255
        wb.at[pl.ds(first, size)][n] = pltpu.bitcast(raw[_ds(at, 128), :].T, U32)

    def w_combine(c, u, r, i):
        tiles, dst = wb.at[pl.ds(c * CG * LT, CG * LT)], wz.at[pl.ds(c * CG, CG)]

        def rows(i):
            return slice(i * 64 + 8 * r, i * 64 + 8 * r + 8)

        def tile(i, j):
            return pltpu.bitcast(tiles[u * LT + j, rows(i), :], BF16).astype(F32)
        row = col = tile(i, i)
        for k in range(LT):
            if k != i:
                a, b = tile(i, k), tile(k, i)
                row, col = row - a, col - b
                if k > i:
                    dst[u, LT + PAIRS.index((i, k)), rows(0), :] = _pack(a - b)
        dst[u, i, rows(0), :] = _pack(row)
        dst[u, NZ + i, rows(0), :] = _pack(col)

    def halves(s):
        x = bx[_ds(s, SEG), :].astype(F32)
        return [[x[r:r + HALF, i * 128:(i + 1) * 128] for i in range(LT)] for r in (0, HALF)]

    def z_lhs(s, i):
        a, b = halves(s)
        p = [a[k] + LAM[k] * b[k] if LAM[k] else a[k] for k in range(LT)]
        dst = lz.at[:, _ds(s, HALF // 2), :]
        dst[i] = _pack(b[i])
        for k in ((i + 1) % LT, (i + 2) % LT):
            lo, hi = sorted((i, k))
            dst[LT + PAIRS.index((lo, hi))] = _pack((p[lo] + p[hi]) * (1.0 / (LAM[lo] - LAM[hi])))

    def z_batch(t):
        return [functools.partial(z_lhs, t * ZB + u, i) for u in range(ZB) for i in range(LT)]

    def z_product(g, n, batch):
        return _dot(pltpu.bitcast(lz[n, _ds(batch, ZB * HALF // 2), :], BF16), pltpu.bitcast(wz[g, n], BF16))

    def z_group(g, batch):
        dst = z.at[z_index(g, batch)]

        def tile(n):
            r = z_product(g, n, batch)
            z_add(dst, n, r)
            return r
        return [(ZB * HALF, functools.partial(tile, n), None) for n in range(NZ)]

    def z_add(dst, n, r):
        for i in (n,) if n < LT else PAIRS[n - LT]:
            for u in range(ZB):
                x = r[u * HALF:(u + 1) * HALF]
                dst[u, i * HALF:(i + 1) * HALF, :] = x if n < LT else x + dst[u, i * HALF:(i + 1) * HALF, :]

    def z_index(g, batch):
        if isinstance(batch, int) and batch == 0:
            return g
        if isinstance(g, int) and g >= G0:
            return g + (batch % 2) * (NG - G0)
        return jnp.where(batch == 0, g, 2 * (NG - G0) + batch * G0 + g)

    if not CFG.get('onlyB'):
        start([c_wqkv[0], c_ax0, c_wqkv[1]])
        c_wqkv[0].wait()
        c_wqkv[2].start()
        prep_wqkv(0)
        wait([c_ax0, c_wqkv[1]])
        start([c_awo, c_bx0] + c_x(1, sem_a.at[3]))
        a_input(0)
        overlap(a_proj(0, 0))
        prep_wqkv(1)
        c_wqkv[2].wait()
        start(c_first)
        overlap(a_proj(0, 1))
        prep_wqkv(2)
        overlap(a_proj(0, 2))
        wait([c_awo, c_bx0] + c_x(1, sem_a.at[3]))
        a_attention_now(0)
        prep_wo()
        for t in range(G0 // 2):
            _run(z_batch(t))
        a_input(1)
        _run(a_pack())
        overlap(a_proj(1, 0) + a_proj(1, 1) + a_proj(1, 2) + a_out(0))
        start(c_step(1))
        a_attention_now(1)
        wait(c_first)

        def a_step(c, carry):
            whole = raw.at[pl.ds(0, sum(STEP) + 2 * TB), :]
            pl.when((c > 0) & (c < NCH - 1))(cp(whole, whole, sem_w.at[c]).wait)

            @pl.when(c < NCH - 3)
            def _():
                start(c_step(c + 2) + [c_rows(wo_hbm, wo, 0, c, WO_STEP, sem_a.at[5])])

            @pl.when(c >= NCH - 3)
            def _():
                pl.when(c == NCH - 3)(lambda: start(c_last))
                pl.when(c == NCH - 1)(lambda: wait(c_last))
                first = (NCH - 3) * WO_STEP
                pl.when(c < NCH - 1)(
                    lambda: c_rows(wo_hbm, wo, first, c - (NCH - 3), (H * DH - first) // 2, sem_a.at[5]).start())
            zero = lax.shift_right_logical(c, 16)
            a_input(c + 2)
            f = CFG["f"]
            if G0 == 2:
                early = z_group(0, c + 1) + z_group(1, c + 1)
            else:
                early = [x for u in range(2) for t in range(2) for x in z_group((c & 1) * 2 + u, (c | 1) + t)]
            overlap(a_proj(c + 2, 0) + a_proj(c + 2, 1) + a_proj(c + 2, 2) + a_out(c + 1)
                    + z_group(c * CG, 0) + early + z_group(c * CG + 1, 0), [
                (0, f[0], [functools.partial(w_transpose, c, n) for n in range(CG * LT)], None),
                (0, f[1], z_batch(c + G0 // 2), bx),
                (0, f[1], a_pack(), oa_s),
                (f[1], f[2], [functools.partial(w_combine, c, u, r, i)
                              for u in range(CG) for r in range(8) for i in range(LT)], wb),
            ] + [(f[3] + d, f[4] + d, tasks, "value") for d, tasks in zip(CFG["lags"], a_attention(c + 2))], zero)
            return carry

        lax.fori_loop(0, NCH, a_step, 0)
        for t in range(NCH + G0 // 2, NSEG // ZB):
            _run(z_batch(t))
        for n in range(NPL):
            w_transpose(NCH, n)
        _run(a_pack())
        overlap(a_out(NB - 1) + [x for g in range(G0) for x in z_group(g, NSEG // ZB - 1)])

    def rows(r0, n):
        return slice(r0, r0 + n)

    def r_lhs(hb, i, j):
        return R_LHS + ((hb * LT + i) * LT + j) * (M + HALF)

    def r_qkv(j, t):
        return rows(R_QKV + (j * FT + t) * L, L)

    def token_lhs(s, hb):
        a, b = halves(s)
        for j in range(LT):
            buf[rows(R_H + (hb * LT + j) * L + M, SEG)] = jnp.concatenate([a[j], b[j]], axis=0)
            p = [a[i] + LAM[j] * b[i] if LAM[j] else a[i] for i in range(LT)]
            for i in range(LT):
                buf[rows(r_lhs(hb, i, j) + M, HALF)] = (
                    p[j] if i == j else (p[i] + p[j]) * (1.0 / (LAM[j] - LAM[i])))

    def memory_lhs(m, n, hb):
        buf[rows(R_H + (hb * LT + n) * L, M)] = m[n]
        buf[rows(r_lhs(hb, n, n), M)] = m[n]
        for k in range(n):
            buf[rows(r_lhs(hb, n, k), M)] = buf[rows(r_lhs(hb, k, n), M)] = m[n] + m[k]

    def segment(plan, batch, part, hb, nh, before=()):
        s = batch * ZB + part
        key = lax.broadcasted_iota(jnp.int32, (L, 128), 0)
        col = lax.broadcasted_iota(jnp.int32, (L, 128), 1)
        head0 = col < L
        query = jnp.where(head0, col, col - L)
        visible = (query < M) | (query >= key)
        low = lax.broadcasted_iota(jnp.int32, (L, 128), 1) < 64
        val = {}
        z_next = z.at[pl.ds(z_index(G0, batch + 1), NG - G0)]
        new_mem = []

        def add(name, x):
            val[name] = val[name] + x if name in val else x

        def product(*args):
            r = _dot(*args)
            val["latest"] = r[-8:]
            return r

        def short(g, i, j):
            w = pltpu.bitcast(wz[g, NZ + i] if i == j else wb[g * LT + j, rows(i * 64, 64), :], BF16)
            val[g, i, j] = product(buf[rows(r_lhs(hb, i, j), M + HALF)], w)

        def take(g, i, j):
            r = val.pop((g, i, j))
            add(("m", g, j), r[0:M])
            if i != j:
                add(("y", g, i), r[M:])
                add(("d", g, j), r[M:])
                if LAM[i]:
                    add(("c", g, j), r[M:] * -LAM[i])
                return
            y = z[z_index(g, batch), part, rows(j * HALF, HALF), :] + val.pop(("y", g, j))
            c = val.pop(("c", g, j)) + r[M:]
            if LAM[j]:
                c = c - LAM[j] * y
            buf[r_qkv(*TILES[g * LT + j])] = jnp.concatenate(
                [val.pop(("m", g, j)), c, val.pop(("d", g, j)) + y], axis=0)

        def plain(n, k):
            w = pltpu.bitcast(wb[NG * LT + n, rows(k * 64, 64), :], BF16)
            val["plain", n, k] = product(buf[rows(R_H + (hb * LT + k) * L, L)], w)

        def plain_end(n, k):
            dst = r_qkv(*TILES[NG * LT + n])
            r = val.pop(("plain", n, k))
            buf[dst] = r + buf[dst] if k else r

        def long(g, n):
            val["long", g, n] = z_product(g, n, batch + 1)
            val["latest"] = val["long", g, n][24:32]

        def long_end(g, n):
            z_add(z_next.at[g - G0], n, val.pop(("long", g, n)))

        def score(t):
            q = buf[r_qkv(0, t)]
            none = jnp.zeros((L, 128), F32)
            q = ((q, none), (jnp.where(low, q, 0.0), jnp.where(low, 0.0, q)), (none, q))[t % 3]
            q = jnp.concatenate(q + (jnp.zeros((128 - 2 * L, 128), F32),), axis=0)
            add(("s", t // 3), product(buf[r_qkv(1, t)], q.astype(BF16), NT))

        def softmax(p, step):
            def late(x):
                return jnp.where(col[0:8] < 2 * L, x, val["latest"]) if step in CFG["ties"] else x

            def groups(x):
                return [x[r:r + 8] for r in range(0, L, 8)]

            def spread(x):
                return jnp.concatenate([x] * (L // 8), axis=0)
            x, y = val["s", p], val.get(("t", p))
            if step == 0:
                x = jnp.where(visible, x * (DH ** -0.5), MASKED)
                y = functools.reduce(jnp.maximum, groups(x))
            elif step == 1:
                y = jnp.broadcast_to(jnp.max(late(y), axis=0, keepdims=True), (8, 128))
            elif step == 2:
                x = jnp.exp(x - spread(late(y)))
                y = functools.reduce(jnp.add, groups(x))
            elif step == 3:
                y = jnp.broadcast_to(jnp.sum(late(y), axis=0, keepdims=True), (8, 128))
            elif step == 4:
                y = _inverse(late(y))
            else:
                x = x * spread(late(y))
                x = jnp.concatenate([x, x], axis=0)[:, 0:2 * L]
                buf[rows(R_P + p * 2 * L, 2 * L), 0:2 * L] = x.astype(BF16).T.astype(F32) if CFG.get("xp16", 1) else x.T
            val["s", p], val["t", p] = x, y

        def pv(t):
            pa, pb = [buf[rows(R_P + (2 * (t // 3) + u) * L, L), 0:2 * L] for u in range(2)]
            v = buf[r_qkv(2, t)]
            if t % 3 == 1:
                v = jnp.concatenate([jnp.where(low, v, 0.0), jnp.where(low, 0.0, v)], axis=0)
            pr = (pa[:, 0:L], jnp.where(head0[:, 0:2 * L], pa, pb), pb[:, 0:L])[t % 3]
            val["o", t] = product(pr, v.astype(BF16))

        def pv_end(t):
            buf[rows(R_O + t * L, L)] = val.pop(("o", t))

        def out(t, n):
            add(("out", t // KC, n), product(buf[rows(R_O + t * L, L)], wo[rows(t * 128, 128), rows(n * 128, 128)]))

        def out_end(t, n):
            r = val.pop(("out", t // KC, n))
            if t >= KC:
                r = r + buf[rows(R_ACC + n * L, L)]
            if t < FT - 1:
                buf[rows(R_ACC + n * L, L)] = r
                return
            new_mem.append(r[0:M])
            memory_lhs(new_mem, n, nh)
            outb[_ds(s, SEG), rows(n * 128, 128)] = r[M:L].astype(BF16)

        tasks = dict(short=short, take=take, plain=plain, plain_end=plain_end, long=long, long_end=long_end,
                     score=score, softmax=softmax, pv=pv, pv_end=pv_end,
                     out=out, out_end=out_end,
                     token_lhs=lambda: token_lhs(jnp.minimum(s + 1, NSEG - 1), nh))
        before = list(before)
        for name, *args in plan[0]:
            need = max(args[1:]) if name in ("short", "plain") else -1
            while len(before) > LT - 1 - need:
                before.pop(0)()
            tasks[name](*args)
        return [functools.partial(tasks[name], *args) for name, *args in plan[1]]

    if CFG.get('onlyB'):
        start(c_first + [cp(wo_hbm, wo, sem_a.at[5]), c_mem])
        w_transpose(0, 0)
        w_combine(0, 0, 0, 0)
        z_lhs(0, 0)
        overlap(z_group(0, 0))
    token_lhs(0, 0)
    mem0 = mem[0:M, :].astype(F32)
    for n in range(LT):
        memory_lhs([mem0[:, k * 128:(k + 1) * 128] for k in range(LT)], n, 0)

    longs = [("long", g, n) for g in range(G0, NG) for n in range(NZ)]
    main_plans = [_make_plan(CFG["rounds"] if u % 2 else CFG["rounds0"], longs) for u in range(UN)]
    assert not longs or UN < ZB
    last_plan = _make_plan(CFG["last_rounds"], None)
    n_main = NSEG // ZB - 1

    def b_step(it, carry):
        rest = ()
        for u in range(UN):
            rest = segment(main_plans[u], it, u, u, (u + 1) % UN, rest)
        _run(rest)
        c_outb(pl.multiple_of(it * ZB * SEG, SEG), ZB * SEG).start()
        return carry

    def last_step(s, carry):
        _run(segment(last_plan, s // ZB, s % ZB, 0, 0))
        c_outb(pl.multiple_of(s * SEG, SEG), SEG).start()
        return carry

    cp(wo, wo, sem_a.at[5]).wait()
    c_outa.start()
    if CFG.get('onlyB') != 2 and not CFG.get('onlyA'):
        lax.fori_loop(0, n_main, b_step, 0)
    if CFG.get('onlyB') != 1 and not CFG.get('onlyA'):
        lax.fori_loop(n_main * ZB, NSEG, last_step, 0)
    if CFG.get('onlyA'):
        outb[0:16, 0:128] = (z[0, 0, 0:16] + pltpu.bitcast(wb[0, 0:16], F32) + buf[0:16] + pltpu.bitcast(lz[0, 32:48], F32)).astype(BF16)
        start([c_outb(0, S)])
    c_outa.wait()
    c_outb(0, S).wait()


def pallas_concat_heads__sliding_local_dilated__memory_aug_recurrent_mem_tr__prompt_kernel(
    A_x, A_wqkv, A_wo, B_x, B_mem0, B_Wq, B_Wk, B_Wv, B_Wo, B_seg_len,
):
    assert B_seg_len == SEG
    assert A_x.shape == B_x.shape == (1, S, D) and B_mem0.shape == (1, M, D)
    assert B_Wq.shape == B_Wk.shape == B_Wv.shape == (D, H, DH) and B_Wo.shape == (H, DH, D)
    vmem, dma = pltpu.VMEM, pltpu.SemaphoreType.DMA
    call = pl.pallas_call(
        _kernel,
        out_shape=jax.ShapeDtypeStruct((S, 2 * D), BF16),
        in_specs=[pl.BlockSpec(memory_space=pl.ANY)] * 9,
        out_specs=pl.BlockSpec(memory_space=pl.ANY),
        scratch_shapes=[
            vmem((S, D), BF16),
            vmem((3, D, D), BF16),
            vmem((D, D), BF16),
            vmem((LT, D, 128), F32),
            vmem((3 * D // 2, D), U32),
            vmem((D // 2, D), U32),
            vmem((LT + 1, TB, 128), F32),
            vmem((2 * LT, HALO + TB, 128), F32),
            vmem((LT + 1, TB, 128), F32),
            vmem((LT, TB // 2, 128), U32),
            vmem((LT, TB // 2, 128), U32),
            vmem((S, D), BF16),
            vmem((S + 64, D), BF16),
            vmem((64, D), BF16),
            vmem((3 * H * DH, D), BF16),
            vmem((len(TILES) + 1, D // 2, 128), U32),
            vmem((NG, NZ + LT, 64, 128), U32),
            vmem((H * DH, D), BF16),
            vmem((NZ, S // 4, 128), U32),
            vmem((2 * (NG - G0) + NSEG // ZB * G0, ZB, LT * HALF, 128), F32),
            vmem((R_END, 128), F32),
            vmem((S, D), BF16),
            dma((7,)), dma((NCH,)), dma((2,)),
        ],
        compiler_params=pltpu.CompilerParams(vmem_limit_bytes=126 * 1024 * 1024,
                                             internal_scratch_in_bytes=48 * 1024, disable_bounds_checks=True),
        name="sliding_and_memory_attention",
    )

    def by_feature(w):
        return w.transpose(1, 2, 0).reshape(H * DH, D)

    out = call(A_x.reshape(S, D), A_wqkv, A_wo, B_x.reshape(S, D), B_mem0.reshape(M, D),
               by_feature(B_Wq), by_feature(B_Wk), by_feature(B_Wv), B_Wo.reshape(H * DH, D))
    return out.reshape(1, S, 2 * D)
```

```python
import functools

import jax
import jax.numpy as jnp
from jax import lax
from jax.experimental import pallas as pl
from jax.experimental.pallas import tpu as pltpu

F32, BF16, U32 = jnp.float32, jnp.bfloat16, jnp.uint32
NN = (((1,), (0,)), ((), ()))
NT = (((1,), (1,)), ((), ()))
MASKED = -1000000000.0
CFG = dict(UN=4, UT=1, G0=4, lags0=[0, 22, 120, 142, 330, 500, 510], lags1=[0, 22, 120, 142, 330, 600, 620], h=[500, 0, 1700], n1=7, e=[300, 1000, 1700], WG=2, trim=0, d_lhs=48, fence=[], d_p=0, lag="2222222233334444", pl=4, f=[1240, 600, 2700, 2391, 4199], lags=[2, 50, 174, 227, 346, 364, 416], cuts=[2, 3, 4, 6, 7, 8, 10, 11, 12, 14, 15, 16, 17, 18, 19], vlag=2, kc=3, lat=120, ties=[1, 2, 3, 4, 5], d_step=24, d_norm=280,
           r0="PsLsssssLsssssLssPsssLssssLQssssLssssLssssLQssssLssPsssLsssssLssPQsPsssVssssLssssLssssLssssLssssVQssssLssssLssssVQssssLssssLssWsWQsssVssssLsWssssLssssLssssVssWQsWsWsssVQsWsWsWssWQsWsWsWsssVssssLssWWsWsWsWssssLssssVsWQssWsWsWQsWsssVsWsWsWsWsWQsssWWsWssVsWwsWwWswVsWsWwWwwWwVwWwWwWwWwwWWWWW",
r1="LPssPsssLssssLssssLssssLssssLssssLsPssssLssssLQsPssssLQssssLssssLssssLssssLssssVQsPssssLssssLssssLssssLssssVQssssLssssVQssssLssssLsWsWssssLssssVQssssLsWssssLssssLsWssssVsWQssWsWsssVQsWsWsWsWsWsWssWQsWsWsssVsWssWQsWsssVsWsWsWsWsWsssVQssWWsWssWQsssWWWswsVssWwWsWssVwWsWwWWwwwVwWwwWWWwWwwWWWW",
r2="LPssssLssPsssLssssLssssLQssssLssssLQssPPssssLssssLssssLssssLssssVQssssLssssLssPsssLssssVQssssLssssVQsssssLssssLssWQsssVsssssLsssssLssssLssWsssVQsWsWssWWsssVQssssLsWsWssWWsWssWWssWsssLssWQsssVssWssssLssWsWsssLsWssWsssVsWssWQsWsWsssVQsWsWsWssWQsssWWWwswVsWssWWsWswVsWwsWwWWwwVwWwwWWwwWwWWWW",
r3="LPssPsssLssssLssssLssssLssssLssssLsPssssLssssLQsPssssLQssssLssssLssssLssssLssssVQsPssssLssssLssssLssssLssssVQssssLssssVQssssLssssLsWsWssssLssssVQssssLsWssssLssssLsWssssVsWQssWsWsssVQsWsWsWsWsWsWssWQsWsWsssVsWssWQsWsssVsWsWsWsWsWsssVQssWWsWssWQsssWWWswsVssWwWsWssVwWsWwWWwwwVwWwwWWWwWwwWWWW",
           last_rounds="PsssssssssssssssssssssssssPQQssPssssssssssssssPPQssssssssVsssssWWsssssVWsssWQssWssVsssWssWQssssssWWQssWssssssVssWsWssssssWssVsWssssssWWsWssssssWsVssWsssssWsWQQssssssWssWWssssWQsssVsWsWsssWssWWssWssssWsWsVsssWQssWQsWssVsWssWssWsWQssWssWWWssssVssWsWsVWWWWVWWWWWWWWWW")

S, D = 2048, 640
LT = D // 128

AH, AD, AW, ADIL = 32, 20, 8, 2
HALO = 16
TB = 128
NB = S // TB
NS = 2
RC = 8

H, DH, M, SEG = 32, 192, 8, 32
L = M + SEG
HALF = SEG // 2
NP = H // 2
FT = 3 * NP
NSEG = S // SEG
LAM = (0.0, 0.625, -0.625, 1.875, -1.875)
PAIRS = [(i, j) for i in range(LT) for j in range(i + 1, LT)]
NZ = LT + len(PAIRS)
NG = 28
ZB = 4
GS = NG // ZB
ZS = (GS * LT + 1) * HALF
G0 = CFG["G0"]
UN, UT = CFG["UN"], CFG["UT"]
NBUF = max(UN, UT)
CG = 2
NCH = NG // CG
FIRST, STEP = (864, 864, 0), (480, 480, 448)
NST = NCH - 2
WO_STEP = 256
WO_FIRST = (NST - 3) * WO_STEP
KC = CFG["kc"]
VLAG = 2
WG = CFG["WG"]


def _tile_order():
    lag = [int(x) for x in str(CFG["lag"])]
    order = []
    for p in range(NP + max(lag)):
        if p < NP:
            order += [(j, 3 * p + t) for j in (0, 1) for t in range(3)]
        order += [(2, 3 * x + t) for x in range(NP) if x + lag[x] == p for t in range(3)]
    plain = [(2, t) for t in range(CFG["pl"], CFG["pl"] + 4)]
    order = [x for x in order if x not in plain] + plain
    return order


TILES = _tile_order()
assert all((t + 1) * 128 <= FIRST[j] + n // (CG * LT) * STEP[j] for n, (j, t) in enumerate(TILES[:NST * CG * LT]))
NPL = len(TILES) - NG * LT

R_LHS = 0
R_H = R_LHS + NBUF * LT * LT * (M + HALF)
R_QKV = R_H + NBUF * LT * L
R_O = R_QKV + 3 * FT * L
R_P = R_O + FT * L
R_ACC = R_P + NP * 2 * L
R_OL = R_ACC + LT * L
R_END = (R_OL + WG * LT * LT * (M + HALF) + 31) // 32 * 32


def _make_plan(rounds, longs):
    shell = []
    for k in range(LT):
        for n in range(k + 1, LT):
            shell += [(k, n), (n, k)]
        shell += [(k, k)]
    fast = WG if longs is not None else 0
    todo = dict(
        L=longs,
        s=[("short", g, i, j) for g in range(NG) for (i, j) in shell],
        w=[("short", NG + g, i, j) for (i, j) in shell for g in range(fast)],
        W=[("out", t, n) for k1 in range(FT % KC, FT + 1, KC) for n in range(LT) for t in range(max(k1 - KC, fast * LT), k1)],
        P=[("plain", n, k) for k in range(LT) for n in range(NPL)],
        Q=[("score", t) for t in range(FT)],
        V=[("pv", t) for t in range(FT)])
    plan, timed, now = [], [], 0

    def later(time, *task):
        timed.append((time, task))
        timed.sort(key=lambda x: x[0])

    def flush(time):
        timed.sort(key=lambda x: x[0])
        while timed and timed[0][0] <= time:
            plan.append(timed.pop(0)[1])

    def needs(task):
        if task[0] == "out":
            return [("pv_end", task[1])]
        if task[0] == "short" and task[1] >= NG:
            return [("out_lhs_end", task[1] - NG, task[3])]
        if task[0] not in ("score", "pv"):
            return []
        need = [("softmax", task[1] // 3, 6)] if task[0] == "pv" else []
        for j in (2,) if task[0] == "pv" else (0, 1):
            n = TILES.index((j, task[1]))
            need.append(("take", n // LT, n % LT, n % LT) if n < NG * LT else ("plain_end", n - NG * LT, LT - 1))
        return need

    for n, kind in enumerate(rounds):
        four = todo[kind][:4]
        del todo[kind][:4]
        while kind == "w" and len(four) < 4:
            four.append(todo["W"].pop(0))
        need = [x for task in four for x in needs(task)]
        for need_time, needed in [x for x in timed if x[1] in need]:
            key = needed[:2] if needed[0] == "softmax" else needed[:1]
            timed[:] = [(min(time, now) if task[:len(key)] == key and time <= need_time else time, task)
                        for time, task in timed]
        flush(now)
        assert all(x in plan for x in need)
        plan += four
        now += dict(s=M + HALF if longs is not None else 30, w=M + HALF, L=ZB * HALF).get(kind, L)
        end = now + CFG["lat"]
        for name, *args in four:
            if name == "short":
                later(end, "take", *args)
            elif name == "out" and args[0] % KC == KC - 1:
                later(end, "out_end", *args)
            elif name in ("plain", "long", "pv"):
                later(end, name + "_end", *args)
                if name == "pv" and args[0] < fast * LT and args[0] % LT == LT - 1:
                    for j in range(LT):
                        later(end + CFG["d_lhs"] * j, "out_lhs", args[0] // LT, j)
                        later(end + CFG["d_lhs"] * j + CFG["lat"], "out_lhs_end", args[0] // LT, j)
            elif name == "score" and args[0] % 3 == 2:
                for step in range(6):
                    later(now + CFG["trim"] + CFG["d_step"] * sum(x <= step for x in CFG["ties"]), "softmax", args[0] // 3, step)
                later(now + CFG["d_step"] * 6 + 10000, "softmax", args[0] // 3, 6)
        if kind not in rounds[n + 1:] and kind == "s":
            plan.append(("token_lhs",))
    assert not any(todo[kind] for kind in "swWPQV")
    return plan, [task for _, task in sorted(timed, key=lambda x: x[0])]


def _ds(i, n):
    return pl.ds(i * n if isinstance(i, int) else pl.multiple_of(i * n, n), n)


def _dot(a, b, dims=NN):
    r = lax.dot_general(a, b, dims, preferred_element_type=F32)
    return jnp.concatenate([r[0:8], r[8:]], axis=0)


def _share(tasks, k, n):
    return tasks[k * len(tasks) // n:(k + 1) * len(tasks) // n]


def _mark(name):
    if CFG.get("trace"):
        with jax.named_scope(name):
            pl.delay(1)


def _run(tasks):
    for task in tasks:
        task()


def _inverse(x):
    r = pltpu.reciprocal(x, approx=True)
    return r + r * (1.0 - x * r)


def _load(ref, *index):
    return pltpu.bitcast(ref.bitcast(U32)[index], BF16)


def _kernel(ax_hbm, awqkv_hbm, awo_hbm, bx_hbm, mem_hbm, wq_hbm, wk_hbm, wv_hbm, wo_hbm,
            out_hbm,
            ax, awqkv, awo, tmp, wqkv_p, wo_p, q_s, kv_s, oa_s, ob, outa,
            bx, mem, raw, wb, wz, wo, lz, z, lo, zo, op, buf,
            flag, sem_a, sem_w, sem_o):
    cp = pltpu.make_async_copy
    outb = raw.at[pl.ds(0, S), :]

    def rows_copy(src, dst, r0, r1, sem):
        return cp(src.at[pl.ds(r0, r1 - r0), :], dst.at[pl.ds(r0, r1 - r0), :], sem)

    c_wqkv = [cp(awqkv_hbm.at[:, pl.ds(j * D, D)], awqkv.at[j], sem_a.at[j]) for j in range(3)]
    c_awo = cp(awo_hbm, awo, sem_a.at[3])
    c_mem = cp(mem_hbm, mem.at[pl.ds(0, M), :], sem_a.at[4])
    c_outa = cp(outa, out_hbm.at[:, pl.ds(0, D)], sem_o.at[0])

    def c_rows(src, dst, first, i, n, sem):
        at = pl.ds(first + i * n if isinstance(i, int) else pl.multiple_of(first + i * n, 16), n)
        return cp(src.at[at, :], dst.at[at, :], sem)

    def c_wo(first, i, n, sem):
        at = pl.ds(pl.multiple_of(first + i * n, 16), n)
        return [cp(wo_hbm.at[at, pl.ds(t * 128, 128)], wo.at[t, at, :], sem) for t in range(LT)]

    def wo_rows(r0, n, t):
        return _load(wo, t, slice(r0 // 2, (r0 + n) // 2))

    def c_ax(i, n, sem):
        return [cp(ax_hbm.at[_ds(i, n), pl.ds(t * 128, 128)], ax.at[t, _ds(i, n), :], sem) for t in range(LT)]

    def c_x(c, sem):
        return c_ax(c + NS, TB, sem) + [c_rows(bx_hbm, bx, 0, c + 2, TB, sem)]

    def c_w(j, first, i, n, c):
        return c_rows((wq_hbm, wk_hbm, wv_hbm)[j], raw.at[pl.ds(j * H * DH, H * DH), :], first, i, n, sem_w.at[c])

    def c_step(c):
        return c_x(c, sem_w.at[c]) + [c_w(j, FIRST[j], c - 1, STEP[j], c) for j in range(3)]

    c_first = c_x(0, sem_w.at[0]) + [c_w(j, 0, 0, FIRST[j], 0) for j in range(2)]
    c_last = c_x(NST, sem_w.at[NST]) + c_x(NST + 1, sem_w.at[NST]) + [
        c_mem, c_w(2, (NST - 1) * STEP[2], 0, H * DH - (NST - 1) * STEP[2], NST)]
    c_bx0 = c_rows(bx_hbm, bx, 0, 0, 2 * TB, sem_a.at[2])

    def c_outb(r0, n):
        return cp(outb.at[pl.ds(r0, n), :], out_hbm.at[pl.ds(r0, n), pl.ds(D, D)], sem_o.at[1])

    def start(copies):
        for c in copies:
            c.start()

    def wait(copies):
        for c in copies:
            c.wait()

    def permute_rows(dst, base):
        def move(t, d0):
            for d in range(d0, d0 + AD // 4):
                dst[t, pl.ds(base + d * AH, AH), :] = tmp[t, pl.ds(d, AH, stride=AD), :].astype(BF16)
        return [functools.partial(move, t, d0) for t in range(LT) for d0 in range(0, AD, AD // 4)]

    def prep_wqkv(j):
        def transpose(t):
            tmp[t] = awqkv[j, t * 128:(t + 1) * 128, :].astype(F32).T
        return [functools.partial(transpose, t) for t in range(LT)], permute_rows(wqkv_p, j * D)

    def prep_wo():
        def widen(t, r):
            tmp[t, r:r + D // 4, :] = awo[r:r + D // 4, t * 128:(t + 1) * 128].astype(F32)
        moves = permute_rows(wo_p, 0)
        return [task for t in range(LT)
                for task in [functools.partial(widen, t, r) for r in range(0, D, D // 4)] + moves[4 * t:4 * t + 4]]

    def slot(i):
        return i * TB if isinstance(i, int) and i < NS else (NS - 1) * TB

    def a_proj(i, j):
        acc = {}
        at = slot(i)

        def tile(t, k):
            r = _dot(_load(ax, k, _ds(i, TB // 2)), _load(wqkv_p, k, _ds(j * LT + t, 64)), NT)
            acc[t] = acc[t] + r if k else r
            return r

        def end(t):
            if j == 0:
                q_s[t, at:at + TB, :] = acc[t]
                return
            c = (j - 1) * LT + t
            if not isinstance(i, int):
                kv_s[c, at:at + HALO, :] = kv_s[c, at + TB:at + TB + HALO, :]
            elif i == 0:
                kv_s[c, 0:HALO, :] = jnp.broadcast_to(acc[t][0:1, :], (HALO, 128))
            kv_s[c, at + HALO:at + HALO + TB, :] = acc[t]
        return [(TB, functools.partial(tile, t, k), functools.partial(end, t) if k == LT - 1 else None)
                for t in range(LT) for k in range(LT)]

    def a_attention(i):
        state = {}

        def window(c, r0, w):
            lo = HALO + r0 - ADIL * w
            return kv_s[c, lo:lo + RC, :]

        def logits(r0, half, late):
            q = [q_s[t, r0:r0 + RC, :] for t in range(LT)]
            q[0] = late(q[0])
            for w in range(half * AW // 2, (half + 1) * AW // 2):
                a = q[0] * window(0, r0, w)
                for t in range(1, LT):
                    a = a + q[t] * window(t, r0, w)
                state.setdefault(r0, []).append(a + pltpu.roll(a, 2 * AH, 1))

        def fold(r0, half, late):
            for w in range(half * AW // 2, (half + 1) * AW // 2):
                a = state[r0][w]
                a = (a + pltpu.roll(a, AH, 1)) * (AD ** -0.5)
                if isinstance(i, int) and r0 < ADIL * w:
                    pos = lax.broadcasted_iota(jnp.int32, (RC, 128), 0) + r0
                    a = jnp.where(pos >= ADIL * w, a, MASKED)
                state[r0][w] = a

        def weights(r0, late):
            m = late(functools.reduce(jnp.maximum, state[r0]))
            state[r0] = [jnp.exp(a - m) for a in state[r0]]

        def mix(r0, tiles, late):
            e = [late(state[r0][0])] + state[r0][1:]
            if 0 in tiles:
                state[r0, "inv"] = _inverse(functools.reduce(jnp.add, e))
            for t in tiles:
                o = e[0] * window(LT + t, r0, 0)
                for w in range(1, AW):
                    o = o + e[w] * window(LT + t, r0, w)
                oa_s[t, r0:r0 + RC, :] = o * state[r0, "inv"]

        stages = ((logits, 0), (logits, 1), (fold, 0), (fold, 1), (weights,), (mix, (0, 1)), (mix, (2, 3, 4)))
        return [[functools.partial(f, r0, *args) for r0 in range(slot(i), slot(i) + TB, RC)] for f, *args in stages]

    def a_pack(i):
        def pack(k):
            ob[k, slot(i):slot(i) + TB, :] = oa_s[k, slot(i):slot(i) + TB, :].astype(BF16)
        return [functools.partial(pack, k) for k in range(LT)]

    def a_out(i):
        acc = {}

        def tile(t, k):
            r = _dot(_load(ob, k, _ds(slot(i) // TB, TB // 2)), _load(wo_p, t, _ds(k, 64)))
            acc[t] = acc[t] + r if k else r
            return r

        def end(t):
            outa[_ds(i, TB), t * 128:(t + 1) * 128] = acc[t].astype(BF16)
        return [(TB, functools.partial(tile, t, k), functools.partial(end, t) if k == LT - 1 else None)
                for t in range(LT) for k in range(LT)]

    def overlap(tiles, side=(), zero=None, lag=0):
        due = sorted((lo + (hi - lo) * n / len(tasks), m, n, task, ref)
                     for m, (lo, hi, tasks, ref) in enumerate(side) for n, task in enumerate(tasks))
        free = [0] * 4
        results = []
        for count, tile, end in tiles:
            now = min(free)
            free[free.index(now)] += count
            results.append((now, tile()))
            while due and due[0][0] + lag < min(free):
                time, _, _, task, ref = due.pop(0)
                begin, r = [x for x in results if x[0] <= time][-1]
                row = min(int(time - begin), r.shape[0] - 1) // 8 * 8
                if isinstance(ref, str):
                    task(lambda x: jnp.where(zero == 0, x, r[row:row + 8]))
                    continue
                if ref is bx:
                    ref[pl.ds(pl.multiple_of(S + 16 * zero, 16), 16), 0:128] = r[row // 16 * 16:row // 16 * 16 + 16].astype(BF16)
                elif ref is not None:
                    ref[(ref.shape[0] - 1 - zero,) + (0,) * (len(ref.shape) - 3) + (slice(0, 8),)] = (
                        pltpu.bitcast(r[row:row + 8], ref.dtype))
                task()
            if end:
                end()
        assert not due

    def w_transpose(c, n):
        size = NPL if isinstance(c, int) else CG * LT
        first = c * CG * LT
        at = [FT * j + t for j, t in TILES[n::CG * LT]]
        if isinstance(c, int):
            at = at[c]
        else:
            words = [sum(x << 8 * k for k, x in enumerate(at[m::5])) for m in range(5)]
            word = functools.reduce(lambda x, m: jnp.where(lax.rem(c, 5) == m, words[m], x), range(1, 5), words[0])
            at = lax.shift_right_logical(word, lax.div(c, 5) * 8) & 255
        wb.at[pl.ds(first, size)][n] = pltpu.bitcast(raw[_ds(at, 128), :].T, U32)

    def combine(tile, dst, r, i):
        row = col = tile(i, i)
        for k in range(LT):
            if k != i:
                a, b = tile(i, k), tile(k, i)
                row, col = row - a, col - b
                if k > i:
                    dst[LT + PAIRS.index((i, k)), 16 * r:16 * r + 16, :] = (a - b).astype(BF16)
        dst[i, 16 * r:16 * r + 16, :] = row.astype(BF16)
        dst[NZ + i, 16 * r:16 * r + 16, :] = col.astype(BF16)

    def w_combine(c, u, r, i):
        tiles = wb.at[pl.ds(c * CG * LT, CG * LT)]
        combine(lambda i, j: pltpu.bitcast(tiles[u * LT + j, pl.ds(i * 64 + 8 * r, 8), :], BF16).astype(F32),
                wz.at[pl.ds(c * CG, CG)].at[u], r, i)

    def wo_combine(g, r, i, late):
        def tile(a, b):
            x = wo_rows((g * LT + a) * 128 + 16 * r, 16, b).astype(F32)
            return jnp.concatenate([late(x[0:8]), x[8:]], axis=0)
        combine(tile, wz.at[NG + g], r, i)

    def halves(s):
        x = bx[_ds(s, SEG), :].astype(F32)
        return [[x[r:r + HALF, i * 128:(i + 1) * 128] for i in range(LT)] for r in (0, HALF)]

    def long_lhs(a, b, dst, i):
        p = [a[k] + LAM[k] * b[k] if LAM[k] else a[k] for k in range(LT)]
        dst[i] = b[i].astype(BF16)
        for k in ((i + 1) % LT, (i + 2) % LT):
            lo, hi = sorted((i, k))
            dst[LT + PAIRS.index((lo, hi))] = ((p[lo] + p[hi]) * (1.0 / (LAM[lo] - LAM[hi]))).astype(BF16)

    def short_lhs(a, b, j):
        p = [a[i] + LAM[j] * b[i] if LAM[j] else a[i] for i in range(LT)]
        return [p[j] if i == j else (p[i] + p[j]) * (1.0 / (LAM[j] - LAM[i])) for i in range(LT)]

    def z_lhs(s, i):
        long_lhs(*halves(s), lz.at[:, _ds(s, HALF), :], i)

    def z_batch(t):
        return [functools.partial(z_lhs, t * ZB + u, i) for u in range(ZB) for i in range(LT)]

    def z_product(g, n, batch):
        return _dot(_load(lz, n, _ds(batch, ZB * HALF // 2)), _load(wz, g, n))

    def z_group(g, batch):
        dst = z.at[z_index(g, batch)]

        sums, stored = {}, set()

        def tile(n):
            r = z_product(g, n, batch)
            for i in (n,) if n < LT else PAIRS[n - LT]:
                sums[i] = sums[i] + r if i in sums else r
            return r

        def end():
            for i in sums:
                z_add(dst, i, sums[i], i not in stored)
                stored.add(i)
            sums.clear()
        sets = (((0, 1), (0, 2), (1, 2), 0, 1), ((0, 3), (0, 4), (3, 4), 3, 4), ((1, 3), (1, 4), (2, 3), (2, 4), 2))
        return [(ZB * HALF, functools.partial(tile, LT + PAIRS.index(n) if n in PAIRS else n), end if n == some[-1] else None)
                for some in sets for n in some]

    def z_add(dst, n, r, first=True):
        for i in (n,) if n < LT else PAIRS[n - LT]:
            for u in range(ZB):
                x = r[u * HALF:(u + 1) * HALF]
                dst[u, i * HALF:(i + 1) * HALF, :] = x if n < LT and first else x + dst[u, i * HALF:(i + 1) * HALF, :]

    def z_index(g, batch):
        if isinstance(batch, int) and batch == 0:
            return g
        if isinstance(g, int) and g >= G0:
            return g + (batch % 2) * (NG - G0)
        return jnp.where(batch == 0, g, 2 * (NG - G0) + batch * G0 + g)

    if not CFG.get('onlyB'):
        flag[0] = 0
        c_second = [c_wqkv[1]] + c_ax(0, NS * TB, sem_a.at[1])
        start([c_wqkv[0]] + c_second)
        c_wqkv[0].wait()
        zero = flag[0]
        _mark('w0')
        _run(sum(prep_wqkv(0), []))
        start([c_wqkv[2], c_bx0])
        wait(c_second)
        _mark('w1')
        first, second = prep_wqkv(1)
        overlap(a_proj(0, 0) + a_proj(1, 0), [(0, 0, first, None), (700, 1500, second, tmp)], zero)
        start([c_awo] + c_first[:CFG["n1"]])
        wait([c_wqkv[2], c_bx0])
        _mark('w2')
        first, second = prep_wqkv(2)
        overlap(a_proj(0, 1) + a_proj(1, 1),
                [(0, 0, first, None), (700, 1500, second, tmp), (0, 1500, z_batch(0) + z_batch(1), bx)], zero)
        start(c_first[CFG["n1"]:])
        c_awo.wait()
        _mark('w3')
        e = CFG["e"]
        overlap(a_proj(0, 2) + a_proj(1, 2) + a_out(0),
                [(0, 800, prep_wo(), tmp), (1500, 1500, a_pack(0), None)]
                + [(e[i] + d, e[i + 1] + d, tasks, "value")
                   for i in range(NS) for d, tasks in zip(CFG["lags%d" % i], a_attention(i))], zero)
        start(c_step(1) + c_step(2))
        _mark('pre_first')
        wait(c_first)

        def a_step(c, carry):
            _mark('a_top')
            whole = raw.at[pl.ds(0, sum(STEP) + 2 * TB), :]
            pl.when((c > 0) & (c < NST))(cp(whole, whole, sem_w.at[c]).wait)

            for copy in c_last:
                pl.when(c == NST)(copy.wait)

            _mark('a_go')
            f = CFG["f"]
            zero = lax.shift_right_logical(c, 16)
            flag[zero] = 0
            if G0 == 2:
                early = z_group(0, c + 1) + z_group(1, c + 1)
            else:
                early = [x for u in range(2) for t in range(2) for x in z_group((c & 1) * 2 + u, (c | 1) + t)]
            overlap(a_proj(c + NS, 0) + a_proj(c + NS, 1) + a_proj(c + NS, 2) + a_out(c + NS - 1)
                    + z_group(c * CG, 0) + early + z_group(c * CG + 1, 0), [
                (0, f[0], [functools.partial(w_transpose, c, n) for n in range(CG * LT)], None),
                (0, f[1], z_batch(c + G0 // 2), bx),
                (0, f[1], a_pack(c + NS - 1), oa_s),
                (f[1], f[2], [functools.partial(w_combine, c, u, r, i)
                              for u in range(CG) for r in range(8) for i in range(LT)], wb),
            ] + [(f[3] + d, f[4] + d, tasks, "value") for d, tasks in zip(CFG["lags"], a_attention(c + NS))], zero)
            for copy in c_step(jnp.minimum(c + 3, NST - 1)) + c_wo(0, c, WO_STEP, sem_a.at[5]):
                pl.when(c < NST - 3)(copy.start)
            for copy in c_last:
                pl.when(c == NST - 3)(copy.start)
            for copy in c_wo(WO_FIRST, jnp.clip(c - (NST - 2), 0, 1), (H * DH - WO_FIRST) // 2, sem_a.at[7]):
                pl.when((c > NST - 3) & (c < NST))(copy.start)
            return carry

        lax.fori_loop(0, NCH, a_step, 0)
        _mark('epi')
        part = wo.at[:, pl.ds(0, WO_FIRST), :]
        cp(part, part, sem_a.at[5]).wait()
        h = CFG['h']
        overlap([x for g in range(G0) for x in z_group(g, NSEG // ZB - 1)] + a_out(NB - 1),
                [(0, 0, [functools.partial(w_transpose, NCH, n) for n in range(NPL)], None),
                 (0, h[0], a_pack(NB - 1), oa_s),
                 (h[1], h[2], [functools.partial(wo_combine, g, r, i)
                               for g in range(WG) for r in range(8) for i in range(LT)], "value")], zero)
        _mark('pre_wo')
        part = wo.at[:, pl.ds(WO_FIRST, H * DH - WO_FIRST), :]
        cp(part, part, sem_a.at[7]).wait()

    def rows(r0, n):
        return slice(r0, r0 + n)

    def r_lhs(hb, i, j):
        return R_LHS + ((hb * LT + i) * LT + j) * (M + HALF)

    def r_qkv(j, t):
        return rows(R_QKV + (j * FT + t) * L, L)

    def token_lhs(s, hb):
        a, b = halves(s)
        for j in range(LT):
            buf[rows(R_H + (hb * LT + j) * L + M, SEG)] = jnp.concatenate([a[j], b[j]], axis=0)
            for i, x in enumerate(short_lhs(a, b, j)):
                buf[rows(r_lhs(hb, i, j) + M, HALF)] = x

    def memory_lhs(m, n, hb):
        buf[rows(R_H + (hb * LT + n) * L, M)] = m[n]
        buf[rows(r_lhs(hb, n, n), M)] = m[n]
        for k in range(n):
            buf[rows(r_lhs(hb, n, k), M)] = buf[rows(r_lhs(hb, k, n), M)] = m[n] + m[k]

    def out_product(g, n):
        return _dot(_load(lo, g - NG, n), _load(wz, g, n))

    def out_finish(g, n, r, batch):
        z_add(zo, n, r, g == NG)
        for i in range(LT):
            if g == NG + WG - 1 and n == LT + max(k for k, pair in enumerate(PAIRS) if i in pair):
                for u in range(ZB):
                    y = zo[u, rows(i * HALF, HALF), :]
                    y = jnp.concatenate([-LAM[i] * y, y], axis=0)
                    outb[_ds(batch * ZB + u, SEG), rows(i * 128, 128)] = (op[u, i] + y).astype(BF16)

    lo_next, op_next = lo, op

    def segment(plan, batch, part, hb, nh, before=()):
        s = batch * ZB + part
        key = lax.broadcasted_iota(jnp.int32, (L, 128), 0)
        col = lax.broadcasted_iota(jnp.int32, (L, 128), 1)
        head0 = col < L
        query = jnp.where(head0, col, col - L)
        visible = (query < M) | (query >= key)
        low = lax.broadcasted_iota(jnp.int32, (L, 128), 1) < 64
        val = {}
        fenced = buf.at[pl.ds(pl.multiple_of(lax.shift_right_logical(batch, 16) * 32, 32), R_END)]
        z_next = z.at[pl.ds(z_index(G0, batch + 1), NG - G0)]
        new_mem = []

        def add(name, x):
            val[name] = val[name] + x if name in val else x

        def product(*args):
            r = _dot(*args)
            val["latest"] = r[-8:]
            return r

        def short(g, i, j):
            if i == j:
                w = _load(wz, g, NZ + i)
            elif g < NG:
                w = pltpu.bitcast(wb[g * LT + j, rows(i * 64, 64), :], BF16)
            else:
                w = wo_rows(((g - NG) * LT + i) * 128, 128, j)
            at = r_lhs(hb, i, j) if g < NG else R_OL + r_lhs(g - NG, i, j)
            if CFG["fence"] and g > 0 and i == j and i in CFG["fence"]:
                x = jnp.concatenate([buf[rows(at, 16)], fenced[rows(at + 16, 8)]], axis=0)
            else:
                x = buf[rows(at, M + HALF)]
            add((min(g, NG), i, j), product(x, w))

        def take(g, i, j):
            if NG <= g < NG + WG - 1:
                return
            g = min(g, NG)
            r = val.pop((g, i, j))
            add(("m", g, j), r[0:M])
            if i != j:
                add(("y", g, i), r[M:])
                add(("d", g, j), r[M:])
                if LAM[i]:
                    add(("c", g, j), r[M:] * -LAM[i])
                return
            y = val.pop(("y", g, j))
            if g < NG:
                y = y + z[z_index(g, batch), part, rows(j * HALF, HALF), :]
            c = val.pop(("c", g, j)) + r[M:]
            if LAM[j]:
                c = c - LAM[j] * y
            r = jnp.concatenate([val.pop(("m", g, j)), c, val.pop(("d", g, j)) + y], axis=0)
            if g < NG:
                buf[r_qkv(*TILES[g * LT + j])] = r
            else:
                buf[rows(R_ACC + j * L, L)] = out_sum(j, r)

        def out_sum(n, r):
            if ("acc", n) in val:
                r = r + buf[rows(R_ACC + n * L, L)]
            val["acc", n] = True
            return r

        def out_lhs(g, j):
            o = [buf[rows(R_O + (g * LT + i) * L, L)] for i in range(LT)]
            a, b = [x[M:M + HALF] for x in o], [x[M + HALF:] for x in o]
            a[j] = jnp.concatenate([jnp.where(batch >= 0, x, val["latest"]) for x in (a[j][0:8], a[j][8:])], axis=0)
            for i, x in enumerate(short_lhs(a, b, j)):
                m = o[j][0:M] if i == j else o[i][0:M] + o[j][0:M]
                val["lhs", g, j, i] = jnp.concatenate([m, x], axis=0)
            long_lhs(a, b, lo_next.at[g, :, rows(part * HALF, HALF), :], j)

        def out_lhs_end(g, j):
            for i in range(LT):
                buf[rows(R_OL + r_lhs(g, i, j), M + HALF)] = val.pop(("lhs", g, j, i))

        def plain(n, k):
            w = pltpu.bitcast(wb[NG * LT + n, rows(k * 64, 64), :], BF16)
            val["plain", n, k] = product(buf[rows(R_H + (hb * LT + k) * L, L)], w)

        def plain_end(n, k):
            dst = r_qkv(*TILES[NG * LT + n])
            r = val.pop(("plain", n, k))
            buf[dst] = r + buf[dst] if k else r

        def long(g, n):
            val["long", g, n] = z_product(g, n, batch + 1) if g < NG else out_product(g, n)
            val["latest"] = val["long", g, n][24:32]

        def long_end(g, n):
            if g < NG:
                z_add(z_next.at[g - G0], n, val.pop(("long", g, n)))
            else:
                out_finish(g, n, val.pop(("long", g, n)), jnp.maximum(batch - 1, 0))

        def score(t):
            q = buf[r_qkv(0, t)]
            none = jnp.zeros((L, 128), F32)
            q = ((q, none), (jnp.where(low, q, 0.0), jnp.where(low, 0.0, q)), (q, none) if CFG["trim"] else (none, q))[t % 3]
            q = jnp.concatenate(q + (jnp.zeros((128 - 2 * L, 128), F32),), axis=0)
            r = product(buf[r_qkv(1, t)], q.astype(BF16), NT)
            add(("s", t // 3), pltpu.roll(r, L, 1) if t % 3 == 2 and CFG["trim"] else r)

        def softmax(p, step):
            def late(x):
                return jnp.where(col[0:8] < 2 * L, x, val["latest"]) if step in CFG["ties"] else x

            def groups(x):
                return [x[r:r + 8] for r in range(0, L, 8)]

            def spread(x):
                return jnp.concatenate([x] * (L // 8), axis=0)
            x, y = val["s", p], val.get(("t", p))
            if step == 0:
                x = jnp.where(visible, x * (DH ** -0.5), MASKED)
                y = functools.reduce(jnp.maximum, groups(x))
            elif step == 1:
                y = jnp.broadcast_to(jnp.max(late(y), axis=0, keepdims=True), (8, 128))
            elif step == 2:
                x = jnp.exp(x - spread(late(y)))
                y = functools.reduce(jnp.add, groups(x))
            elif step == 3:
                y = jnp.broadcast_to(jnp.sum(late(y), axis=0, keepdims=True), (8, 128))
            elif step == 4:
                y = _inverse(late(y))
            elif step == 6:
                buf[rows(R_P + p * 2 * L, 2 * L), 0:2 * L] = x
            else:
                x = x * spread(late(y))
                x = jnp.concatenate([x, x], axis=0)[:, 0:2 * L]
                x = x.astype(BF16).T.astype(F32)
            val["s", p], val["t", p] = x, y

        def pv(t):
            pa, pb = [buf[rows(R_P + (2 * (t // 3) + u) * L, L), 0:2 * L] for u in range(2)]
            v = buf[r_qkv(2, t)]
            if t % 3 == 1:
                v = jnp.concatenate([jnp.where(low, v, 0.0), jnp.where(low, 0.0, v)], axis=0)
            pr = (pa[:, 0:L], jnp.where(head0[:, 0:2 * L], pa, pb), pb[:, 0:L])[t % 3]
            val["o", t] = product(pr, v.astype(BF16))

        def pv_end(t):
            buf[rows(R_O + t * L, L)] = val.pop(("o", t))

        def out(t, n):
            add(("out", t // KC, n), product(buf[rows(R_O + t * L, L)], wo_rows(t * 128, 128, n)))

        def out_end(t, n):
            r = out_sum(n, val.pop(("out", t // KC, n)))
            if t < FT - 1:
                buf[rows(R_ACC + n * L, L)] = r
                return
            new_mem.append(r[0:M])
            memory_lhs(new_mem, n, nh)
            if isinstance(part, int) and WG:
                op_next[part, n] = r[M:L]
            else:
                outb[_ds(s, SEG), rows(n * 128, 128)] = r[M:L].astype(BF16)

        tasks = dict(short=short, take=take, plain=plain, plain_end=plain_end, long=long, long_end=long_end,
                     score=score, softmax=softmax, pv=pv, pv_end=pv_end,
                     out=out, out_end=out_end, out_lhs=out_lhs, out_lhs_end=out_lhs_end,
                     token_lhs=lambda: token_lhs(jnp.minimum(s + 1, NSEG - 1), nh))
        before = list(before)
        for name, *args in plan[0]:
            need = max(args[1:]) if name in ("short", "plain") else LT - 1 if name == "pv" else -1
            while len(before) > LT - 1 - need:
                before.pop(0)()
            tasks[name](*args)
        return [functools.partial(tasks[name], *args) for name, *args in plan[1]]

    if CFG.get('onlyB'):
        start(c_first + [cp(wo_hbm.at[:, pl.ds(0, 128)], wo.at[0], sem_a.at[5]), c_mem])
        w_transpose(0, 0)
        w_combine(0, 0, 0, 0)
        z_lhs(0, 0)
        overlap(z_group(0, 0))
    token_lhs(0, 0)
    mem0 = mem[0:M, :].astype(F32)
    for n in range(LT):
        memory_lhs([mem0[:, k * 128:(k + 1) * 128] for k in range(LT)], n, 0)

    longs = ([("long", NG + g, n) for n in range(NZ) for g in range(WG)]
             + [("long", g, n) for g in range(G0, NG) for n in range(NZ)])
    main_plans = [_make_plan(CFG["r%d" % u] if "r%d" % u in CFG else CFG["rounds"], longs) for u in range(UN)]
    if WG:
        order = main_plans[0][0]
        assert order.index(("long", NG + WG - 1, NZ - 1)) < order.index(("out_lhs", 0, 0))
    assert not longs or UN < ZB
    last_plan = _make_plan(CFG["last_rounds"], None)
    n_main = NSEG // ZB - 1

    def b_step(it, carry):
        _mark('b')
        rest = ()
        for u in range(UN):
            rest = segment(main_plans[u], it, u, u, (u + 1) % UN, rest)
        _run(rest)
        if WG:
            pl.when(it > 0)(lambda: c_outb(pl.multiple_of((it - 1) * ZB * SEG, SEG), ZB * SEG).start())
        else:
            c_outb(pl.multiple_of(it * ZB * SEG, SEG), ZB * SEG).start()
        return carry

    def last_step(s, carry):
        _mark('last')
        _run(segment(last_plan, s // ZB, s % ZB, 0, 0))
        c_outb(pl.multiple_of(s * SEG, SEG), SEG).start()
        return carry

    c_outa.start()
    if CFG.get('onlyB') != 2 and not CFG.get('onlyA'):
        lax.fori_loop(0, n_main, b_step, 0)
        if WG:
            for n in range(NZ):
                for g in range(NG, NG + WG):
                    out_finish(g, n, out_product(g, n), n_main - 1)
            c_outb((n_main - 1) * ZB * SEG, ZB * SEG).start()
    if CFG.get('onlyB') != 1 and not CFG.get('onlyA'):
        lax.fori_loop(n_main * ZB, NSEG, last_step, 0)
    if CFG.get('onlyA'):
        outb[0:16, 0:128] = (z[0, 0, 0:16] + pltpu.bitcast(wb[0, 0:16], F32) + buf[0:16] + lz[0, 32:48].astype(F32)).astype(BF16)
        start([c_outb(0, S)])
    _mark('end')
    c_outa.wait()
    c_outb(0, S).wait()


def pallas_concat_heads__sliding_local_dilated__memory_aug_recurrent_mem_tr__prompt_kernel(
    A_x, A_wqkv, A_wo, B_x, B_mem0, B_Wq, B_Wk, B_Wv, B_Wo, B_seg_len,
):
    assert B_seg_len == SEG
    assert A_x.shape == B_x.shape == (1, S, D) and B_mem0.shape == (1, M, D)
    assert B_Wq.shape == B_Wk.shape == B_Wv.shape == (D, H, DH) and B_Wo.shape == (H, DH, D)
    vmem, dma = pltpu.VMEM, pltpu.SemaphoreType.DMA
    call = pl.pallas_call(
        _kernel,
        out_shape=jax.ShapeDtypeStruct((S, 2 * D), BF16),
        in_specs=[pl.BlockSpec(memory_space=pl.ANY)] * 9,
        out_specs=pl.BlockSpec(memory_space=pl.ANY),
        scratch_shapes=[
            vmem((LT, S, 128), BF16),
            vmem((3, D, D), BF16),
            vmem((D, D), BF16),
            vmem((LT + 1, D, 128), F32),
            vmem((LT, 3 * D, 128), BF16),
            vmem((LT, D, 128), BF16),
            vmem((LT, NS * TB, 128), F32),
            vmem((2 * LT, HALO + NS * TB, 128), F32),
            vmem((LT + 1, NS * TB, 128), F32),
            vmem((LT, NS * TB, 128), BF16),
            vmem((S, D), BF16),
            vmem((S + 64, D), BF16),
            vmem((64, D), BF16),
            vmem((3 * H * DH, D), BF16),
            vmem((len(TILES) + 1, D // 2, 128), U32),
            vmem((NG + WG, NZ + LT, 128, 128), BF16),
            vmem((LT, H * DH, 128), BF16),
            vmem((NZ, S // 2, 128), BF16),
            vmem((2 * (NG - G0) + NSEG // ZB * G0, ZB, LT * HALF, 128), F32),
            vmem((max(WG, 1), NZ, ZB * HALF, 128), BF16),
            vmem((ZB, LT * HALF, 128), F32),
            vmem((ZB, LT, SEG, 128), F32),
            vmem((R_END, 128), F32),
            pltpu.SMEM((2,), jnp.int32), dma((8,)), dma((NCH,)), dma((2,)),
        ],
        compiler_params=pltpu.CompilerParams(vmem_limit_bytes=126 * 1024 * 1024,
                                             internal_scratch_in_bytes=48 * 1024, disable_bounds_checks=True, disable_semaphore_checks=bool(CFG.get('nosem')), flags=CFG.get("flags")),
        name="sliding_and_memory_attention",
    )

    def by_feature(w):
        return w.transpose(1, 2, 0).reshape(H * DH, D)

    out = call(A_x.reshape(S, D), A_wqkv, A_wo, B_x.reshape(S, D), B_mem0.reshape(M, D),
               by_feature(B_Wq), by_feature(B_Wk), by_feature(B_Wv), B_Wo.reshape(H * DH, D))
    return out.reshape(1, S, 2 * D)
```

```python
import functools

import jax
import jax.numpy as jnp
from jax import lax
from jax.experimental import pallas as pl
from jax.experimental.pallas import tpu as pltpu

F32, BF16, U32 = jnp.float32, jnp.bfloat16, jnp.uint32
NN = (((1,), (0,)), ((), ()))
NT = (((1,), (1,)), ((), ()))
MASKED = -1000000000.0
CFG = dict(UN=4, UT=1, G0=4, zsum=1, qv16=0, W0=0, TL=32, lags0=[0, 22, 120, 142, 330, 500, 510], lags1=[0, 22, 120, 142, 330, 650, 655], h=[500, 0, 1530], n1=7, e=[300, 950, 1550], WG=2, skew=1, d_lhs=48, fence=[], d_p=0, lag="2222222233334444", pl=[11, 23, 35, 42], f=[1240, 600, 2600, 2391, 4010], lags=[2, 50, 174, 227, 346, 364, 416], cuts=[2, 3, 4, 6, 7, 8, 10, 11, 12, 14, 15, 16, 17, 18, 19], vlag=2, kc=3, lat=120, ties=[1, 2, 3, 4, 5], d_step=24, d_norm=280,
           r0="PsLssssLssssLssssLssssLssssLssssLssssLsQssssLssssLssssLssssLssQsssVssssLssssLssssLssssLsssVssssLssQsssVssssLssssLssssLssssLssQsssVsWssssLssssLssWWssssLsssVsWssWssVssWsssQsWsWsWsssQsWssWsWWssWsWssVssWsWWsssVsWsWsWssWssWWWsssVssQsWsWsWsQsssWWWsssVswWsWwWssVwWwWwwwVwWwWwWwwWWWwWWWWW",
r1="LPssssLssssLssssLssssLssssLssssLssssLssssLssssLssssLssssLsssQsQssssLssssLssssLssssVssVssQsssVsssLsWssWsssLssQsssVssssLssssLssssLssssLssssLssssLssssLssssVsWsWsWssVssWsWWssWssQsWsWsWsQssWWssWsssVsWsWsWsWsWsWssVssssLsWsssWWsWssVssQsWsWsWsQsssWWsWswVswWsWWswwVwsWsWWwWwwwVwWWwWwwWWWWWW",
r2="LPssssLssssLssssLssssLssssLsQssssLssssLssssLssssLssssLssssVsQssssLssssLssssLsssVssQsssVssssLssssLssssLssWWssQsssVssssLsssssLssssLssssLssssLssWsssVsWsWsWssVssssQsWsWsWssQssWsssLsWsWssssLsWsWsWssssVsWsWsWsssVsWsWsWsWsssWWWsssVssQsWsWsWsQsssWWsWssVsWwwWWwwsVssWWwWwwwVwWWwWwWWwwWWWWW",
r3="LPssssLssssLssssLssssLssssLssssLssssLssssLssssLssssLssssLsssQsQssssLssssLssssLssssVssVssQsssVsssLsWssWsssLssQsssVssssLssssLssssLssssLssssLssssLssssLssssVsWsWsWssVssWsWWssWssQsWsWsWsQssWWssWsssVsWsWsWsWsWsWssVssssLsWsssWWsWssVssQsWsWsWsQsssWWsWswVswWsWWswwVwsWsWWwWwwwVwWWwWwwWWWWWW",
           last_rounds="PsssLssssLssssssLssssLssssQssLssssLssssLssssLssssssQssVssssWssssLssssLssssVsWsWsWsssVsWsWssssLsWssWssWssQsssssssQsssWWsssssLssssVssWWsssVsWsWsWsWsssVsWsWssssssLssWsWsssQsWsWsWsssQsssWssssVssWWsWssWWssWWssWsWssVssssWsWsssWQsssVsWsssWWsQsWsssWWsWssVsWsssWWVWWVWWWWWWWWWWW")

S, D = 2048, 640
LT = D // 128

AH, AD, AW, ADIL = 32, 20, 8, 2
HALO = 16
TB = 128
NB = S // TB
NS = 2
TL = CFG['TL']
TE = TB - TL
RC = 8

H, DH, M, SEG = 32, 192, 8, 32
L = M + SEG
HALF = SEG // 2
NP = H // 2
FT = 3 * NP
NSEG = S // SEG
LAM = (0.0, 0.625, -0.625, 1.875, -1.875)
PAIRS = [(i, j) for i in range(LT) for j in range(i + 1, LT)]
NZ = LT + len(PAIRS)
Z_ORDER = [LT + PAIRS.index(n) if n in PAIRS else n
           for n in ((0, 1), (0, 2), (1, 2), 0, (0, 3), (0, 4), (3, 4), 3, 4, (1, 4), 1, (1, 3), (2, 3), (2, 4), 2)]
NG = 28
ZB = 4
GS = NG // ZB
ZS = (GS * LT + 1) * HALF
G0 = CFG["G0"]
UN, UT = CFG["UN"], CFG["UT"]
NBUF = max(UN, UT)
CG = 2
NCH = NG // CG
FIRST, STEP = (864, 688, 0), (480, 496, 432)
NST = NCH - 2
WO_STEP = 256
WO_FIRST = (NST - 3) * WO_STEP
assert CFG['W0'] % CFG['kc'] == 0
KC = CFG["kc"]
VLAG = 2
W0 = CFG["W0"]
WG = CFG["WG"]


def _tile_order():
    lag = [int(x) for x in str(CFG["lag"])]
    order = []
    for p in range(NP + max(lag)):
        if p < NP:
            order += [(j, 3 * p + t) for j in (0, 1) for t in range(3)]
        order += [(2, 3 * x + t) for x in range(NP) if x + lag[x] == p for t in range(3)]
    plain = [(2, t) for t in CFG["pl"]]
    order = [x for x in order if x not in plain] + plain
    return order


TILES = _tile_order()
assert CFG.get('onlyB') or all((t + 1) * 128 <= FIRST[j] + n // (CG * LT) * STEP[j] for n, (j, t) in enumerate(TILES[:NST * CG * LT]))
NPL = len(TILES) - NG * LT

R_LHS = 0
R_H = R_LHS + NBUF * LT * LT * (M + HALF)
R_QKV = R_H + NBUF * LT * L
R_O = R_QKV + 3 * FT * L
R_P = R_O + FT * L
R_ACC = R_P + NP * 2 * L
R_OL = R_ACC + LT * L
R_END = (R_OL + WG * LT * LT * (M + HALF) + 31) // 32 * 32


def _make_plan(rounds, longs, fast):
    shell = []
    for k in range(LT):
        for n in range(k + 1, LT):
            shell += [(k, n), (n, k)]
        shell += [(k, k)]
    todo = dict(
        L=longs,
        s=[("short", g, i, j) for g in range(NG) for (i, j) in shell],
        w=[("short", NG + g, i, j) for (i, j) in shell for g in range(fast)],
        W=[("out", t, n) for k in range(0, FT, KC) for n in range(LT) for t in range(k, k + KC)
           if not W0 <= t < W0 + fast * LT],
        P=[("plain", n, 0) for n in range(NPL)] + [("plain", n, k) for n in range(NPL) for k in range(1, LT)],
        Q=[("score", p + u, both) for p in range(0, NP, 2) for both in (p // 2 % 2, 1 - p // 2 % 2) for u in range(2)],
        V=[("pv", t) for t in range(FT)])
    plan, timed, now = [], [], 0

    def later(time, *task):
        timed.append((time, task))
        timed.sort(key=lambda x: x[0])

    def flush(time):
        timed.sort(key=lambda x: x[0])
        while timed and timed[0][0] <= time:
            plan.append(timed.pop(0)[1])

    def needs(task):
        if task[0] == "out":
            return [("pv_end", task[1])]
        if task[0] == "short" and task[1] >= NG:
            return [("out_lhs_end", task[1] - NG, task[3])]
        if task[0] not in ("score", "pv"):
            return []
        need = [("softmax", task[1] // 3, 6)] if task[0] == "pv" else []
        for tile in [(2, task[1])] if task[0] == "pv" else [(j, 3 * task[1] + t) for j in (0, 1) for t in range(3)]:
            n = TILES.index(tile)
            need.append(("take", n // LT, n % LT, n % LT) if n < NG * LT else ("plain_end", n - NG * LT, LT - 1))
        return need

    for n, kind in enumerate(rounds):
        four = todo[kind][:4]
        del todo[kind][:4]
        if kind == "Q":
            four += [todo["P"].pop(0), todo["P"].pop(0)]
        while kind == "w" and len(four) < 4:
            four.append(todo["W"].pop(0))
        need = [x for task in four for x in needs(task)]
        for need_time, needed in [x for x in timed if x[1] in need]:
            key = needed[:2] if needed[0] == "softmax" else needed[:1]
            timed[:] = [(min(time, now) if task[:len(key)] == key and time <= need_time else time, task)
                        for time, task in timed]
        flush(now)
        assert all(x in plan for x in need)
        plan += four
        now += dict(s=M + HALF, w=M + HALF, L=ZB * HALF, Q=2 * L).get(kind, L)
        end = now + CFG["lat"]
        for name, *args in four:
            if name == "short":
                later(end, "take", *args)
            elif name == "out" and args[0] % KC == KC - 1:
                later(end, "out_end", *args)
            elif name in ("plain", "long", "pv"):
                later(end, name + "_end", *args)
                if name == "pv" and W0 <= args[0] < W0 + fast * LT and (args[0] - W0) % LT == LT - 1:
                    for j in range(LT):
                        later(end + CFG["d_lhs"] * j, "out_lhs", (args[0] - W0) // LT, j)
                        later(end + CFG["d_lhs"] * j + CFG["lat"], "out_lhs_end", (args[0] - W0) // LT, j)
            elif name == "score" and args[1]:
                for step in range(6):
                    later(now + CFG["d_step"] * (step + CFG["skew"] * (args[0] % 2)), "softmax", args[0], step)
                later(now + CFG["d_step"] * 6 + 10000, "softmax", args[0], 6)
        if kind == "L":
            later(end, "long_store")
        if kind not in rounds[n + 1:] and kind == "s":
            plan.append(("token_lhs",))
    assert not any(todo[kind] for kind in "swWPQV")
    return plan, [task for _, task in sorted(timed, key=lambda x: x[0])]


def _ds(i, n):
    return pl.ds(i * n if isinstance(i, int) else pl.multiple_of(i * n, n), n)


def _dot(a, b, dims=NN):
    r = lax.dot_general(a, b, dims, preferred_element_type=F32)
    return jnp.concatenate([r[0:8], r[8:]], axis=0)


def _share(tasks, k, n):
    return tasks[k * len(tasks) // n:(k + 1) * len(tasks) // n]


def _mark(name):
    if CFG.get("trace"):
        with jax.named_scope(name):
            pl.delay(1)


def _run(tasks):
    for task in tasks:
        task()


def _inverse(x):
    r = pltpu.reciprocal(x, approx=True)
    return r + r * (1.0 - x * r)


def _load(ref, *index):
    return pltpu.bitcast(ref.bitcast(U32)[index], BF16)


def _kernel(ax_hbm, awqkv_hbm, awo_hbm, bx_hbm, mem_hbm, wq_hbm, wk_hbm, wv_hbm, wo_hbm,
            out_hbm,
            ax, awo, tmp, wqkv_p, wo_p, q_s, kv_s, oa_s, ob, ol, outa, outl,
            bx, mem, raw, wb, wz, wo, lz, z, lo, zo, op, qv, buf,
            flag, sem_a, sem_w, sem_o):
    cp = pltpu.make_async_copy
    outb = raw.at[pl.ds(0, S), :]

    def rows_copy(src, dst, r0, r1, sem):
        return cp(src.at[pl.ds(r0, r1 - r0), :], dst.at[pl.ds(r0, r1 - r0), :], sem)

    c_wqkv = [cp(awqkv_hbm.at[:, pl.ds(j * D, D)], raw.at[pl.ds(3 * (H * DH - D) + j * D, D), :], sem_a.at[j]) for j in range(3)]
    c_awo = cp(awo_hbm, awo, sem_a.at[3])
    c_mem = cp(mem_hbm, mem.at[pl.ds(0, M), :], sem_a.at[4])
    c_outa = cp(outa, out_hbm.at[:, pl.ds(0, TE), pl.ds(0, D)], sem_o.at[0])

    def c_rows(src, dst, first, i, n, sem):
        at = pl.ds(first + i * n if isinstance(i, int) else pl.multiple_of(first + i * n, 16), n)
        return cp(src.at[at, :], dst.at[at, :], sem)

    def c_wo(first, i, n, sem):
        at = pl.ds(pl.multiple_of(first + i * n, 16), n)
        return [cp(wo_hbm.at[at, pl.ds(t * 128, 128)], wo.at[t, at, :], sem) for t in range(LT)]

    def wo_rows(r0, n, t):
        return _load(wo, t, slice(r0 // 2, (r0 + n) // 2))

    def c_ax(i, n, sem):
        return [cp(ax_hbm.at[_ds(i, n), pl.ds(t * 128, 128)], ax.at[t, _ds(i, n), :], sem) for t in range(LT)]

    def c_x(c, sem):
        return c_ax(c + NS, TB, sem) + [c_rows(bx_hbm, bx, 0, c + 2, TB, sem)]

    def c_w(j, first, i, n, c):
        return c_rows((wq_hbm, wk_hbm, wv_hbm)[j], raw.at[pl.ds(j * H * DH, H * DH), :], first, i, n, sem_w.at[c])

    def c_step(c):
        return c_x(c, sem_w.at[c]) + [c_w(j, FIRST[j], c - 1, STEP[j], c) for j in range(3)]

    c_first = c_x(0, sem_w.at[0]) + [c_w(j, 0, 0, FIRST[j], 0) for j in range(2)]
    c_last = c_x(NST, sem_w.at[NST]) + c_x(NST + 1, sem_w.at[NST]) + [
        c_mem, c_w(2, (NST - 1) * STEP[2], 0, H * DH - (NST - 1) * STEP[2], NST)]
    c_bx0 = c_rows(bx_hbm, bx, 0, 0, 2 * TB, sem_a.at[2])

    def c_outb(r0, n):
        at = r0 % TB if isinstance(r0, int) else pl.multiple_of(lax.rem(r0, TB), n)
        return cp(outb.at[pl.ds(r0, n), :], out_hbm.at[r0 // TB, pl.ds(at, n), pl.ds(D, D)], sem_o.at[1])

    def c_late(u):
        at = pl.ds(u * (NB // ZB), NB // ZB)
        return cp(outl.at[at], out_hbm.at[at, pl.ds(TE, TL), pl.ds(0, D)], sem_o.at[2])

    def start(copies):
        for c in copies:
            c.start()

    def wait(copies):
        for c in copies:
            c.wait()

    def permute_rows(dst, base):
        def move(t, d0):
            for d in range(d0, d0 + AD // 4):
                dst[t, pl.ds(base + d * AH, AH), :] = tmp[t, pl.ds(d, AH, stride=AD), :].astype(BF16)
        return [functools.partial(move, t, d0) for t in range(LT) for d0 in range(0, AD, AD // 4)]

    def prep_wqkv(j):
        def transpose(t):
            tmp[t] = raw[pl.ds(3 * (H * DH - D) + j * D + t * 128, 128), :].astype(F32).T
        return [functools.partial(transpose, t) for t in range(LT)], permute_rows(wqkv_p, j * D)

    def prep_wo():
        def widen(t, r):
            tmp[t, r:r + D // 4, :] = awo[r:r + D // 4, t * 128:(t + 1) * 128].astype(F32)
        moves = permute_rows(wo_p, 0)
        return [task for t in range(LT)
                for task in [functools.partial(widen, t, r) for r in range(0, D, D // 4)] + moves[4 * t:4 * t + 4]]

    def slot(i):
        return i * TB if isinstance(i, int) and i < NS else (NS - 1) * TB

    def a_proj(i, j):
        acc = {}
        at = slot(i)

        def tile(t, k):
            r = _dot(_load(ax, k, _ds(i, TB // 2)), _load(wqkv_p, k, _ds(j * LT + t, 64)), NT)
            acc[t] = acc[t] + r if k else r
            return r

        def end(t):
            if j == 0:
                q_s[t, at:at + TB, :] = acc[t]
                return
            c = (j - 1) * LT + t
            if not isinstance(i, int):
                kv_s[c, at:at + HALO, :] = kv_s[c, at + TB:at + TB + HALO, :]
            elif i == 0:
                kv_s[c, 0:HALO, :] = jnp.broadcast_to(acc[t][0:1, :], (HALO, 128))
            kv_s[c, at + HALO:at + HALO + TB, :] = acc[t]
        return [(TB, functools.partial(tile, t, k), functools.partial(end, t) if k == LT - 1 else None)
                for t in range(LT) for k in range(LT)]

    def a_attention(i):
        state = {}

        def window(c, r0, w):
            lo = HALO + r0 - ADIL * w
            return kv_s[c, lo:lo + RC, :]

        def logits(r0, half, late):
            q = [q_s[t, r0:r0 + RC, :] for t in range(LT)]
            q[0] = late(q[0])
            for w in range(half * AW // 2, (half + 1) * AW // 2):
                a = q[0] * window(0, r0, w)
                for t in range(1, LT):
                    a = a + q[t] * window(t, r0, w)
                state.setdefault(r0, []).append(a + pltpu.roll(a, 2 * AH, 1))

        def fold(r0, half, late):
            for w in range(half * AW // 2, (half + 1) * AW // 2):
                a = state[r0][w]
                a = (a + pltpu.roll(a, AH, 1)) * (AD ** -0.5)
                if isinstance(i, int) and r0 < ADIL * w:
                    pos = lax.broadcasted_iota(jnp.int32, (RC, 128), 0) + r0
                    a = jnp.where(pos >= ADIL * w, a, MASKED)
                state[r0][w] = a

        def weights(r0, late):
            m = late(functools.reduce(jnp.maximum, state[r0]))
            state[r0] = [jnp.exp(a - m) for a in state[r0]]

        def mix(r0, tiles, late):
            e = [late(state[r0][0])] + state[r0][1:]
            if 0 in tiles:
                state[r0, "inv"] = _inverse(functools.reduce(jnp.add, e))
            for t in tiles:
                o = e[0] * window(LT + t, r0, 0)
                for w in range(1, AW):
                    o = o + e[w] * window(LT + t, r0, w)
                oa_s[t, r0:r0 + RC, :] = o * state[r0, "inv"]

        stages = ((logits, 0), (logits, 1), (fold, 0), (fold, 1), (weights,), (mix, (0, 1)), (mix, (2, 3, 4)))
        return [[functools.partial(f, r0, *args) for r0 in range(slot(i), slot(i) + TB, RC)] for f, *args in stages]

    def a_pack(i):
        def pack(k):
            ob[k] = oa_s[k, slot(i):slot(i) + TE, :].astype(BF16)
            ol[k, _ds(i, TL), :] = oa_s[k, slot(i) + TE:slot(i) + TB, :].astype(BF16)
        return [functools.partial(pack, k) for k in range(LT)]

    def a_out(i):
        acc = {}

        def tile(t, k):
            r = _dot(_load(ob, k), _load(wo_p, t, _ds(k, 64)))
            acc[t] = acc[t] + r if k else r
            return r

        def end(t):
            outa[i, :, t * 128:(t + 1) * 128] = acc[t].astype(BF16)
        return [(TE, functools.partial(tile, t, k), functools.partial(end, t) if k == LT - 1 else None)
                for t in range(LT) for k in range(LT)]

    def overlap(tiles, side=(), zero=None):
        due = sorted((lo + (hi - lo) * n / len(tasks), m, n, task, ref)
                     for m, (lo, hi, tasks, ref) in enumerate(side) for n, task in enumerate(tasks))
        free = [0] * 4
        results = []
        for count, tile, end in tiles:
            now = min(free)
            free[free.index(now)] += count
            results.append((now, tile()))
            while due and (due[0][0] < min(free) or len(results) == len(tiles)):
                time, _, _, task, ref = due.pop(0)
                begin, r = [x for x in results if x[0] <= time][-1]
                row = min(int(time - begin), r.shape[0] - 1) // 8 * 8
                if isinstance(ref, str):
                    task(lambda x: jnp.where(zero == 0, x, r[row:row + 8]))
                    continue
                if ref is bx:
                    ref[pl.ds(pl.multiple_of(S + 16 * zero, 16), 16), 0:128] = r[row // 16 * 16:row // 16 * 16 + 16].astype(BF16)
                elif ref is not None:
                    ref[(ref.shape[0] - 1 - zero,) + (0,) * (len(ref.shape) - 3) + (slice(0, 8),)] = (
                        pltpu.bitcast(r[row:row + 8], ref.dtype))
                task()
            if end:
                end()

    def w_transpose(c, n):
        size = NPL if isinstance(c, int) else CG * LT
        first = c * CG * LT
        at = [FT * j + t for j, t in TILES[n::CG * LT]]
        if isinstance(c, int):
            at = at[c]
        else:
            words = [sum(x << 8 * k for k, x in enumerate(at[m::5])) for m in range(5)]
            word = functools.reduce(lambda x, m: jnp.where(lax.rem(c, 5) == m, words[m], x), range(1, 5), words[0])
            at = lax.shift_right_logical(word, lax.div(c, 5) * 8) & 255
        wb.at[pl.ds(first, size)][n] = pltpu.bitcast(raw[_ds(at, 128), :].T, U32)

    def combine(tile, dst, r, i):
        row = col = tile(i, i)
        for k in range(LT):
            if k != i:
                a, b = tile(i, k), tile(k, i)
                row, col = row - a, col - b
                if k > i:
                    dst[LT + PAIRS.index((i, k)), 16 * r:16 * r + 16, :] = (a - b).astype(BF16)
        dst[i, 16 * r:16 * r + 16, :] = row.astype(BF16)
        dst[NZ + i, 16 * r:16 * r + 16, :] = col.astype(BF16)

    def w_combine(c, u, r, i):
        tiles = wb.at[pl.ds(c * CG * LT, CG * LT)]
        combine(lambda i, j: pltpu.bitcast(tiles[u * LT + j, pl.ds(i * 64 + 8 * r, 8), :], BF16).astype(F32),
                wz.at[pl.ds(c * CG, CG)].at[u], r, i)

    def wo_combine(g, r, i, late):
        def tile(a, b):
            x = wo_rows((W0 + g * LT + a) * 128 + 16 * r, 16, b).astype(F32)
            return jnp.concatenate([late(x[0:8]), x[8:]], axis=0)
        combine(tile, wz.at[NG + g], r, i)

    def halves(s):
        x = bx[_ds(s, SEG), :].astype(F32)
        return [[x[r:r + HALF, i * 128:(i + 1) * 128] for i in range(LT)] for r in (0, HALF)]

    def long_lhs(a, b, dst, i):
        p = [a[k] + LAM[k] * b[k] if LAM[k] else a[k] for k in range(LT)]
        dst[i] = b[i].astype(BF16)
        for k in ((i + 1) % LT, (i + 2) % LT):
            lo, hi = sorted((i, k))
            dst[LT + PAIRS.index((lo, hi))] = ((p[lo] + p[hi]) * (1.0 / (LAM[lo] - LAM[hi]))).astype(BF16)

    def short_lhs(a, b, j):
        p = [a[i] + LAM[j] * b[i] if LAM[j] else a[i] for i in range(LT)]
        return [p[j] if i == j else (p[i] + p[j]) * (1.0 / (LAM[j] - LAM[i])) for i in range(LT)]

    def z_lhs(s, i):
        long_lhs(*halves(s), lz.at[:, _ds(s, HALF), :], i)

    def z_batch(t):
        return [functools.partial(z_lhs, t * ZB + u, i) for u in range(ZB) for i in range(LT)]

    def z_product(g, n, batch):
        return _dot(_load(lz, n, _ds(batch, ZB * HALF // 2)), _load(wz, g, n))

    def z_group(g, batch):
        dst = z.at[z_index(g, batch)]

        sums, stored = {}, set()

        def tile(n):
            r = z_product(g, n, batch)
            for i in (n,) if n < LT else PAIRS[n - LT]:
                sums[i] = sums[i] + r if i in sums else r
            return r

        def end():
            for i in sums:
                z_add(dst, i, sums[i], i not in stored)
                stored.add(i)
            sums.clear()
        sets = (((0, 1), (0, 2), (1, 2), 0, 1), ((0, 3), (0, 4), (3, 4), 3, 4), ((1, 3), (1, 4), (2, 3), (2, 4), 2))
        return [(ZB * HALF, functools.partial(tile, LT + PAIRS.index(n) if n in PAIRS else n), end if n == some[-1] else None)
                for some in sets for n in some]

    def z_add(dst, n, r, first=True):
        for i in (n,) if n < LT else PAIRS[n - LT]:
            for u in range(ZB):
                x = r[u * HALF:(u + 1) * HALF]
                dst[u, i * HALF:(i + 1) * HALF, :] = x if n < LT and first else x + dst[u, i * HALF:(i + 1) * HALF, :]

    def z_index(g, batch):
        if isinstance(batch, int) and batch == 0:
            return g
        if isinstance(g, int) and g >= G0:
            return g + (batch % 2) * (NG - G0)
        return jnp.where(batch == 0, g, 2 * (NG - G0) + batch * G0 + g)

    if not CFG.get('onlyB'):
        flag[0] = 0
        c_second = [c_wqkv[1]] + c_ax(0, NS * TB, sem_a.at[1])
        start([c_wqkv[0]] + c_second)
        c_wqkv[0].wait()
        zero = flag[0]
        _mark('w0')
        _run(sum(prep_wqkv(0), []))
        start([c_wqkv[2], c_bx0])
        wait(c_second)
        _mark('w1')
        first, second = prep_wqkv(1)
        overlap(a_proj(0, 0) + a_proj(1, 0), [(0, 0, first, None), (700, 1500, second, tmp)], zero)
        start([c_awo] + c_first[:CFG["n1"]])
        wait([c_wqkv[2], c_bx0])
        _mark('w2')
        first, second = prep_wqkv(2)
        overlap(a_proj(0, 1) + a_proj(1, 1),
                [(0, 0, first, None), (700, 1500, second, tmp), (0, 1500, z_batch(0) + z_batch(1), bx)], zero)
        start(c_first[CFG["n1"]:])
        c_awo.wait()
        _mark('w3')
        e = CFG["e"]
        overlap(a_proj(0, 2) + a_proj(1, 2) + a_out(0),
                [(0, 800, prep_wo(), tmp), (1500, 1500, a_pack(0), None)]
                + [(e[i] + d, e[i + 1] + d, tasks, "value")
                   for i in range(NS) for d, tasks in zip(CFG["lags%d" % i], a_attention(i))], zero)
        start(c_step(1) + c_step(2))
        _mark('pre_first')
        wait(c_first)

        def a_step(c, carry):
            _mark('a_top')
            whole = raw.at[pl.ds(0, sum(STEP) + 2 * TB), :]
            pl.when((c > 0) & (c < NST))(cp(whole, whole, sem_w.at[c]).wait)

            for copy in c_last:
                pl.when(c == NST)(copy.wait)

            _mark('a_go')
            f = CFG["f"]
            zero = lax.shift_right_logical(c, 16)
            flag[zero] = 0
            if G0 == 2:
                early = z_group(0, c + 1) + z_group(1, c + 1)
            else:
                early = [x for u in range(2) for t in range(2) for x in z_group((c & 1) * 2 + u, (c | 1) + t)]
            overlap(a_proj(c + NS, 0) + a_proj(c + NS, 1) + a_proj(c + NS, 2) + a_out(c + NS - 1)
                    + z_group(c * CG, 0) + early + z_group(c * CG + 1, 0), [
                (0, f[0], [functools.partial(w_transpose, c, n) for n in range(CG * LT)], None),
                (0, f[1], z_batch(c + G0 // 2), bx),
                (0, f[1], a_pack(c + NS - 1), oa_s),
                (f[1], f[2], [functools.partial(w_combine, c, u, r, i)
                              for u in range(CG) for r in range(8) for i in range(LT)], wb),
            ] + [(f[3] + d, f[4] + d, tasks, "value") for d, tasks in zip(CFG["lags"], a_attention(c + NS))], zero)
            for copy in c_step(jnp.minimum(c + 3, NST - 1)) + c_wo(0, c, WO_STEP, sem_a.at[5]):
                pl.when(c < NST - 3)(copy.start)
            for copy in c_last:
                pl.when(c == NST - 3)(copy.start)
            for copy in c_wo(WO_FIRST, jnp.clip(c - (NST - 2), 0, 1), (H * DH - WO_FIRST) // 2, sem_a.at[7]):
                pl.when((c > NST - 3) & (c < NST))(copy.start)
            return carry

        lax.fori_loop(0, NCH, a_step, 0)
        _mark('epi')
        part = wo.at[:, pl.ds(0, WO_FIRST), :]
        cp(part, part, sem_a.at[5]).wait()
        h = CFG['h']
        overlap([x for g in range(G0) for x in z_group(g, NSEG // ZB - 1)] + a_out(NB - 1),
                [(0, 0, [functools.partial(w_transpose, NCH, n) for n in range(NPL)], None),
                 (0, h[0], a_pack(NB - 1), oa_s),
                 (h[1], h[2], [functools.partial(wo_combine, g, r, i)
                               for g in range(WG) for r in range(8) for i in range(LT)], "value")], zero)
        _mark('pre_wo')
        part = wo.at[:, pl.ds(WO_FIRST, H * DH - WO_FIRST), :]
        cp(part, part, sem_a.at[7]).wait()

    def rows(r0, n):
        return slice(r0, r0 + n)

    def r_lhs(hb, i, j):
        return R_LHS + ((hb * LT + i) * LT + j) * (M + HALF)

    def r_qkv(j, t):
        return rows(R_QKV + (j * FT + t) * L, L)

    def token_lhs(s, hb):
        a, b = halves(s)
        for j in range(LT):
            buf[rows(R_H + (hb * LT + j) * L + M, SEG)] = jnp.concatenate([a[j], b[j]], axis=0)
            for i, x in enumerate(short_lhs(a, b, j)):
                buf[rows(r_lhs(hb, i, j) + M, HALF)] = x

    def memory_lhs(m, n, hb):
        buf[rows(R_H + (hb * LT + n) * L, M)] = m[n]
        buf[rows(r_lhs(hb, n, n), M)] = m[n]
        for k in range(n):
            buf[rows(r_lhs(hb, n, k), M)] = buf[rows(r_lhs(hb, k, n), M)] = m[n] + m[k]

    def out_product(g, n):
        return _dot(_load(lo, g - NG, n), _load(wz, g, n))

    def out_finish(g, n, r, batch):
        z_add(zo, n, r, g == NG)
        for i in range(LT):
            if g == NG + WG - 1 and n == LT + max(k for k, pair in enumerate(PAIRS) if i in pair):
                for u in range(ZB):
                    y = zo[u, rows(i * HALF, HALF), :]
                    y = jnp.concatenate([-LAM[i] * y, y], axis=0)
                    outb[_ds(batch * ZB + u, SEG), rows(i * 128, 128)] = (op[u, i] + y).astype(BF16)

    lo_next, op_next = lo, op
    stored = set()

    def segment(plan, batch, part, hb, nh, before=()):
        s = batch * ZB + part
        key = lax.broadcasted_iota(jnp.int32, (L, 128), 0)
        col = lax.broadcasted_iota(jnp.int32, (L, 128), 1)
        head0 = col < L
        query = jnp.where(head0, col, col - L)
        visible = (query < M) | (query >= key)
        low = lax.broadcasted_iota(jnp.int32, (L, 128), 1) < 64
        val, sums = {}, {}
        fenced = buf.at[pl.ds(pl.multiple_of(lax.shift_right_logical(batch, 16) * 32, 32), R_END)]
        z_next = z.at[pl.ds(z_index(G0, batch + 1), NG - G0)]
        new_mem = []

        def add(name, x):
            val[name] = val[name] + x if name in val else x

        def product(*args):
            r = _dot(*args)
            val["latest"] = r[-8:]
            return r

        def short(g, i, j):
            if i == j:
                w = _load(wz, g, NZ + i)
            elif g < NG:
                w = pltpu.bitcast(wb[g * LT + j, rows(i * 64, 64), :], BF16)
            else:
                w = wo_rows((W0 + (g - NG) * LT + i) * 128, 128, j)
            at = r_lhs(hb, i, j) if g < NG else R_OL + r_lhs(g - NG, i, j)
            if CFG["fence"] and g > 0 and i == j and i in CFG["fence"]:
                x = jnp.concatenate([buf[rows(at, 16)], fenced[rows(at + 16, 8)]], axis=0)
            else:
                x = buf[rows(at, M + HALF)]
            add((min(g, NG), i, j), product(x, w))

        def take(g, i, j):
            if NG <= g < NG + WG - 1:
                return
            g = min(g, NG)
            r = val.pop((g, i, j))
            add(("m", g, j), r[0:M])
            if i != j:
                add(("y", g, i), r[M:])
                add(("d", g, j), r[M:])
                if LAM[i]:
                    add(("c", g, j), r[M:] * -LAM[i])
                return
            y = val.pop(("y", g, j))
            if g < NG:
                y = y + z[z_index(g, batch), part, rows(j * HALF, HALF), :]
            c = val.pop(("c", g, j)) + r[M:]
            if LAM[j]:
                c = c - LAM[j] * y
            r = jnp.concatenate([val.pop(("m", g, j)), c, val.pop(("d", g, j)) + y], axis=0)
            if g < NG:
                put(*TILES[g * LT + j], r)
            else:
                buf[rows(R_ACC + j * L, L)] = out_sum(j, r)

        def put(j, t, r):
            if j == 1 or not CFG["qv16"]:
                buf[r_qkv(j, t)] = r
                return
            none = jnp.zeros((8, 128), F32)
            if t % 3 == 1:
                r = [jnp.where(low, r, 0.0), jnp.where(low, 0.0, r)]
            else:
                r = [none, r] if (j, t % 3) == (0, 2) else [r, none]
            r = jnp.concatenate(r, axis=0).astype(BF16)
            qv[j // 2, t, 0:r.shape[0], :] = r

        def get(j, t, height):
            n = L if t % 3 == 1 else 24
            before = 16 if (j, t % 3) == (0, 2) else 0
            parts = [jnp.zeros((before, 128), U32), qv.bitcast(U32)[j // 2, t, 0:n, :],
                     jnp.zeros((max(height - before - n, 0), 128), U32)]
            return pltpu.bitcast(jnp.concatenate([x for x in parts if x.shape[0]], axis=0), BF16)

        def out_sum(n, r):
            if ("acc", n) in val:
                r = r + buf[rows(R_ACC + n * L, L)]
            val["acc", n] = True
            return r

        def out_lhs(g, j):
            o = [buf[rows(R_O + (W0 + g * LT + i) * L, L)] for i in range(LT)]
            a, b = [x[M:M + HALF] for x in o], [x[M + HALF:] for x in o]
            a[j] = jnp.concatenate([jnp.where(batch >= 0, x, val["latest"]) for x in (a[j][0:8], a[j][8:])], axis=0)
            for i, x in enumerate(short_lhs(a, b, j)):
                m = o[j][0:M] if i == j else o[i][0:M] + o[j][0:M]
                val["lhs", g, j, i] = jnp.concatenate([m, x], axis=0)
            long_lhs(a, b, lo_next.at[g, :, rows(part * HALF, HALF), :], j)

        def out_lhs_end(g, j):
            for i in range(LT):
                buf[rows(R_OL + r_lhs(g, i, j), M + HALF)] = val.pop(("lhs", g, j, i))

        def plain(n, k):
            w = pltpu.bitcast(wb[NG * LT + n, rows(k * 64, 64), :], BF16)
            val["plain", n, k] = product(buf[rows(R_H + (hb * LT + k) * L, L)], w)

        def plain_end(n, k):
            dst = r_qkv(*TILES[NG * LT + n])
            r = val.pop(("plain", n, k))
            r = r + buf[dst] if k else r
            if k < LT - 1:
                buf[dst] = r
            else:
                put(*TILES[NG * LT + n], r)

        def long(g, n):
            val["long", g, n] = z_product(g, n, batch + 1) if g < NG else out_product(g, n)
            val["latest"] = val["long", g, n][24:32]

        def long_end(g, n):
            if g < NG:
                r = val.pop(("long", g, n))
                if not CFG["zsum"]:
                    return z_add(z_next.at[g - G0], n, r)
                for i in (n,) if n < LT else PAIRS[n - LT]:
                    sums[g, i] = sums[g, i] + r if (g, i) in sums else r
            else:
                out_finish(g, n, val.pop(("long", g, n)), jnp.maximum(batch - 1, 0))

        def long_store():
            for (g, i), r in sums.items():
                z_add(z_next.at[g - G0], i, r, (g, i) not in stored)
                stored.add((g, i))
            sums.clear()

        def late(u, t, k):
            n = ZB * HALF
            x = _load(ol, k, _ds(part * (NB * TL // (ZB * n)) + u, n // 2))
            add("late", product(x, _load(wo_p, t, _ds(k, 64))))
            if k == LT - 1:
                r = val.pop("late").astype(BF16)
                for m in range(n // TL):
                    outl[part * (NB // ZB) + u * (n // TL) + m, :, rows(t * 128, 128)] = r[m * TL:(m + 1) * TL]

        def score(p, both):
            if both:
                q, k = [[buf[r_qkv(j, 3 * p + t)] for t in (0, 2)] for j in (0, 1)]
            else:
                q, k = buf[r_qkv(0, 3 * p + 1)], [buf[r_qkv(1, 3 * p + 1)]]
                q = [jnp.where(low, q, 0.0), jnp.where(low, 0.0, q)]
            q = jnp.concatenate(q + [jnp.zeros((128 - 2 * L, 128), F32)], axis=0)
            r = product(jnp.concatenate(k, axis=0), q.astype(BF16), NT)
            add(("s", p), jnp.where(head0, r[0:L], r[L:]) if both else r)

        def softmax(p, step):
            def late(x):
                return jnp.where(col[0:8] < 2 * L, x, val["latest"]) if step in CFG["ties"] else x

            def groups(x):
                return [x[r:r + 8] for r in range(0, L, 8)]

            def spread(x):
                return jnp.concatenate([x] * (L // 8), axis=0)
            x, y = val["s", p], val.get(("t", p))
            if step == 0:
                x = jnp.where(visible, x * (DH ** -0.5), MASKED)
                y = functools.reduce(jnp.maximum, groups(x))
            elif step == 1:
                y = jnp.broadcast_to(jnp.max(late(y), axis=0, keepdims=True), (8, 128))
            elif step == 2:
                x = jnp.exp(x - spread(late(y)))
                y = functools.reduce(jnp.add, groups(x))
            elif step == 3:
                y = jnp.broadcast_to(jnp.sum(late(y), axis=0, keepdims=True), (8, 128))
            elif step == 4:
                y = _inverse(late(y))
            elif step == 6:
                buf[rows(R_P + p * 2 * L, 2 * L), 0:2 * L] = x
            else:
                x = x * spread(late(y))
                x = jnp.concatenate([x, x], axis=0)[:, 0:2 * L]
                x = x.astype(BF16).T.astype(F32)
            val["s", p], val["t", p] = x, y

        def pv(t):
            pa, pb = [buf[rows(R_P + (2 * (t // 3) + u) * L, L), 0:2 * L] for u in range(2)]
            v = buf[r_qkv(2, t)]
            if t % 3 == 1:
                v = jnp.concatenate([jnp.where(low, v, 0.0), jnp.where(low, 0.0, v)], axis=0)
            pr = (pa[:, 0:L], jnp.where(head0[:, 0:2 * L], pa, pb), pb[:, 0:L])[t % 3]
            if CFG["qv16"]:
                pr = (pa[:, 0:48], pr, pb[:, 0:48])[t % 3]
            val["o", t] = product(pr, get(2, t, 0) if CFG["qv16"] else v.astype(BF16))

        def pv_end(t):
            buf[rows(R_O + t * L, L)] = val.pop(("o", t))

        def out(t, n):
            add(("out", t // KC, n), product(buf[rows(R_O + t * L, L)], wo_rows(t * 128, 128, n)))

        def out_end(t, n):
            r = out_sum(n, val.pop(("out", t // KC, n)))
            if t < FT - 1:
                buf[rows(R_ACC + n * L, L)] = r
                return
            new_mem.append(r[0:M])
            memory_lhs(new_mem, n, nh)
            if isinstance(part, int) and WG:
                op_next[part, n] = r[M:L]
            else:
                outb[_ds(s, SEG), rows(n * 128, 128)] = r[M:L].astype(BF16)

        tasks = dict(short=short, take=take, plain=plain, plain_end=plain_end, long=long, long_end=long_end,
                     score=score, softmax=softmax, pv=pv, pv_end=pv_end,
                     late=late, long_store=long_store, out=out, out_end=out_end, out_lhs=out_lhs, out_lhs_end=out_lhs_end,
                     token_lhs=lambda: token_lhs(jnp.minimum(s + 1, NSEG - 1), nh))
        before = list(before)
        for name, *args in plan[0]:
            need = max(args[1:]) if name in ("short", "plain") else LT - 1 if name == "pv" else -1
            while len(before) > LT - 1 - need:
                before.pop(0)()
            tasks[name](*args)
        return [functools.partial(tasks[name], *args) for name, *args in plan[1]]

    if CFG.get('onlyB'):
        start(c_first + [cp(wo_hbm.at[:, pl.ds(0, 128)], wo.at[0], sem_a.at[5]), c_mem])
        w_transpose(0, 0)
        w_combine(0, 0, 0, 0)
        z_lhs(0, 0)
        zero = flag[0]
        ol[0, 0:16] = wo_p[0, 0:16] = bx[0:16, 0:128]
        overlap(z_group(0, 0))
    token_lhs(0, 0)
    mem0 = mem[0:M, :].astype(F32)
    for n in range(LT):
        memory_lhs([mem0[:, k * 128:(k + 1) * 128] for k in range(LT)], n, 0)

    longs = ([("long", NG + g, n) for n in range(NZ) for g in range(WG)]
             + [("long", g, n) for g in range(G0, NG) for n in (Z_ORDER if CFG['zsum'] else range(NZ))])
    main_plans = [_make_plan(CFG["r%d" % u] if "r%d" % u in CFG else CFG["rounds"], longs, WG) for u in range(UN)]
    if WG:
        order = main_plans[0][0]
        assert order.index(("long", NG + WG - 1, NZ - 1)) < order.index(("out_lhs", 0, 0))
    assert not longs or UN < ZB
    late = [("late", u, t, k) for u in range(NB * TL // (ZB * ZB * HALF)) for t in range(LT) for k in range(LT)]
    last_plan = _make_plan(CFG["last_rounds"], late, 0)
    assert not late
    n_main = NSEG // ZB - 1

    def b_step(it, carry):
        _mark('b')
        rest = ()
        for u in range(UN):
            rest = segment(main_plans[u], it, u, u, (u + 1) % UN, rest)
        _run(rest)
        if WG:
            pl.when(it > 0)(lambda: c_outb(pl.multiple_of((it - 1) * ZB * SEG, SEG), ZB * SEG).start())
        else:
            c_outb(pl.multiple_of(it * ZB * SEG, SEG), ZB * SEG).start()
        return carry

    def last_step(s, carry):
        _mark('last')
        _run(segment(last_plan, s // ZB, s % ZB, 0, 0))
        c_late(s % ZB).start()
        c_outb(pl.multiple_of(s * SEG, SEG), SEG).start()
        return carry

    c_outa.start()
    if CFG.get('onlyB') != 2 and not CFG.get('onlyA'):
        lax.fori_loop(0, n_main, b_step, 0)
        if WG:
            for n in range(NZ):
                for g in range(NG, NG + WG):
                    out_finish(g, n, out_product(g, n), n_main - 1)
            c_outb((n_main - 1) * ZB * SEG, ZB * SEG).start()
    if CFG.get('onlyB') != 1 and not CFG.get('onlyA'):
        lax.fori_loop(n_main * ZB, NSEG, last_step, 0)
    if CFG.get('onlyA'):
        outb[0:16, 0:128] = (z[0, 0, 0:16] + pltpu.bitcast(wb[0, 0:16], F32) + buf[0:16] + lz[0, 32:48].astype(F32)).astype(BF16)
        start([c_outb(t * TB, TB) for t in range(NB)] + [c_late(u) for u in range(ZB)])
    _mark('end')
    c_outa.wait()
    cp(outb, outb, sem_o.at[1]).wait()
    cp(outl, outl, sem_o.at[2]).wait()


def pallas_concat_heads__sliding_local_dilated__memory_aug_recurrent_mem_tr__prompt_kernel(
    A_x, A_wqkv, A_wo, B_x, B_mem0, B_Wq, B_Wk, B_Wv, B_Wo, B_seg_len,
):
    assert B_seg_len == SEG
    assert A_x.shape == B_x.shape == (1, S, D) and B_mem0.shape == (1, M, D)
    assert B_Wq.shape == B_Wk.shape == B_Wv.shape == (D, H, DH) and B_Wo.shape == (H, DH, D)
    vmem, dma = pltpu.VMEM, pltpu.SemaphoreType.DMA
    call = pl.pallas_call(
        _kernel,
        out_shape=jax.ShapeDtypeStruct((NB, TB, 2 * D), BF16),
        in_specs=[pl.BlockSpec(memory_space=pl.ANY)] * 9,
        out_specs=pl.BlockSpec(memory_space=pl.ANY),
        scratch_shapes=[
            vmem((LT, S, 128), BF16),
            vmem((D, D), BF16),
            vmem((LT + 1, D, 128), F32),
            vmem((LT, 3 * D, 128), BF16),
            vmem((LT, D, 128), BF16),
            vmem((LT, NS * TB, 128), F32),
            vmem((2 * LT, HALO + NS * TB, 128), F32),
            vmem((LT + 1, NS * TB, 128), F32),
            vmem((LT + 1, TE, 128), BF16),
            vmem((LT, NB * TL, 128), BF16),
            vmem((NB, TE, D), BF16),
            vmem((NB, TL, D), BF16),
            vmem((S + 64, D), BF16),
            vmem((64, D), BF16),
            vmem((3 * H * DH, D), BF16),
            vmem((len(TILES) + 1, D // 2, 128), U32),
            vmem((NG + WG, NZ + LT, 128, 128), BF16),
            vmem((LT, H * DH, 128), BF16),
            vmem((NZ, S // 2, 128), BF16),
            vmem((2 * (NG - G0) + NSEG // ZB * G0, ZB, LT * HALF, 128), F32),
            vmem((max(WG, 1), NZ, ZB * HALF, 128), BF16),
            vmem((ZB, LT * HALF, 128), F32),
            vmem((ZB, LT, SEG, 128), F32),
            vmem((2, FT, 2 * L, 128), BF16),
            vmem((R_END, 128), F32),
            pltpu.SMEM((2,), jnp.int32), dma((8,)), dma((NCH,)), dma((3,)),
        ],
        compiler_params=pltpu.CompilerParams(vmem_limit_bytes=126 * 1024 * 1024,
                                             internal_scratch_in_bytes=48 * 1024, disable_bounds_checks=True, disable_semaphore_checks=bool(CFG.get('nosem')), flags=CFG.get("flags")),
        name="sliding_and_memory_attention",
    )

    def by_feature(w):
        return w.transpose(1, 2, 0).reshape(H * DH, D)

    out = call(A_x.reshape(S, D), A_wqkv, A_wo, B_x.reshape(S, D), B_mem0.reshape(M, D),
               by_feature(B_Wq), by_feature(B_Wk), by_feature(B_Wv), B_Wo.reshape(H * DH, D))
    return out.reshape(1, S, 2 * D)
```

```python
import functools

import jax
import jax.numpy as jnp
from jax import lax
from jax.experimental import pallas as pl
from jax.experimental.pallas import tpu as pltpu

F32, BF16, U32 = jnp.float32, jnp.bfloat16, jnp.uint32
NN = (((1,), (0,)), ((), ()))
NT = (((1,), (1,)), ((), ()))
MASKED = -1000000000.0

S, D = 2048, 640
LT = D // 128

AH, AD, AW, ADIL = 32, 20, 8, 2
HALO = 16
TB = 128
NB = S // TB
NS = 2
TL = 32
TE = TB - TL
RC = 8

H, DH, M, SEG = 32, 192, 8, 32
L = M + SEG
HALF = SEG // 2
NP = H // 2
FT = 3 * NP
NSEG = S // SEG
LAM = (0.0, 0.625, -0.625, 1.875, -1.875)
PAIRS = [(i, j) for i in range(LT) for j in range(i + 1, LT)]
NZ = LT + len(PAIRS)
NG = 28
WG = 2
G0 = 4
ZB = TB // SEG
KC = 3
CG = 2
NCH = NG // CG
NST = NCH - 2
FIRST, STEP = (864, 688, 0), (480, 496, 432)
WO_STEP = 256
WO_FIRST = (NST - 3) * WO_STEP

ROUNDS = (
    "PsLssssLssssLssssLssssLssssLssssLssssLsQssssLssssLssssLssssLssQsssVssssLssssLssssLssssLsssVssssLssQsssVs"
    "sssLssssLssssLssssLssQsssVsWssssLssssLssWWssssLsssVsWssWssVssWsssQsWsWssssWQsWssWsWWssWsWssVsssWWWsssVsW"
    "sWsWssWssWWWsssVssQsWsWsWsQsssWWWsssVswWsWwWssVwWwwwWWVwwwWwWWwwWWwWWWWW",
    "LPssssLssssLssssLssssLssssLssssLssssLssssLssssLssssLssssLsssQsQsssssLssssLssssLsssVsssVsQssssVssLssWssWs"
    "sLssQsssVssssLssssLssssLssssLssssLssssLssssLssssVsWsWsWssVssWsWWssWssQsWsWsWsQssWWssWsssVsWsWsWsWsWsWssV"
    "ssssLsWsssWWsWssVssQsWsWsWsQsssWWsWswVswWsWWswwVwsWWsWwWwwwVwWWwWwwWWWWWW",
    "LPssssLssssLssssLssssLssssLsQssssLssssLssssLssssLssssLssssVsQssssLssssLssssLsssVssQsssVssssLssssLssssLss"
    "WWssQsssVssssLsssssLssssLssssLssssLssWsssVsWsWsWssVssssQsWsWsWssQsWssssLsWsWssssLsWsWsWssssVsWsWsWsssVsW"
    "sWsWssWssWWWsssVssQsWsWsWsQsssWWsWssVsWwwWWwwsVssWWwWwwwVwWWwWwWWwwWWWWW",
    "LPssssLssssLssssLssssLssssLssssLssssLssssLssssLssssLssssLsssQsQssssLssssLssssLssssVssVssQsssVsssLsWssWss"
    "sLssQsssVssssLssssLssssLssssLssssLssssLssssLssssVsWsWsWssVssWsWWssWssQsWsWsWsQssWWssWsssVsWsWsWsWsWsWssV"
    "ssssLsWsssWWsWssVssQsWsWsWsQsssWWsWswVswWsWWswwVwsWsWWwWwwwVwWWwWwwWWWWWW",
)
LAST_ROUNDS = (
    "PsssLssssLssssssLssssLssssQssLssssLssssLssssLssssssQssVssssWssssLssssLssssVsWsWsWsssVsWsWssssLsWssWssWss"
    "QsssssssQsssWWsssssLssssVssWWsssVsWsWsWsWsssVsWsWssssssLssWsWsssQsWsWsWsssQsssWssssVssWWsWssWWssWWssWsWs"
    "sVssssWsWsssWQsssVsWsssWWsQsWsssWWsWssVsWsssWWVWWVWWWWWWWWWWW"
)
LATENCY, SOFTMAX_STEP, LHS_STEP = 120, 24, 48
START_TIMES, START_LAGS = [300, 950, 1550], [[0, 22, 120, 142, 330, 500, 510], [0, 22, 120, 142, 330, 650, 655]]
LOOP_TIMES, LOOP_LAGS = [1240, 600, 2600, 2391, 4010], [2, 50, 174, 227, 346, 364, 416]
END_TIMES = [500, 0, 1530]


def _tile_order():
    lag = [2] * 8 + [3] * 4 + [4] * 4
    order = []
    for p in range(NP + max(lag)):
        if p < NP:
            order += [(j, 3 * p + t) for j in (0, 1) for t in range(3)]
        order += [(2, 3 * x + t) for x in range(NP) if x + lag[x] == p for t in range(3)]
    rest = [(2, t) for t in (11, 23, 35, 42)]
    return [x for x in order if x not in rest] + rest


TILES = _tile_order()
NPL = len(TILES) - NG * LT
assert all((t + 1) * 128 <= FIRST[j] + n // (CG * LT) * STEP[j] for n, (j, t) in enumerate(TILES[:NST * CG * LT]))

R_LHS = 0
R_H = R_LHS + ZB * LT * LT * (M + HALF)
R_QKV = R_H + ZB * LT * L
R_O = R_QKV + 3 * FT * L
R_P = R_O + FT * L
R_ACC = R_P + NP * 2 * L
R_OL = R_ACC + LT * L
R_END = (R_OL + WG * LT * LT * (M + HALF) + 31) // 32 * 32


def _targets(n):
    return (n,) if n < LT else PAIRS[n - LT]


def _long_index(name):
    return LT + PAIRS.index(name) if name in PAIRS else name


def _make_plan(rounds, longs, fast):
    shell = []
    for k in range(LT):
        for n in range(k + 1, LT):
            shell += [(k, n), (n, k)]
        shell += [(k, k)]
    todo = dict(
        L=longs,
        s=[("short", g, i, j) for g in range(NG) for (i, j) in shell],
        w=[("short", NG + g, i, j) for (i, j) in shell for g in range(fast)],
        W=[("out", t, n) for k in range(0, FT, KC) for n in range(LT) for t in range(max(k, fast * LT), k + KC)],
        P=[("plain", n, 0) for n in range(NPL)] + [("plain", n, k) for n in range(NPL) for k in range(1, LT)],
        Q=[("score", p + u, both) for p in range(0, NP, 2) for both in (p // 2 % 2, 1 - p // 2 % 2) for u in (0, 1)],
        V=[("pv", t) for t in range(FT)])
    plan, timed, now = [], [], 0

    def needs(name, *args):
        if name == "out":
            return [("pv_end", args[0])]
        if name == "short" and args[0] >= NG:
            return [("out_lhs", args[0] - NG, args[2])]
        if name not in ("score", "pv"):
            return []
        need = [("softmax", args[0] // 3, 5)] if name == "pv" else []
        for tile in [(2, args[0])] if name == "pv" else [(j, 3 * args[0] + t) for j in (0, 1) for t in range(3)]:
            g, j = divmod(TILES.index(tile), LT)
            need.append(("short_end", g, j, j) if g < NG else ("plain_end", j, LT - 1))
        return need

    for n, kind in enumerate(rounds):
        tasks = todo[kind][:4]
        del todo[kind][:4]
        if kind == "Q":
            tasks += [todo["P"].pop(0), todo["P"].pop(0)]
        while kind == "w" and len(tasks) < 4:
            tasks.append(todo["W"].pop(0))
        need = [x for task in tasks for x in needs(*task)]
        until = max([now] + [time for time, task in timed if task in need])
        timed.sort(key=lambda x: x[0])
        while timed and timed[0][0] <= until:
            plan.append(timed.pop(0)[1])
        assert all(x in plan for x in need)
        plan += tasks
        now += dict(s=M + HALF, w=M + HALF, L=ZB * HALF, Q=2 * L).get(kind, L)
        for name, *args in tasks:
            if name in ("short", "plain", "long", "pv") or (name == "out" and args[0] % KC == KC - 1):
                timed.append((now + LATENCY, (name + "_end", *args)))
            if name == "pv" and args[0] < fast * LT and args[0] % LT == LT - 1:
                timed += [(now + LATENCY + LHS_STEP * j, ("out_lhs", args[0] // LT, j)) for j in range(LT)]
            if name == "score" and args[1]:
                timed += [(now + SOFTMAX_STEP * (step + args[0] % 2), ("softmax", args[0], step)) for step in range(6)]
        if kind == "L":
            timed.append((now + LATENCY, ("long_store",)))
        if kind == "s" and kind not in rounds[n + 1:]:
            plan.append(("next_tokens",))
    assert not any(todo[kind] for kind in "swWPQV")
    return plan, [task for _, task in sorted(timed, key=lambda x: x[0])]


def _ds(i, n):
    return pl.ds(i * n if isinstance(i, int) else pl.multiple_of(i * n, n), n)


def _rows(r0, n):
    return slice(r0, r0 + n)


def _dot(a, b, dims=NN):
    r = lax.dot_general(a, b, dims, preferred_element_type=F32)
    return jnp.concatenate([r[0:8], r[8:]], axis=0)


def _inverse(x):
    r = pltpu.reciprocal(x, approx=True)
    return r + r * (1.0 - x * r)


def _load(ref, *index):
    return pltpu.bitcast(ref.bitcast(U32)[index], BF16)


def _run(tasks):
    for task in tasks:
        task()


def _short_lhs(a, b, j):
    p = [a[i] + LAM[j] * b[i] if LAM[j] else a[i] for i in range(LT)]
    return [p[j] if i == j else (p[i] + p[j]) * (1.0 / (LAM[j] - LAM[i])) for i in range(LT)]


def _long_lhs(a, b, dst, i):
    p = [a[k] + LAM[k] * b[k] if LAM[k] else a[k] for k in range(LT)]
    dst[i] = b[i].astype(BF16)
    for k in ((i + 1) % LT, (i + 2) % LT):
        lo, hi = sorted((i, k))
        dst[_long_index((lo, hi))] = ((p[lo] + p[hi]) * (1.0 / (LAM[lo] - LAM[hi]))).astype(BF16)


def _combine(tile, dst, r, i):
    row = col = tile(i, i)
    for k in range(LT):
        if k != i:
            a, b = tile(i, k), tile(k, i)
            row, col = row - a, col - b
            if k > i:
                dst[_long_index((i, k)), _rows(16 * r, 16), :] = (a - b).astype(BF16)
    dst[i, _rows(16 * r, 16), :] = row.astype(BF16)
    dst[NZ + i, _rows(16 * r, 16), :] = col.astype(BF16)


def _add_long(dst, i, r, first):
    for u in range(ZB):
        x = r[_rows(u * HALF, HALF)]
        dst[u, _rows(i * HALF, HALF), :] = x if first else x + dst[u, _rows(i * HALF, HALF), :]


def _z_index(g, batch):
    if isinstance(batch, int) and batch == 0:
        return g
    if isinstance(g, int) and g >= G0:
        return g + (batch % 2) * (NG - G0)
    return jnp.where(batch == 0, g, 2 * (NG - G0) + batch * G0 + g)


def _kernel(ax_hbm, awqkv_hbm, awo_hbm, bx_hbm, mem_hbm, wq_hbm, wk_hbm, wv_hbm, wo_hbm,
            out_hbm,
            ax, awo, tmp, wqkv_p, wo_p, q_s, kv_s, oa, ob, ol, outa, outl,
            bx, mem, raw, wb, wz, wo, lz, z, lo, zo, op, buf,
            flag, sem_a, sem_w, sem_o):
    awqkv = raw.at[pl.ds(3 * (H * DH - D), 3 * D), :]
    outb = raw.at[pl.ds(0, S), :]

    cp = pltpu.make_async_copy

    def span(first, i, n):
        return pl.ds(first + i * n if isinstance(i, int) else pl.multiple_of(first + i * n, 16), n)

    def c_strips(src, dst, at, sem):
        return [cp(src.at[at, pl.ds(t * 128, 128)], dst.at[t, at, :], sem) for t in range(LT)]

    def c_bx(i, n, sem):
        return cp(bx_hbm.at[_ds(i, n), :], bx.at[_ds(i, n), :], sem)

    def c_w(j, first, i, n, sem):
        return cp((wq_hbm, wk_hbm, wv_hbm)[j].at[span(first, i, n), :], raw.at[span(j * H * DH + first, i, n), :], sem)

    def c_x(c, sem):
        return c_strips(ax_hbm, ax, _ds(c + NS, TB), sem) + [c_bx(c + 2, TB, sem)]

    def c_step(c):
        return c_x(c, sem_w.at[c]) + [c_w(j, FIRST[j], c - 1, STEP[j], sem_w.at[c]) for j in range(3)]

    def c_outb(r0, n):
        at = r0 % TB if isinstance(r0, int) else pl.multiple_of(lax.rem(r0, TB), n)
        return cp(outb.at[pl.ds(r0, n), :], out_hbm.at[r0 // TB, pl.ds(at, n), pl.ds(D, D)], sem_o.at[1])

    def c_outl(u):
        at = pl.ds(u * (NB // ZB), NB // ZB)
        return cp(outl.at[at], out_hbm.at[at, pl.ds(TE, TL), pl.ds(0, D)], sem_o.at[2])

    def start(copies):
        for c in copies:
            c.start()

    def wait(copies):
        for c in copies:
            c.wait()

    def wait_filled(ref, sem):
        cp(ref, ref, sem).wait()

    def permute_rows(dst, base):
        def move(t, d0):
            for d in range(d0, d0 + AD // 4):
                dst[t, pl.ds(base + d * AH, AH), :] = tmp[t, pl.ds(d, AH, stride=AD), :].astype(BF16)
        return [functools.partial(move, t, d0) for t in range(LT) for d0 in range(0, AD, AD // 4)]

    def prep_wqkv(j):
        def transpose(t):
            tmp[t] = awqkv[_rows(j * D + t * 128, 128), :].astype(F32).T
        return [functools.partial(transpose, t) for t in range(LT)], permute_rows(wqkv_p, j * D)

    def prep_wo():
        def widen(t, r):
            tmp[t, _rows(r, D // 4), :] = awo[_rows(r, D // 4), _rows(t * 128, 128)].astype(F32)
        moves = permute_rows(wo_p, 0)
        return [task for t in range(LT)
                for task in [functools.partial(widen, t, r) for r in range(0, D, D // 4)] + moves[4 * t:4 * t + 4]]

    def slot(i):
        return i * TB if isinstance(i, int) and i < NS else (NS - 1) * TB

    def a_tiles(count, product, store):
        acc = {}

        def tile(t, k):
            r = product(t, k)
            acc[t] = acc[t] + r if k else r
            return r
        return [(count, functools.partial(tile, t, k), (lambda t=t: store(t, acc[t])) if k == LT - 1 else None)
                for t in range(LT) for k in range(LT)]

    def a_proj(i, j):
        at = slot(i)

        def store(t, r):
            if j == 0:
                q_s[t, _rows(at, TB), :] = r
                return
            c = (j - 1) * LT + t
            if not isinstance(i, int):
                kv_s[c, _rows(at, HALO), :] = kv_s[c, _rows(at + TB, HALO), :]
            elif i == 0:
                kv_s[c, 0:HALO, :] = jnp.broadcast_to(r[0:1, :], (HALO, 128))
            kv_s[c, _rows(at + HALO, TB), :] = r
        return a_tiles(TB, lambda t, k: _dot(_load(ax, k, _ds(i, TB // 2)), _load(wqkv_p, k, _ds(j * LT + t, 64)), NT),
                       store)

    def a_attention(i):
        state = {}

        def window(c, r0, w):
            return kv_s[c, _rows(HALO + r0 - ADIL * w, RC), :]

        def logits(r0, half, late):
            q = [q_s[t, _rows(r0, RC), :] for t in range(LT)]
            q[0] = late(q[0])
            for w in range(half * AW // 2, (half + 1) * AW // 2):
                a = q[0] * window(0, r0, w)
                for t in range(1, LT):
                    a = a + q[t] * window(t, r0, w)
                state.setdefault(r0, []).append(a + pltpu.roll(a, 2 * AH, 1))

        def fold(r0, half, late):
            for w in range(half * AW // 2, (half + 1) * AW // 2):
                a = state[r0][w]
                a = (a + pltpu.roll(a, AH, 1)) * (AD ** -0.5)
                if isinstance(i, int) and r0 < ADIL * w:
                    pos = lax.broadcasted_iota(jnp.int32, (RC, 128), 0) + r0
                    a = jnp.where(pos >= ADIL * w, a, MASKED)
                state[r0][w] = a

        def weights(r0, late):
            m = late(functools.reduce(jnp.maximum, state[r0]))
            state[r0] = [jnp.exp(a - m) for a in state[r0]]

        def mix(r0, tiles, late):
            e = [late(state[r0][0])] + state[r0][1:]
            if 0 in tiles:
                state[r0, "inverse"] = _inverse(functools.reduce(jnp.add, e))
            for t in tiles:
                o = e[0] * window(LT + t, r0, 0)
                for w in range(1, AW):
                    o = o + e[w] * window(LT + t, r0, w)
                oa[t, _rows(r0, RC), :] = o * state[r0, "inverse"]

        stages = ((logits, 0), (logits, 1), (fold, 0), (fold, 1), (weights,), (mix, (0, 1)), (mix, (2, 3, 4)))
        return [[functools.partial(f, r0, *args) for r0 in range(slot(i), slot(i) + TB, RC)] for f, *args in stages]

    def a_pack(i):
        def pack(k):
            ob[k] = oa[k, _rows(slot(i), TE), :].astype(BF16)
            ol[k, _ds(i, TL), :] = oa[k, _rows(slot(i) + TE, TL), :].astype(BF16)
        return [functools.partial(pack, k) for k in range(LT)]

    def a_out(i):
        def store(t, r):
            outa[i, :, _rows(t * 128, 128)] = r.astype(BF16)
        return a_tiles(TE, lambda t, k: _dot(_load(ob, k), _load(wo_p, t, _ds(k, 64))), store)

    def overlap(tiles, side, zero):
        due = sorted((lo + (hi - lo) * n / len(tasks), m, n, task, tie)
                     for m, (lo, hi, tasks, tie) in enumerate(side) for n, task in enumerate(tasks))
        free = [0] * 4
        results = []
        for count, tile, end in tiles:
            now = min(free)
            free[free.index(now)] += count
            results.append((now, tile()))
            while due and (due[0][0] < min(free) or len(results) == len(tiles)):
                time, _, _, task, tie = due.pop(0)
                begin, r = [x for x in results if x[0] <= time][-1]
                row = min(int(time - begin), r.shape[0] - 1) // 8 * 8
                if isinstance(tie, str):
                    task(lambda x: jnp.where(zero == 0, x, r[_rows(row, 8)]))
                    continue
                if tie is bx:
                    tie[span(S, zero, 16), 0:128] = r[_rows(row // 16 * 16, 16)].astype(BF16)
                elif tie is not None:
                    tie[tie.shape[0] - 1 - zero, 0:8, :] = pltpu.bitcast(r[_rows(row, 8)], tie.dtype)
                task()
            if end:
                end()

    def wo_rows(r0, n, t):
        return _load(wo, t, _rows(r0 // 2, n // 2))

    def w_transpose(c, n):
        at = [FT * j + t for j, t in TILES[n::CG * LT]]
        if isinstance(c, int):
            at = at[c]
        else:
            words = [sum(x << 8 * k for k, x in enumerate(at[m::5])) for m in range(5)]
            word = functools.reduce(lambda x, m: jnp.where(lax.rem(c, 5) == m, words[m], x), range(1, 5), words[0])
            at = lax.shift_right_logical(word, lax.div(c, 5) * 8) & 255
        chunk = wb.at[pl.ds(c * CG * LT, NPL if isinstance(c, int) else CG * LT)]
        chunk[n] = pltpu.bitcast(raw[_ds(at, 128), :].T, U32)

    def w_combine(c, u, r, i):
        chunk = wb.at[pl.ds(c * CG * LT, CG * LT)]
        _combine(lambda a, b: pltpu.bitcast(chunk[u * LT + b, _rows(a * 64 + 8 * r, 8), :], BF16).astype(F32),
                 wz.at[pl.ds(c * CG, CG)].at[u], r, i)

    def wo_combine(g, r, i, late):
        def tile(a, b):
            x = wo_rows((g * LT + a) * 128 + 16 * r, 16, b).astype(F32)
            return jnp.concatenate([late(x[0:8]), x[8:]], axis=0)
        _combine(tile, wz.at[NG + g], r, i)

    def halves(s):
        x = bx[_ds(s, SEG), :].astype(F32)
        return [[x[_rows(r, HALF), _rows(i * 128, 128)] for i in range(LT)] for r in (0, HALF)]

    def z_lhs(batch):
        def task(s, i):
            _long_lhs(*halves(s), lz.at[:, _ds(s, HALF), :], i)
        return [functools.partial(task, batch * ZB + u, i) for u in range(ZB) for i in range(LT)]

    def z_product(g, n, batch):
        return _dot(_load(lz, n, _ds(batch, ZB * HALF // 2)), _load(wz, g, n))

    def z_group(g, batch):
        dst = z.at[_z_index(g, batch)]
        sums, stored = {}, []

        def tile(n):
            r = z_product(g, n, batch)
            for i in _targets(n):
                sums[i] = sums[i] + r if i in sums else r
            return r

        def end():
            for i in sums:
                _add_long(dst, i, sums[i], i not in stored)
                stored.append(i)
            sums.clear()
        sets = (((0, 1), (0, 2), (1, 2), 0, 1), ((0, 3), (0, 4), (3, 4), 3, 4), ((1, 3), (1, 4), (2, 3), (2, 4), 2))
        return [(ZB * HALF, functools.partial(tile, _long_index(n)), end if n == some[-1] else None)
                for some in sets for n in some]

    def part_a():
        c_wqkv = [cp(awqkv_hbm.at[:, pl.ds(j * D, D)], awqkv.at[pl.ds(j * D, D), :], sem_a.at[j]) for j in range(3)]
        c_second = [c_wqkv[1]] + c_strips(ax_hbm, ax, pl.ds(0, NS * TB), sem_a.at[1])
        c_third = [c_wqkv[2], c_bx(0, 2 * TB, sem_a.at[2])]
        c_awo = cp(awo_hbm, awo, sem_a.at[3])
        c_first = c_x(0, sem_w.at[0]) + [c_w(j, 0, 0, FIRST[j], sem_w.at[0]) for j in range(2)]
        c_last = c_x(NST, sem_w.at[NST]) + c_x(NST + 1, sem_w.at[NST]) + [
            cp(mem_hbm, mem.at[pl.ds(0, M), :], sem_w.at[NST]),
            c_w(2, (NST - 1) * STEP[2], 0, H * DH - (NST - 1) * STEP[2], sem_w.at[NST])]

        flag[0] = 0
        start([c_wqkv[0]] + c_second)
        c_wqkv[0].wait()
        zero = flag[0]
        _run(sum(prep_wqkv(0), []))
        start(c_third)
        wait(c_second)
        first, second = prep_wqkv(1)
        overlap(a_proj(0, 0) + a_proj(1, 0), [(0, 0, first, None), (700, 1500, second, tmp)], zero)
        start([c_awo] + c_first[:-1])
        wait(c_third)
        first, second = prep_wqkv(2)
        overlap(a_proj(0, 1) + a_proj(1, 1),
                [(0, 0, first, None), (700, 1500, second, tmp), (0, 1500, z_lhs(0) + z_lhs(1), bx)], zero)
        c_first[-1].start()
        c_awo.wait()
        for i in range(NS):
            assert START_TIMES[i] + START_LAGS[i][-2] >= (i + 1) * 800
        assert START_TIMES[1] + START_LAGS[0][-1] <= 1500
        overlap(a_proj(0, 2) + a_proj(1, 2) + a_out(0),
                [(0, 800, prep_wo(), tmp), (1500, 1500, a_pack(0), None)]
                + [(START_TIMES[i] + d, START_TIMES[i + 1] + d, tasks, "value")
                   for i in range(NS) for d, tasks in zip(START_LAGS[i], a_attention(i))], zero)
        start(c_step(1) + c_step(2))
        wait(c_first)

        def step(c, carry):
            @pl.when((c > 0) & (c < NST))
            def _():
                wait_filled(ax.at[:, _ds(c + NS, TB), :], sem_w.at[c])
            for copy in c_step(jnp.clip(c, 1, NST - 1))[LT:]:
                pl.when((c > 0) & (c < NST))(copy.wait)
            pl.when(c == NST)(lambda: wait_filled(ax.at[:, pl.ds((NST + NS) * TB, 2 * TB), :], sem_w.at[NST]))
            for copy in [c_last[LT]] + c_last[2 * LT + 1:]:
                pl.when(c == NST)(copy.wait)

            zero = lax.shift_right_logical(c, 16)
            flag[zero] = 0
            i, t = c + NS, LOOP_TIMES
            assert t[0] / 2 <= t[1] + 100 and t[2] < 2900 and t[3] + LOOP_LAGS[-2] > 2500
            early = [x for u in range(2) for b in range(2) for x in z_group((c & 1) * 2 + u, (c | 1) + b)]
            overlap(a_proj(i, 0) + a_proj(i, 1) + a_proj(i, 2) + a_out(i - 1)
                    + z_group(c * CG, 0) + early + z_group(c * CG + 1, 0),
                    [(0, t[0], [functools.partial(w_transpose, c, n) for n in range(CG * LT)], None),
                     (0, t[1], z_lhs(c + 2), bx),
                     (0, t[1], a_pack(i - 1), oa),
                     (t[1], t[2], [functools.partial(w_combine, c, u, r, k)
                                   for u in range(CG) for r in range(8) for k in range(LT)], wb)]
                    + [(t[3] + d, t[4] + d, tasks, "value") for d, tasks in zip(LOOP_LAGS, a_attention(i))], zero)

            for copy in c_step(jnp.minimum(c + 3, NST - 1)) + c_strips(wo_hbm, wo, _ds(c, WO_STEP), sem_a.at[4]):
                pl.when(c < NST - 3)(copy.start)
            for copy in c_last:
                pl.when(c == NST - 3)(copy.start)
            at = span(WO_FIRST, jnp.clip(c - (NST - 2), 0, 1), (H * DH - WO_FIRST) // 2)
            for copy in c_strips(wo_hbm, wo, at, sem_a.at[5]):
                pl.when((c > NST - 3) & (c < NST))(copy.start)
            return carry

        lax.fori_loop(0, NCH, step, 0)
        wait_filled(wo.at[:, pl.ds(0, WO_FIRST), :], sem_a.at[4])
        t = END_TIMES
        overlap([x for g in range(G0) for x in z_group(g, NB - 1)] + a_out(NB - 1),
                [(0, 0, [functools.partial(w_transpose, NCH, n) for n in range(NPL)], None),
                 (0, t[0], a_pack(NB - 1), oa),
                 (t[1], t[2], [functools.partial(wo_combine, g, r, i)
                               for g in range(WG) for r in range(8) for i in range(LT)], "value")], zero)

    def r_lhs(hb, i, j):
        return R_LHS + ((hb * LT + i) * LT + j) * (M + HALF)

    def r_qkv(j, t):
        return _rows(R_QKV + (j * FT + t) * L, L)

    def token_lhs(s, hb):
        a, b = halves(s)
        for j in range(LT):
            buf[_rows(R_H + (hb * LT + j) * L + M, SEG)] = jnp.concatenate([a[j], b[j]], axis=0)
            for i, x in enumerate(_short_lhs(a, b, j)):
                buf[_rows(r_lhs(hb, i, j) + M, HALF)] = x

    def memory_lhs(m, n, hb):
        buf[_rows(R_H + (hb * LT + n) * L, M)] = m[n]
        buf[_rows(r_lhs(hb, n, n), M)] = m[n]
        for k in range(n):
            buf[_rows(r_lhs(hb, n, k), M)] = buf[_rows(r_lhs(hb, k, n), M)] = m[n] + m[k]

    def out_product(g, n):
        return _dot(_load(lo, g - NG, n), _load(wz, g, n))

    def out_finish(g, n, r, batch):
        for i in _targets(n):
            _add_long(zo, i, r, n < LT and g == NG)
            if g == NG + WG - 1 and n == max(k for k in range(NZ) if i in _targets(k)):
                for u in range(ZB):
                    y = zo[u, _rows(i * HALF, HALF), :]
                    y = jnp.concatenate([-LAM[i] * y, y], axis=0)
                    outb[_ds(batch * ZB + u, SEG), _rows(i * 128, 128)] = (op[u, i] + y).astype(BF16)

    stored = []

    def segment(plan, batch, part, hb, nh, before=()):
        s = batch * ZB + part
        key = lax.broadcasted_iota(jnp.int32, (L, 128), 0)
        col = lax.broadcasted_iota(jnp.int32, (L, 128), 1)
        head0 = col < L
        query = jnp.where(head0, col, col - L)
        visible = (query < M) | (query >= key)
        low = col < 64
        z_next = z.at[pl.ds(_z_index(G0, batch + 1), NG - G0)]
        val, sums, new_mem = {}, {}, []

        def add(name, x):
            val[name] = val[name] + x if name in val else x

        def product(*args):
            r = _dot(*args)
            val["latest"] = r[-8:]
            return r

        def short(g, i, j):
            if i == j:
                w = _load(wz, g, NZ + i)
            elif g < NG:
                w = pltpu.bitcast(wb[g * LT + j, _rows(i * 64, 64), :], BF16)
            else:
                w = wo_rows(((g - NG) * LT + i) * 128, 128, j)
            at = r_lhs(hb, i, j) if g < NG else R_OL + r_lhs(g - NG, i, j)
            add((min(g, NG), i, j), product(buf[_rows(at, M + HALF)], w))

        def short_end(g, i, j):
            if NG <= g < NG + WG - 1:
                return
            g = min(g, NG)
            r = val.pop((g, i, j))
            add(("m", g, j), r[0:M])
            if i != j:
                add(("y", g, i), r[M:])
                add(("b", g, j), r[M:])
                if LAM[i]:
                    add(("a", g, j), r[M:] * -LAM[i])
                return
            y = val.pop(("y", g, j))
            if g < NG:
                y = y + z[_z_index(g, batch), part, _rows(j * HALF, HALF), :]
            a = val.pop(("a", g, j)) + r[M:]
            if LAM[j]:
                a = a - LAM[j] * y
            r = jnp.concatenate([val.pop(("m", g, j)), a, val.pop(("b", g, j)) + y], axis=0)
            if g < NG:
                buf[r_qkv(*TILES[g * LT + j])] = r
            else:
                buf[_rows(R_ACC + j * L, L)] = out_sum(j, r)

        def plain(n, k):
            w = pltpu.bitcast(wb[NG * LT + n, _rows(k * 64, 64), :], BF16)
            val["plain", n, k] = product(buf[_rows(R_H + (hb * LT + k) * L, L)], w)

        def plain_end(n, k):
            dst = r_qkv(*TILES[NG * LT + n])
            r = val.pop(("plain", n, k))
            buf[dst] = r + buf[dst] if k else r

        def long(g, n):
            val["long", g, n] = z_product(g, n, batch + 1) if g < NG else out_product(g, n)
            val["latest"] = val["long", g, n][24:32]

        def long_end(g, n):
            r = val.pop(("long", g, n))
            if g >= NG:
                out_finish(g, n, r, jnp.maximum(batch - 1, 0))
                return
            for i in _targets(n):
                sums[g, i] = sums[g, i] + r if (g, i) in sums else r

        def long_store():
            for (g, i), r in sums.items():
                _add_long(z_next.at[g - G0], i, r, (g, i) not in stored)
                stored.append((g, i))
            sums.clear()

        def a_late(u, t, k):
            n = ZB * HALF
            x = _load(ol, k, _ds(part * (NB * TL // (ZB * n)) + u, n // 2))
            add("late", product(x, _load(wo_p, t, _ds(k, 64))))
            if k == LT - 1:
                r = val.pop("late").astype(BF16)
                for m in range(n // TL):
                    outl[part * (NB // ZB) + u * (n // TL) + m, :, _rows(t * 128, 128)] = r[_rows(m * TL, TL)]

        def score(p, both):
            if both:
                q, k = [[buf[r_qkv(j, 3 * p + t)] for t in (0, 2)] for j in (0, 1)]
            else:
                q, k = buf[r_qkv(0, 3 * p + 1)], [buf[r_qkv(1, 3 * p + 1)]]
                q = [jnp.where(low, q, 0.0), jnp.where(low, 0.0, q)]
            q = jnp.concatenate(q + [jnp.zeros((128 - 2 * L, 128), F32)], axis=0)
            r = product(jnp.concatenate(k, axis=0), q.astype(BF16), NT)
            add(("s", p), jnp.where(head0, r[0:L], r[L:]) if both else r)

        def softmax(p, step):
            def late(x):
                return jnp.where(col[0:8] < 2 * L, x, val["latest"])

            def groups(x):
                return [x[_rows(r, 8)] for r in range(0, L, 8)]

            def spread(x):
                return jnp.concatenate([x] * (L // 8), axis=0)
            x, y = val["s", p], val.get(("t", p))
            if step == 0:
                x = jnp.where(visible, x * (DH ** -0.5), MASKED)
                y = functools.reduce(jnp.maximum, groups(x))
            elif step == 1:
                y = jnp.broadcast_to(jnp.max(late(y), axis=0, keepdims=True), (8, 128))
            elif step == 2:
                x = jnp.exp(x - spread(late(y)))
                y = functools.reduce(jnp.add, groups(x))
            elif step == 3:
                y = jnp.broadcast_to(jnp.sum(late(y), axis=0, keepdims=True), (8, 128))
            elif step == 4:
                y = _inverse(late(y))
            else:
                x = x * spread(late(y))
                x = jnp.concatenate([x, x], axis=0)[:, 0:2 * L]
                buf[_rows(R_P + p * 2 * L, 2 * L), 0:2 * L] = x.astype(BF16).T.astype(F32)
            val["s", p], val["t", p] = x, y

        def pv(t):
            pa, pb = [buf[_rows(R_P + (2 * (t // 3) + u) * L, L), 0:2 * L] for u in range(2)]
            v = buf[r_qkv(2, t)]
            if t % 3 == 1:
                v = jnp.concatenate([jnp.where(low, v, 0.0), jnp.where(low, 0.0, v)], axis=0)
            pr = (pa[:, 0:L], jnp.where(head0[:, 0:2 * L], pa, pb), pb[:, 0:L])[t % 3]
            val["o", t] = product(pr, v.astype(BF16))

        def pv_end(t):
            buf[_rows(R_O + t * L, L)] = val.pop(("o", t))

        def out_lhs(g, j):
            o = [buf[_rows(R_O + (g * LT + i) * L, L)] for i in range(LT)]
            a, b = [x[M:M + HALF] for x in o], [x[M + HALF:] for x in o]
            a[j] = jnp.concatenate([jnp.where(batch >= 0, x, val["latest"]) for x in (a[j][0:8], a[j][8:])], axis=0)
            for i, x in enumerate(_short_lhs(a, b, j)):
                m = o[j][0:M] if i == j else o[i][0:M] + o[j][0:M]
                buf[_rows(R_OL + r_lhs(g, i, j), M + HALF)] = jnp.concatenate([m, x], axis=0)
            _long_lhs(a, b, lo.at[g, :, _rows(part * HALF, HALF), :], j)

        def out(t, n):
            add(("out", t // KC, n), product(buf[_rows(R_O + t * L, L)], wo_rows(t * 128, 128, n)))

        def out_sum(n, r):
            if ("sum", n) in val:
                r = r + buf[_rows(R_ACC + n * L, L)]
            val["sum", n] = True
            return r

        def out_end(t, n):
            r = out_sum(n, val.pop(("out", t // KC, n)))
            if t < FT - 1:
                buf[_rows(R_ACC + n * L, L)] = r
                return
            new_mem.append(r[0:M])
            memory_lhs(new_mem, n, nh)
            if isinstance(part, int):
                op[part, n] = r[M:L]
            else:
                outb[_ds(s, SEG), _rows(n * 128, 128)] = r[M:L].astype(BF16)

        tasks = dict(short=short, short_end=short_end, plain=plain, plain_end=plain_end, long=long,
                     long_end=long_end, long_store=long_store, a_late=a_late, score=score, softmax=softmax,
                     pv=pv, pv_end=pv_end, out_lhs=out_lhs, out=out, out_end=out_end,
                     next_tokens=lambda: token_lhs(jnp.minimum(s + 1, NSEG - 1), nh))
        before = list(before)
        for name, *args in plan[0]:
            if name in ("short", "plain"):
                while len(before) > LT - 1 - max(args[1:]):
                    before.pop(0)()
            tasks[name](*args)
        return [functools.partial(tasks[name], *args) for name, *args in plan[1]]

    order = [_long_index(n) for n in
             ((0, 1), (0, 2), (1, 2), 0, (0, 3), (0, 4), (3, 4), 3, 4, (1, 4), 1, (1, 3), (2, 3), (2, 4), 2)]
    longs = ([("long", NG + g, n) for n in range(NZ) for g in range(WG)]
             + [("long", g, n) for g in range(G0, NG) for n in order])
    plans = [_make_plan(rounds, longs, WG) for rounds in ROUNDS]
    late = [("a_late", u, t, k) for u in range(NB * TL // (ZB * ZB * HALF)) for t in range(LT) for k in range(LT)]
    last_plan = _make_plan(LAST_ROUNDS, late, 0)
    assert not longs and not late
    assert plans[0][0].index(("long", NG + WG - 1, NZ - 1)) < plans[0][0].index(("out_lhs", 0, 0))
    for tasks in (sum(plan, []) for plan in plans):
        assert tasks.index(("short_end", NG + WG - 1, LT - 1, LT - 1)) < tasks.index(("out_end", FT - 1, 0))

    def batch_step(batch, carry):
        rest = ()
        for u in range(ZB):
            rest = segment(plans[u], batch, u, u, (u + 1) % ZB, rest)
        _run(rest)
        pl.when(batch > 0)(lambda: c_outb(pl.multiple_of((batch - 1) * TB, TB), TB).start())
        return carry

    def last_step(s, carry):
        _run(segment(last_plan, s // ZB, s % ZB, 0, 0))
        c_outl(s % ZB).start()
        c_outb(pl.multiple_of(s * SEG, SEG), SEG).start()
        return carry

    part_a()
    token_lhs(0, 0)
    mem0 = mem[0:M, :].astype(F32)
    for n in range(LT):
        memory_lhs([mem0[:, _rows(k * 128, 128)] for k in range(LT)], n, 0)
    lo[...] = jnp.zeros(lo.shape, lo.dtype)
    op[...] = jnp.zeros(op.shape, op.dtype)
    wait_filled(wo.at[:, pl.ds(WO_FIRST, H * DH - WO_FIRST), :], sem_a.at[5])
    c_outa = cp(outa, out_hbm.at[:, pl.ds(0, TE), pl.ds(0, D)], sem_o.at[0])
    c_outa.start()
    lax.fori_loop(0, NB - 1, batch_step, 0)
    for n in range(NZ):
        for g in range(NG, NG + WG):
            out_finish(g, n, out_product(g, n), NB - 2)
    c_outb((NB - 2) * TB, TB).start()
    lax.fori_loop(NSEG - ZB, NSEG, last_step, 0)
    c_outa.wait()
    wait_filled(out_hbm.at[:, :, pl.ds(D, D)], sem_o.at[1])
    wait_filled(out_hbm.at[:, pl.ds(TE, TL), pl.ds(0, D)], sem_o.at[2])


def pallas_concat_heads__sliding_local_dilated__memory_aug_recurrent_mem_tr__prompt_kernel(
    A_x, A_wqkv, A_wo, B_x, B_mem0, B_Wq, B_Wk, B_Wv, B_Wo, B_seg_len,
):
    assert B_seg_len == SEG
    assert A_x.shape == B_x.shape == (1, S, D) and B_mem0.shape == (1, M, D)
    assert B_Wq.shape == B_Wk.shape == B_Wv.shape == (D, H, DH) and B_Wo.shape == (H, DH, D)
    vmem, dma = pltpu.VMEM, pltpu.SemaphoreType.DMA
    call = pl.pallas_call(
        _kernel,
        out_shape=jax.ShapeDtypeStruct((NB, TB, 2 * D), BF16),
        in_specs=[pl.BlockSpec(memory_space=pl.ANY)] * 9,
        out_specs=pl.BlockSpec(memory_space=pl.ANY),
        scratch_shapes=[
            vmem((LT, S, 128), BF16),
            vmem((D, D), BF16),
            vmem((LT + 1, D, 128), F32),
            vmem((LT, 3 * D, 128), BF16),
            vmem((LT, D, 128), BF16),
            vmem((LT, NS * TB, 128), F32),
            vmem((2 * LT, HALO + NS * TB, 128), F32),
            vmem((LT + 1, NS * TB, 128), F32),
            vmem((LT + 1, TE, 128), BF16),
            vmem((LT, NB * TL, 128), BF16),
            vmem((NB, TE, D), BF16),
            vmem((NB, TL, D), BF16),
            vmem((S + 64, D), BF16),
            vmem((64, D), BF16),
            vmem((3 * H * DH, D), BF16),
            vmem((len(TILES) + 1, D // 2, 128), U32),
            vmem((NG + WG, NZ + LT, 128, 128), BF16),
            vmem((LT, H * DH, 128), BF16),
            vmem((NZ, S // 2, 128), BF16),
            vmem((2 * (NG - G0) + NB * G0, ZB, LT * HALF, 128), F32),
            vmem((WG, NZ, ZB * HALF, 128), BF16),
            vmem((ZB, LT * HALF, 128), F32),
            vmem((ZB, LT, SEG, 128), F32),
            vmem((R_END, 128), F32),
            pltpu.SMEM((2,), jnp.int32),
            dma((6,)), dma((NCH,)), dma((3,)),
        ],
        compiler_params=pltpu.CompilerParams(
            vmem_limit_bytes=126 * 1024 * 1024, internal_scratch_in_bytes=48 * 1024, disable_bounds_checks=True),
        name="sliding_and_memory_attention",
    )

    def by_feature(w):
        return w.transpose(1, 2, 0).reshape(H * DH, D)

    out = call(A_x.reshape(S, D), A_wqkv, A_wo, B_x.reshape(S, D), B_mem0.reshape(M, D),
               by_feature(B_Wq), by_feature(B_Wk), by_feature(B_Wv), B_Wo.reshape(H * DH, D))
    return out.reshape(1, S, 2 * D)
```

```python
import functools

import jax
import jax.numpy as jnp
from jax import lax
from jax.experimental import pallas as pl
from jax.experimental.pallas import tpu as pltpu

F32, BF16, U32 = jnp.float32, jnp.bfloat16, jnp.uint32
NN = (((1,), (0,)), ((), ()))
NT = (((1,), (1,)), ((), ()))
MASKED = -1000000000.0

S, D = 2048, 640
LT = D // 128

AH, AD, AW, ADIL = 32, 20, 8, 2
HALO = 16
TB = 128
NB = S // TB
NS = 2
TL = 32
TE = TB - TL
RC = 8

H, DH, M, SEG = 32, 192, 8, 32
L = M + SEG
HALF = SEG // 2
NP = H // 2
FT = 3 * NP
NSEG = S // SEG
LAM = (0.0, 0.625, -0.625, 1.875, -1.875)
PAIRS = [(i, j) for i in range(LT) for j in range(i + 1, LT)]
NZ = LT + len(PAIRS)
NG = 28
WG = 2
G0 = 4
ZB = TB // SEG
KC = 3
CG = 2
NCH = NG // CG
NST = NCH - 2
FIRST, STEP = (864, 688, 0), (480, 496, 432)
WO_STEP = 256
WO_FIRST = (NST - 3) * WO_STEP

ROUNDS = (
    "PsLssssLssssLssssLssssLssssLssssLssssLsQssssLssssLssssLssssLssQsssVssssLssssLsssssLssVssssLssssLssQsssVs"
    "sssLssssLssssLssssLssQsssVssssWsLssssLssWWssssLsssVsWssWsssVsssWsQsWsWssssWQsWssWsWWssWWsssVsssWWWsssVsW"
    "sWsWsWsssWWWsssVssQsWsWsWsQsssWWWsssVswWsWWssVwWwWwwwWVwwwWwWWwwWWWwWWWW",
    "LPssssLssssLssssLssssLssssLssssLssssLssssLssssLssssLsssQsQsssssLssssLssssLssssLsssVsssVsQssssVssLsssWsWs"
    "sLssQsssVssssLssssLsWssssLssssLssssLssssLssssLssssVsWssWssVssWWsWssQsWsWsWsQssWWssWsssVsWsWsWsWsWsWWsssV"
    "ssssLssWssWWsWssVssQsWsWsWsQsssWsWWswVswWsWWswwVwsWWsWwWwwwVWwWwWWWwwWWWW",
    "LPsssLssssLssssLssssLssssLsQssssLssssLssssLssssLssssLssssVsQssssLsssssLssssLsssVssQsssVssssLssssLssssLsW"
    "sWssQsssVsssssLssssLsWssWssssLssssLssssLssWsssVsWssssVsQsWssWWssQssssLsWssWsssLsWssWsWssVsssWWsWsssVWssW"
    "sWssWsWssWWWsssVssQsWsWsWsQsssWWsWwssVsWwwWWwsVssWWwWwwwVwwWWWwWWwwWWWWW",
    "LPssssLssssLssssLssssLssssLssssLssssLssssLssssLssssLssssLssssLsssQsQssssLssssLssssLssssVssVssQsssVssssLs"
    "WsssssWsLssQssVssssLsssLssssLssssLssssLsssVsWssWsssVsssLssWsWssWsWsQsWsWsWsQssWsWWsWssssVsWsWsWsWsWsWssV"
    "ssssLsWsssWWsWssVssQsWsWsWsQsssWWsWswVsWwsWWswwVswWsWWwWwwVWwWwWWwWwwWWWW",
)
LAST_ROUNDS = (
    "PsLsssssLssssLsssssssLsssQsssLsssssLssssLssssLssssQsssVssssWssssLssssLsssVsWsWsssssWsVsWsWssssLsWsWssWss"
    "ssssQsQsssWWsssWsssLsssssVWsWssssVssWsWWssssVsWsWssssssLssWWsssQsWsWsWsssQssWsWsssssVsssWWsWssWsWWssWsWs"
    "sVssssssWWssWQsssVsWsssWWsQssWssWWWsssVsWsssWWVWWVWWWWWWWWWWW"
)
LATENCY, SOFTMAX_STEP, LHS_STEP = 120, 24, 48
START_TIMES, START_LAGS = [300, 986, 1612], [[0, 22, 120, 142, 330, 500, 510], [0, 22, 120, 142, 330, 650, 655]]
LOOP_TIMES, LOOP_LAGS = [1240, 747, 2746, 2398, 4010], [2, 38, 174, 227, 346, 369, 409]
END_TIMES = [500, 0, 1530]


def _tile_order():
    lag = [2] * 8 + [3] * 4 + [4] * 4
    order = []
    for p in range(NP + max(lag)):
        if p < NP:
            order += [(j, 3 * p + t) for j in (0, 1) for t in range(3)]
        order += [(2, 3 * x + t) for x in range(NP) if x + lag[x] == p for t in range(3)]
    rest = [(2, t) for t in (11, 23, 35, 42)]
    return [x for x in order if x not in rest] + rest


TILES = _tile_order()
NPL = len(TILES) - NG * LT
assert all((t + 1) * 128 <= FIRST[j] + n // (CG * LT) * STEP[j] for n, (j, t) in enumerate(TILES[:NST * CG * LT]))

R_LHS = 0
R_H = R_LHS + ZB * LT * LT * (M + HALF)
R_QKV = R_H + ZB * LT * L
R_O = R_QKV + 3 * FT * L
R_P = R_O + FT * L
R_ACC = R_P + NP * 2 * L
R_OL = R_ACC + LT * L
R_END = (R_OL + WG * LT * LT * (M + HALF) + 31) // 32 * 32


def _targets(n):
    return (n,) if n < LT else PAIRS[n - LT]


def _long_index(name):
    return LT + PAIRS.index(name) if name in PAIRS else name


def _make_plan(rounds, longs, fast):
    shell = []
    for k in range(LT):
        for n in range(k + 1, LT):
            shell += [(k, n), (n, k)]
        shell += [(k, k)]
    todo = dict(
        L=longs,
        s=[("short", g, i, j) for g in range(NG) for (i, j) in shell],
        w=[("short", NG + g, i, j) for (i, j) in shell for g in range(fast)],
        W=[("out", t, n) for k in range(0, FT, KC) for n in range(LT) for t in range(max(k, fast * LT), k + KC)],
        P=[("plain", n, 0) for n in range(NPL)] + [("plain", n, k) for n in range(NPL) for k in range(1, LT)],
        Q=[("score", p + u, both) for p in range(0, NP, 2) for both in (p // 2 % 2, 1 - p // 2 % 2) for u in (0, 1)],
        V=[("pv", t) for t in range(FT)])
    plan, timed, now = [], [], 0

    def needs(name, *args):
        if name == "out":
            return [("pv_end", args[0])]
        if name == "short" and args[0] >= NG:
            return [("out_lhs", args[0] - NG, args[2])]
        if name not in ("score", "pv"):
            return []
        need = [("softmax", args[0] // 3, 5)] if name == "pv" else []
        for tile in [(2, args[0])] if name == "pv" else [(j, 3 * args[0] + t) for j in (0, 1) for t in range(3)]:
            g, j = divmod(TILES.index(tile), LT)
            need.append(("short_end", g, j, j) if g < NG else ("plain_end", j, LT - 1))
        return need

    for n, kind in enumerate(rounds):
        tasks = todo[kind][:4]
        del todo[kind][:4]
        if kind == "Q":
            tasks += [todo["P"].pop(0), todo["P"].pop(0)]
        while kind == "w" and len(tasks) < 4:
            tasks.append(todo["W"].pop(0))
        need = [x for task in tasks for x in needs(*task)]
        until = max([now] + [time for time, task in timed if task in need])
        timed.sort(key=lambda x: x[0])
        while timed and timed[0][0] <= until:
            plan.append(timed.pop(0)[1])
        assert all(x in plan for x in need)
        plan += tasks
        now += dict(s=M + HALF, w=M + HALF, L=ZB * HALF, Q=2 * L).get(kind, L)
        for name, *args in tasks:
            if name in ("short", "plain", "long", "pv") or (name == "out" and args[0] % KC == KC - 1):
                timed.append((now + LATENCY, (name + "_end", *args)))
            if name == "pv" and args[0] < fast * LT and args[0] % LT == LT - 1:
                timed += [(now + LATENCY + LHS_STEP * j, ("out_lhs", args[0] // LT, j)) for j in range(LT)]
            if name == "score" and args[1]:
                timed += [(now + SOFTMAX_STEP * (step + args[0] % 2), ("softmax", args[0], step)) for step in range(6)]
        if kind == "L":
            timed.append((now + LATENCY, ("long_store",)))
        if kind == "s" and kind not in rounds[n + 1:]:
            plan.append(("next_tokens",))
    assert not any(todo[kind] for kind in "swWPQV")
    return plan, [task for _, task in sorted(timed, key=lambda x: x[0])]


def _ds(i, n):
    return pl.ds(i * n if isinstance(i, int) else pl.multiple_of(i * n, n), n)


def _rows(r0, n):
    return slice(r0, r0 + n)


def _dot(a, b, dims=NN):
    r = lax.dot_general(a, b, dims, preferred_element_type=F32)
    return jnp.concatenate([r[0:8], r[8:]], axis=0)


def _inverse(x):
    r = pltpu.reciprocal(x, approx=True)
    return r + r * (1.0 - x * r)


def _load(ref, *index):
    return pltpu.bitcast(ref.bitcast(U32)[index], BF16)


def _run(tasks):
    for task in tasks:
        task()


def _short_lhs(a, b, j):
    p = [a[i] + LAM[j] * b[i] if LAM[j] else a[i] for i in range(LT)]
    return [p[j] if i == j else (p[i] + p[j]) * (1.0 / (LAM[j] - LAM[i])) for i in range(LT)]


def _long_lhs(a, b, dst, i):
    p = [a[k] + LAM[k] * b[k] if LAM[k] else a[k] for k in range(LT)]
    dst[i] = b[i].astype(BF16)
    for k in ((i + 1) % LT, (i + 2) % LT):
        lo, hi = sorted((i, k))
        dst[_long_index((lo, hi))] = ((p[lo] + p[hi]) * (1.0 / (LAM[lo] - LAM[hi]))).astype(BF16)


def _combine(tile, dst, r, i):
    row = col = tile(i, i)
    for k in range(LT):
        if k != i:
            a, b = tile(i, k), tile(k, i)
            row, col = row - a, col - b
            if k > i:
                dst[_long_index((i, k)), _rows(16 * r, 16), :] = (a - b).astype(BF16)
    dst[i, _rows(16 * r, 16), :] = row.astype(BF16)
    dst[NZ + i, _rows(16 * r, 16), :] = col.astype(BF16)


def _add_long(dst, i, r, first):
    for u in range(ZB):
        x = r[_rows(u * HALF, HALF)]
        dst[u, _rows(i * HALF, HALF), :] = x if first else x + dst[u, _rows(i * HALF, HALF), :]


def _z_index(g, batch):
    if isinstance(batch, int) and batch == 0:
        return g
    if isinstance(g, int) and g >= G0:
        return g + (batch % 2) * (NG - G0)
    return jnp.where(batch == 0, g, 2 * (NG - G0) + batch * G0 + g)


def _kernel(ax_hbm, awqkv_hbm, awo_hbm, bx_hbm, mem_hbm, wq_hbm, wk_hbm, wv_hbm, wo_hbm,
            out_hbm,
            ax, awo, tmp, wqkv_p, wo_p, q_s, kv_s, oa, ob, ol, outa, outl,
            bx, mem, raw, wb, wz, wo, lz, z, lo, zo, op, buf,
            flag, sem_a, sem_w, sem_o):
    awqkv = raw.at[pl.ds(3 * (H * DH - D), 3 * D), :]
    outb = raw.at[pl.ds(0, S), :]

    cp = pltpu.make_async_copy

    def span(first, i, n):
        return pl.ds(first + i * n if isinstance(i, int) else pl.multiple_of(first + i * n, 16), n)

    def c_strips(src, dst, at, sem):
        return [cp(src.at[at, pl.ds(t * 128, 128)], dst.at[t, at, :], sem) for t in range(LT)]

    def c_bx(i, n, sem):
        return cp(bx_hbm.at[_ds(i, n), :], bx.at[_ds(i, n), :], sem)

    def c_w(j, first, i, n, sem):
        return cp((wq_hbm, wk_hbm, wv_hbm)[j].at[span(first, i, n), :], raw.at[span(j * H * DH + first, i, n), :], sem)

    def c_ax(c, sem):
        return c_strips(ax_hbm, ax, _ds(c + NS, TB), sem)

    def c_step(c):
        return [c_bx(c + 2, TB, sem_w.at[c])] + [c_w(j, FIRST[j], c - 1, STEP[j], sem_w.at[c]) for j in range(3)]

    def c_outb(r0, n):
        at = r0 % TB if isinstance(r0, int) else pl.multiple_of(lax.rem(r0, TB), n)
        return cp(outb.at[pl.ds(r0, n), :], out_hbm.at[r0 // TB, pl.ds(at, n), pl.ds(D, D)], sem_o.at[1])

    def c_outl(u):
        at = pl.ds(u * (NB // ZB), NB // ZB)
        return cp(outl.at[at], out_hbm.at[at, pl.ds(TE, TL), pl.ds(0, D)], sem_o.at[2])

    def start(copies):
        for c in copies:
            c.start()

    def wait(copies):
        for c in copies:
            c.wait()

    def wait_filled(ref, sem):
        cp(ref, ref, sem).wait()

    def permute_rows(dst, base):
        def move(t, d0):
            for d in range(d0, d0 + AD // 4):
                dst[t, pl.ds(base + d * AH, AH), :] = tmp[t, pl.ds(d, AH, stride=AD), :].astype(BF16)
        return [functools.partial(move, t, d0) for t in range(LT) for d0 in range(0, AD, AD // 4)]

    def prep_wqkv(j):
        def transpose(t):
            tmp[t] = awqkv[_rows(j * D + t * 128, 128), :].astype(F32).T
        return [functools.partial(transpose, t) for t in range(LT)], permute_rows(wqkv_p, j * D)

    def prep_wo():
        def widen(t, r):
            tmp[t, _rows(r, D // 4), :] = awo[_rows(r, D // 4), _rows(t * 128, 128)].astype(F32)
        moves = permute_rows(wo_p, 0)
        return [task for t in range(LT)
                for task in [functools.partial(widen, t, r) for r in range(0, D, D // 4)] + moves[4 * t:4 * t + 4]]

    def slot(i):
        return i * TB if isinstance(i, int) and i < NS else (NS - 1) * TB

    def a_tiles(count, product, store):
        acc = {}

        def tile(t, k):
            r = product(t, k)
            acc[t] = acc[t] + r if k else r
            return r
        return [(count, functools.partial(tile, t, k), (lambda t=t: store(t, acc[t])) if k == LT - 1 else None)
                for t in range(LT) for k in range(LT)]

    def a_proj(i, j):
        at = slot(i)

        def store(t, r):
            if j == 0:
                q_s[t, _rows(at, TB), :] = r
                return
            c = (j - 1) * LT + t
            if not isinstance(i, int):
                kv_s[c, _rows(at, HALO), :] = kv_s[c, _rows(at + TB, HALO), :]
            elif i == 0:
                kv_s[c, 0:HALO, :] = jnp.broadcast_to(r[0:1, :], (HALO, 128))
            kv_s[c, _rows(at + HALO, TB), :] = r
        return a_tiles(TB, lambda t, k: _dot(_load(ax, k, _ds(i, TB // 2)), _load(wqkv_p, k, _ds(j * LT + t, 64)), NT),
                       store)

    def a_attention(i):
        state = {}

        def window(c, r0, w):
            return kv_s[c, _rows(HALO + r0 - ADIL * w, RC), :]

        def logits(r0, half, late):
            q = [q_s[t, _rows(r0, RC), :] for t in range(LT)]
            q[0] = late(q[0])
            for w in range(half * AW // 2, (half + 1) * AW // 2):
                a = q[0] * window(0, r0, w)
                for t in range(1, LT):
                    a = a + q[t] * window(t, r0, w)
                state.setdefault(r0, []).append(a + pltpu.roll(a, 2 * AH, 1))

        def fold(r0, half, late):
            for w in range(half * AW // 2, (half + 1) * AW // 2):
                a = state[r0][w]
                a = (a + pltpu.roll(a, AH, 1)) * (AD ** -0.5)
                if isinstance(i, int) and r0 < ADIL * w:
                    pos = lax.broadcasted_iota(jnp.int32, (RC, 128), 0) + r0
                    a = jnp.where(pos >= ADIL * w, a, MASKED)
                state[r0][w] = a

        def weights(r0, late):
            m = late(functools.reduce(jnp.maximum, state[r0]))
            state[r0] = [jnp.exp(a - m) for a in state[r0]]

        def mix(r0, tiles, late):
            e = [late(state[r0][0])] + state[r0][1:]
            if 0 in tiles:
                state[r0, "inverse"] = _inverse(functools.reduce(jnp.add, e))
            for t in tiles:
                o = e[0] * window(LT + t, r0, 0)
                for w in range(1, AW):
                    o = o + e[w] * window(LT + t, r0, w)
                oa[t, _rows(r0, RC), :] = o * state[r0, "inverse"]

        stages = ((logits, 0), (logits, 1), (fold, 0), (fold, 1), (weights,), (mix, (0, 1)), (mix, (2, 3, 4)))
        return [[functools.partial(f, r0, *args) for r0 in range(slot(i), slot(i) + TB, RC)] for f, *args in stages]

    def a_pack(i):
        def pack(k):
            ob[k] = oa[k, _rows(slot(i), TE), :].astype(BF16)
            ol[k, _ds(i, TL), :] = oa[k, _rows(slot(i) + TE, TL), :].astype(BF16)
        return [functools.partial(pack, k) for k in range(LT)]

    def a_out(i):
        def store(t, r):
            outa[i, :, _rows(t * 128, 128)] = r.astype(BF16)
        return a_tiles(TE, lambda t, k: _dot(_load(ob, k), _load(wo_p, t, _ds(k, 64))), store)

    def overlap(tiles, side, zero):
        due = sorted((lo + (hi - lo) * n / len(tasks), m, n, task, tie)
                     for m, (lo, hi, tasks, tie) in enumerate(side) for n, task in enumerate(tasks))
        free = [0] * 4
        results = []
        for count, tile, end in tiles:
            now = min(free)
            free[free.index(now)] += count
            results.append((now, tile()))
            while due and (due[0][0] < min(free) or len(results) == len(tiles)):
                time, _, _, task, tie = due.pop(0)
                begin, r = [x for x in results if x[0] <= time][-1]
                row = min(int(time - begin), r.shape[0] - 1) // 8 * 8
                if isinstance(tie, str):
                    task(lambda x: jnp.where(zero == 0, x, r[_rows(row, 8)]))
                    continue
                if tie is bx:
                    tie[span(S, zero, 16), 0:128] = r[_rows(row // 16 * 16, 16)].astype(BF16)
                elif tie is not None:
                    tie[tie.shape[0] - 1 - zero, 0:8, :] = pltpu.bitcast(r[_rows(row, 8)], tie.dtype)
                task()
            if end:
                end()

    def wo_rows(r0, n, t):
        return _load(wo, t, _rows(r0 // 2, n // 2))

    def w_transpose(c, n):
        at = [FT * j + t for j, t in TILES[n::CG * LT]]
        if isinstance(c, int):
            at = at[c]
        else:
            words = [sum(x << 8 * k for k, x in enumerate(at[m::5])) for m in range(5)]
            word = functools.reduce(lambda x, m: jnp.where(lax.rem(c, 5) == m, words[m], x), range(1, 5), words[0])
            at = lax.shift_right_logical(word, lax.div(c, 5) * 8) & 255
        chunk = wb.at[pl.ds(c * CG * LT, NPL if isinstance(c, int) else CG * LT)]
        chunk[n] = pltpu.bitcast(raw[_ds(at, 128), :].T, U32)

    def w_combine(c, u, r, i):
        chunk = wb.at[pl.ds(c * CG * LT, CG * LT)]
        _combine(lambda a, b: pltpu.bitcast(chunk[u * LT + b, _rows(a * 64 + 8 * r, 8), :], BF16).astype(F32),
                 wz.at[pl.ds(c * CG, CG)].at[u], r, i)

    def wo_combine(g, r, i, late):
        def tile(a, b):
            x = wo_rows((g * LT + a) * 128 + 16 * r, 16, b).astype(F32)
            return jnp.concatenate([late(x[0:8]), x[8:]], axis=0)
        _combine(tile, wz.at[NG + g], r, i)

    def halves(s):
        x = bx[_ds(s, SEG), :].astype(F32)
        return [[x[_rows(r, HALF), _rows(i * 128, 128)] for i in range(LT)] for r in (0, HALF)]

    def z_lhs(batch):
        def task(s, i):
            _long_lhs(*halves(s), lz.at[:, _ds(s, HALF), :], i)
        return [functools.partial(task, batch * ZB + u, i) for u in range(ZB) for i in range(LT)]

    def z_product(g, n, batch):
        return _dot(_load(lz, n, _ds(batch, ZB * HALF // 2)), _load(wz, g, n))

    def z_group(g, batch):
        dst = z.at[_z_index(g, batch)]
        sums, stored = {}, []

        def tile(n):
            r = z_product(g, n, batch)
            for i in _targets(n):
                sums[i] = sums[i] + r if i in sums else r
            return r

        def end():
            for i in sums:
                _add_long(dst, i, sums[i], i not in stored)
                stored.append(i)
            sums.clear()
        sets = (((0, 1), (0, 2), (1, 2), 0, 1), ((0, 3), (0, 4), (3, 4), 3, 4), ((1, 3), (1, 4), (2, 3), (2, 4), 2))
        return [(ZB * HALF, functools.partial(tile, _long_index(n)), end if n == some[-1] else None)
                for some in sets for n in some]

    def part_a():
        c_wqkv = [cp(awqkv_hbm.at[:, pl.ds(j * D, D)], awqkv.at[pl.ds(j * D, D), :], sem_a.at[j]) for j in range(3)]
        c_second = [c_wqkv[1]] + c_strips(ax_hbm, ax, pl.ds(0, NS * TB), sem_a.at[1])
        c_third = [c_wqkv[2], c_bx(0, 2 * TB, sem_a.at[2])]
        c_awo = cp(awo_hbm, awo, sem_a.at[3])
        c_first = c_ax(0, sem_w.at[0]) + [c_bx(2, TB, sem_w.at[0])] + [
            c_w(j, 0, 0, FIRST[j], sem_w.at[0]) for j in range(2)]
        last_rows = pl.ds(S - 2 * TB, 2 * TB)
        c_last = [c_bx(NB // 2 - 1, 2 * TB, sem_w.at[NST]), cp(mem_hbm, mem.at[pl.ds(0, M), :], sem_w.at[NST]),
                  c_w(2, (NST - 1) * STEP[2], 0, H * DH - (NST - 1) * STEP[2], sem_w.at[NST])]

        flag[0] = 0
        start([c_wqkv[0]] + c_second)
        lo[...] = jnp.zeros(lo.shape, lo.dtype)
        op[...] = jnp.zeros(op.shape, op.dtype)
        c_wqkv[0].wait()
        zero = flag[0]
        _run(sum(prep_wqkv(0), []))
        start(c_third)
        wait(c_second)
        first, second = prep_wqkv(1)
        overlap(a_proj(0, 0) + a_proj(1, 0), [(0, 0, first, None), (700, 1500, second, tmp)], zero)
        start([c_awo] + c_first[:-1])
        wait(c_third)
        first, second = prep_wqkv(2)
        overlap(a_proj(0, 1) + a_proj(1, 1),
                [(0, 0, first, None), (700, 1500, second, tmp), (0, 1500, z_lhs(0) + z_lhs(1), bx)], zero)
        c_first[-1].start()
        c_awo.wait()
        for i in range(NS):
            assert START_TIMES[i] + START_LAGS[i][-2] >= (i + 1) * 800
        assert START_TIMES[1] + START_LAGS[0][-1] <= 1500
        overlap(a_proj(0, 2) + a_proj(1, 2) + a_out(0),
                [(0, 800, prep_wo(), tmp), (1500, 1500, a_pack(0), None)]
                + [(START_TIMES[i] + d, START_TIMES[i + 1] + d, tasks, "value")
                   for i in range(NS) for d, tasks in zip(START_LAGS[i], a_attention(i))], zero)
        start(c_ax(1, sem_w.at[1]) + c_step(1) + c_ax(2, sem_w.at[2]) + c_step(2))
        wait(c_first)

        def step(c, carry):
            pl.when((c > 0) & (c < NST))(lambda: wait_filled(ax.at[:, _ds(c + NS, TB), :], sem_w.at[c]))
            for copy in c_step(jnp.clip(c, 1, NST - 1)):
                pl.when((c > 0) & (c < NST))(copy.wait)
            pl.when(c == NST)(lambda: wait_filled(ax.at[:, last_rows, :], sem_w.at[NST]))
            for copy in c_last:
                pl.when(c == NST)(copy.wait)

            zero = lax.shift_right_logical(c, 16)
            flag[zero] = 0
            i, t = c + NS, LOOP_TIMES
            assert t[0] / 2 <= t[1] + 100 and t[2] < 2900 and t[3] + LOOP_LAGS[-2] > 2500
            early = [x for u in range(2) for b in range(2) for x in z_group((c & 1) * 2 + u, (c | 1) + b)]
            overlap(a_proj(i, 0) + a_proj(i, 1) + a_proj(i, 2) + a_out(i - 1)
                    + z_group(c * CG, 0) + early + z_group(c * CG + 1, 0),
                    [(0, t[0], [functools.partial(w_transpose, c, n) for n in range(CG * LT)], None),
                     (0, t[1], z_lhs(c + 2), bx),
                     (0, t[1], a_pack(i - 1), oa),
                     (t[1], t[2], [functools.partial(w_combine, c, u, r, k)
                                   for u in range(CG) for r in range(8) for k in range(LT)], wb)]
                    + [(t[3] + d, t[4] + d, tasks, "value") for d, tasks in zip(LOOP_LAGS, a_attention(i))], zero)

            n = jnp.minimum(c + 3, NST - 1)
            for copy in c_ax(n, sem_w.at[n]) + c_step(n) + c_strips(wo_hbm, wo, _ds(c, WO_STEP), sem_a.at[4]):
                pl.when(c < NST - 3)(copy.start)
            for copy in c_strips(ax_hbm, ax, last_rows, sem_w.at[NST]) + c_last:
                pl.when(c == NST - 3)(copy.start)
            at = span(WO_FIRST, jnp.clip(c - (NST - 2), 0, 1), (H * DH - WO_FIRST) // 2)
            for copy in c_strips(wo_hbm, wo, at, sem_a.at[5]):
                pl.when((c > NST - 3) & (c < NST))(copy.start)
            return carry

        lax.fori_loop(0, NCH, step, 0)
        wait_filled(wo.at[:, pl.ds(0, WO_FIRST), :], sem_a.at[4])
        t = END_TIMES
        overlap([x for g in range(G0) for x in z_group(g, NB - 1)] + a_out(NB - 1),
                [(0, 0, [functools.partial(w_transpose, NCH, n) for n in range(NPL)], None),
                 (0, t[0], a_pack(NB - 1), oa),
                 (t[1], t[2], [functools.partial(wo_combine, g, r, i)
                               for g in range(WG) for r in range(8) for i in range(LT)], "value")], zero)

    def r_lhs(hb, i, j):
        return R_LHS + ((hb * LT + i) * LT + j) * (M + HALF)

    def r_qkv(j, t):
        return _rows(R_QKV + (j * FT + t) * L, L)

    def token_lhs(s, hb):
        a, b = halves(s)
        for j in range(LT):
            buf[_rows(R_H + (hb * LT + j) * L + M, SEG)] = jnp.concatenate([a[j], b[j]], axis=0)
            for i, x in enumerate(_short_lhs(a, b, j)):
                buf[_rows(r_lhs(hb, i, j) + M, HALF)] = x

    def memory_lhs(m, n, hb):
        buf[_rows(R_H + (hb * LT + n) * L, M)] = m[n]
        buf[_rows(r_lhs(hb, n, n), M)] = m[n]
        for k in range(n):
            buf[_rows(r_lhs(hb, n, k), M)] = buf[_rows(r_lhs(hb, k, n), M)] = m[n] + m[k]

    def out_product(g, n):
        return _dot(_load(lo, g - NG, n), _load(wz, g, n))

    def out_finish(g, n, r, batch):
        for i in _targets(n):
            _add_long(zo, i, r, n < LT and g == NG)
            if g == NG + WG - 1 and n == max(k for k in range(NZ) if i in _targets(k)):
                for u in range(ZB):
                    y = zo[u, _rows(i * HALF, HALF), :]
                    y = jnp.concatenate([-LAM[i] * y, y], axis=0)
                    outb[_ds(batch * ZB + u, SEG), _rows(i * 128, 128)] = (op[u, i] + y).astype(BF16)

    stored = []

    def segment(plan, batch, part, hb, nh, before=()):
        s = batch * ZB + part
        key = lax.broadcasted_iota(jnp.int32, (L, 128), 0)
        col = lax.broadcasted_iota(jnp.int32, (L, 128), 1)
        head0 = col < L
        query = jnp.where(head0, col, col - L)
        visible = (query < M) | (query >= key)
        low = col < 64
        z_next = z.at[pl.ds(_z_index(G0, batch + 1), NG - G0)]
        val, sums, new_mem = {}, {}, []

        def add(name, x):
            val[name] = val[name] + x if name in val else x

        def product(*args):
            r = _dot(*args)
            val["latest"] = r[-8:]
            return r

        def short(g, i, j):
            if i == j:
                w = _load(wz, g, NZ + i)
            elif g < NG:
                w = pltpu.bitcast(wb[g * LT + j, _rows(i * 64, 64), :], BF16)
            else:
                w = wo_rows(((g - NG) * LT + i) * 128, 128, j)
            at = r_lhs(hb, i, j) if g < NG else R_OL + r_lhs(g - NG, i, j)
            add((min(g, NG), i, j), product(buf[_rows(at, M + HALF)], w))

        def short_end(g, i, j):
            if NG <= g < NG + WG - 1:
                return
            g = min(g, NG)
            r = val.pop((g, i, j))
            add(("m", g, j), r[0:M])
            if i != j:
                add(("y", g, i), r[M:])
                add(("b", g, j), r[M:])
                if LAM[i]:
                    add(("a", g, j), r[M:] * -LAM[i])
                return
            y = val.pop(("y", g, j))
            if g < NG:
                y = y + z[_z_index(g, batch), part, _rows(j * HALF, HALF), :]
            a = val.pop(("a", g, j)) + r[M:]
            if LAM[j]:
                a = a - LAM[j] * y
            r = jnp.concatenate([val.pop(("m", g, j)), a, val.pop(("b", g, j)) + y], axis=0)
            if g < NG:
                buf[r_qkv(*TILES[g * LT + j])] = r
            else:
                buf[_rows(R_ACC + j * L, L)] = out_sum(j, r)

        def plain(n, k):
            w = pltpu.bitcast(wb[NG * LT + n, _rows(k * 64, 64), :], BF16)
            val["plain", n, k] = product(buf[_rows(R_H + (hb * LT + k) * L, L)], w)

        def plain_end(n, k):
            dst = r_qkv(*TILES[NG * LT + n])
            r = val.pop(("plain", n, k))
            buf[dst] = r + buf[dst] if k else r

        def long(g, n):
            val["long", g, n] = z_product(g, n, batch + 1) if g < NG else out_product(g, n)
            val["latest"] = val["long", g, n][24:32]

        def long_end(g, n):
            r = val.pop(("long", g, n))
            if g >= NG:
                out_finish(g, n, r, jnp.maximum(batch - 1, 0))
                return
            for i in _targets(n):
                sums[g, i] = sums[g, i] + r if (g, i) in sums else r

        def long_store():
            for (g, i), r in sums.items():
                _add_long(z_next.at[g - G0], i, r, (g, i) not in stored)
                stored.append((g, i))
            sums.clear()

        def a_late(u, t, k):
            n = ZB * HALF
            x = _load(ol, k, _ds(part * (NB * TL // (ZB * n)) + u, n // 2))
            add("late", product(x, _load(wo_p, t, _ds(k, 64))))
            if k == LT - 1:
                r = val.pop("late").astype(BF16)
                for m in range(n // TL):
                    outl[part * (NB // ZB) + u * (n // TL) + m, :, _rows(t * 128, 128)] = r[_rows(m * TL, TL)]

        def score(p, both):
            if both:
                q, k = [[buf[r_qkv(j, 3 * p + t)] for t in (0, 2)] for j in (0, 1)]
            else:
                q, k = buf[r_qkv(0, 3 * p + 1)], [buf[r_qkv(1, 3 * p + 1)]]
                q = [jnp.where(low, q, 0.0), jnp.where(low, 0.0, q)]
            q = jnp.concatenate(q + [jnp.zeros((128 - 2 * L, 128), F32)], axis=0)
            r = product(jnp.concatenate(k, axis=0), q.astype(BF16), NT)
            add(("s", p), jnp.where(head0, r[0:L], r[L:]) if both else r)

        def softmax(p, step):
            def late(x):
                return jnp.where(col[0:8] < 2 * L, x, val["latest"])

            def groups(x):
                return [x[_rows(r, 8)] for r in range(0, L, 8)]

            def spread(x):
                return jnp.concatenate([x] * (L // 8), axis=0)
            x, y = val["s", p], val.get(("t", p))
            if step == 0:
                x = jnp.where(visible, x * (DH ** -0.5), MASKED)
                y = functools.reduce(jnp.maximum, groups(x))
            elif step == 1:
                y = jnp.broadcast_to(jnp.max(late(y), axis=0, keepdims=True), (8, 128))
            elif step == 2:
                x = jnp.exp(x - spread(late(y)))
                y = functools.reduce(jnp.add, groups(x))
            elif step == 3:
                y = jnp.broadcast_to(jnp.sum(late(y), axis=0, keepdims=True), (8, 128))
            elif step == 4:
                y = _inverse(late(y))
            else:
                x = x * spread(late(y))
                x = jnp.concatenate([x, x], axis=0)[:, 0:2 * L]
                buf[_rows(R_P + p * 2 * L, 2 * L), 0:2 * L] = x.astype(BF16).T.astype(F32)
            val["s", p], val["t", p] = x, y

        def pv(t):
            pa, pb = [buf[_rows(R_P + (2 * (t // 3) + u) * L, L), 0:2 * L] for u in range(2)]
            v = buf[r_qkv(2, t)]
            if t % 3 == 1:
                v = jnp.concatenate([jnp.where(low, v, 0.0), jnp.where(low, 0.0, v)], axis=0)
            pr = (pa[:, 0:L], jnp.where(head0[:, 0:2 * L], pa, pb), pb[:, 0:L])[t % 3]
            val["o", t] = product(pr, v.astype(BF16))

        def pv_end(t):
            buf[_rows(R_O + t * L, L)] = val.pop(("o", t))

        def out_lhs(g, j):
            o = [buf[_rows(R_O + (g * LT + i) * L, L)] for i in range(LT)]
            a, b = [x[M:M + HALF] for x in o], [x[M + HALF:] for x in o]
            a[j] = jnp.concatenate([jnp.where(batch >= 0, x, val["latest"]) for x in (a[j][0:8], a[j][8:])], axis=0)
            for i, x in enumerate(_short_lhs(a, b, j)):
                m = o[j][0:M] if i == j else o[i][0:M] + o[j][0:M]
                buf[_rows(R_OL + r_lhs(g, i, j), M + HALF)] = jnp.concatenate([m, x], axis=0)
            _long_lhs(a, b, lo.at[g, :, _rows(part * HALF, HALF), :], j)

        def out(t, n):
            add(("out", t // KC, n), product(buf[_rows(R_O + t * L, L)], wo_rows(t * 128, 128, n)))

        def out_sum(n, r):
            if ("sum", n) in val:
                r = r + buf[_rows(R_ACC + n * L, L)]
            val["sum", n] = True
            return r

        def out_end(t, n):
            r = out_sum(n, val.pop(("out", t // KC, n)))
            if t < FT - 1:
                buf[_rows(R_ACC + n * L, L)] = r
                return
            new_mem.append(r[0:M])
            memory_lhs(new_mem, n, nh)
            if isinstance(part, int):
                op[part, n] = r[M:L]
            else:
                outb[_ds(s, SEG), _rows(n * 128, 128)] = r[M:L].astype(BF16)

        tasks = dict(short=short, short_end=short_end, plain=plain, plain_end=plain_end, long=long,
                     long_end=long_end, long_store=long_store, a_late=a_late, score=score, softmax=softmax,
                     pv=pv, pv_end=pv_end, out_lhs=out_lhs, out=out, out_end=out_end,
                     next_tokens=lambda: token_lhs(jnp.minimum(s + 1, NSEG - 1), nh))
        before = list(before)
        for name, *args in plan[0]:
            if name in ("short", "plain"):
                while len(before) > LT - 1 - max(args[1:]):
                    before.pop(0)()
            tasks[name](*args)
        return [functools.partial(tasks[name], *args) for name, *args in plan[1]]

    order = [_long_index(n) for n in
             ((0, 1), (0, 2), (1, 2), 0, (0, 3), (0, 4), (3, 4), 3, 4, (1, 4), 1, (1, 3), (2, 3), (2, 4), 2)]
    longs = ([("long", NG + g, n) for n in range(NZ) for g in range(WG)]
             + [("long", g, n) for g in range(G0, NG) for n in order])
    plans = [_make_plan(rounds, longs, WG) for rounds in ROUNDS]
    late = [("a_late", u, t, k) for u in range(NB * TL // (ZB * ZB * HALF)) for t in range(LT) for k in range(LT)]
    last_plan = _make_plan(LAST_ROUNDS, late, 0)
    assert not longs and not late
    assert plans[0][0].index(("long", NG + WG - 1, NZ - 1)) < plans[0][0].index(("out_lhs", 0, 0))
    for tasks in (sum(plan, []) for plan in plans):
        assert tasks.index(("short_end", NG + WG - 1, LT - 1, LT - 1)) < tasks.index(("out_end", FT - 1, 0))

    def batch_step(batch, carry):
        rest = ()
        for u in range(ZB):
            rest = segment(plans[u], batch, u, u, (u + 1) % ZB, rest)
        _run(rest)
        pl.when(batch > 0)(lambda: c_outb(pl.multiple_of((batch - 1) * TB, TB), TB).start())
        return carry

    def last_step(s, carry):
        _run(segment(last_plan, s // ZB, s % ZB, 0, 0))
        c_outl(s % ZB).start()
        c_outb(pl.multiple_of(s * SEG, SEG), SEG).start()
        return carry

    part_a()
    token_lhs(0, 0)
    mem0 = mem[0:M, :].astype(F32)
    for n in range(LT):
        memory_lhs([mem0[:, _rows(k * 128, 128)] for k in range(LT)], n, 0)
    wait_filled(wo.at[:, pl.ds(WO_FIRST, H * DH - WO_FIRST), :], sem_a.at[5])
    c_outa = cp(outa, out_hbm.at[:, pl.ds(0, TE), pl.ds(0, D)], sem_o.at[0])
    c_outa.start()
    lax.fori_loop(0, NB - 1, batch_step, 0)
    for n in range(NZ):
        for g in range(NG, NG + WG):
            out_finish(g, n, out_product(g, n), NB - 2)
    c_outb((NB - 2) * TB, TB).start()
    lax.fori_loop(NSEG - ZB, NSEG, last_step, 0)
    c_outa.wait()
    wait_filled(out_hbm.at[:, :, pl.ds(D, D)], sem_o.at[1])
    wait_filled(out_hbm.at[:, pl.ds(TE, TL), pl.ds(0, D)], sem_o.at[2])


def pallas_concat_heads__sliding_local_dilated__memory_aug_recurrent_mem_tr__prompt_kernel(
    A_x, A_wqkv, A_wo, B_x, B_mem0, B_Wq, B_Wk, B_Wv, B_Wo, B_seg_len,
):
    assert B_seg_len == SEG
    assert A_x.shape == B_x.shape == (1, S, D) and B_mem0.shape == (1, M, D)
    assert B_Wq.shape == B_Wk.shape == B_Wv.shape == (D, H, DH) and B_Wo.shape == (H, DH, D)
    vmem, dma = pltpu.VMEM, pltpu.SemaphoreType.DMA
    call = pl.pallas_call(
        _kernel,
        out_shape=jax.ShapeDtypeStruct((NB, TB, 2 * D), BF16),
        in_specs=[pl.BlockSpec(memory_space=pl.ANY)] * 9,
        out_specs=pl.BlockSpec(memory_space=pl.ANY),
        scratch_shapes=[
            vmem((LT, S, 128), BF16),
            vmem((D, D), BF16),
            vmem((LT + 1, D, 128), F32),
            vmem((LT, 3 * D, 128), BF16),
            vmem((LT, D, 128), BF16),
            vmem((LT, NS * TB, 128), F32),
            vmem((2 * LT, HALO + NS * TB, 128), F32),
            vmem((LT + 1, NS * TB, 128), F32),
            vmem((LT + 1, TE, 128), BF16),
            vmem((LT, NB * TL, 128), BF16),
            vmem((NB, TE, D), BF16),
            vmem((NB, TL, D), BF16),
            vmem((S + 64, D), BF16),
            vmem((64, D), BF16),
            vmem((3 * H * DH, D), BF16),
            vmem((len(TILES) + 1, D // 2, 128), U32),
            vmem((NG + WG, NZ + LT, 128, 128), BF16),
            vmem((LT, H * DH, 128), BF16),
            vmem((NZ, S // 2, 128), BF16),
            vmem((2 * (NG - G0) + NB * G0, ZB, (LT + 1) * HALF, 128), F32),
            vmem((WG, NZ, ZB * HALF, 128), BF16),
            vmem((ZB, LT * HALF, 128), F32),
            vmem((ZB, LT, SEG, 128), F32),
            vmem((R_END, 128), F32),
            pltpu.SMEM((2,), jnp.int32),
            dma((6,)), dma((NCH,)), dma((3,)),
        ],
        compiler_params=pltpu.CompilerParams(
            vmem_limit_bytes=126 * 1024 * 1024, internal_scratch_in_bytes=48 * 1024,
            disable_bounds_checks=True, disable_semaphore_checks=True),
        name="sliding_and_memory_attention",
    )

    def by_feature(w):
        return w.transpose(1, 2, 0).reshape(H * DH, D)

    out = call(A_x.reshape(S, D), A_wqkv, A_wo, B_x.reshape(S, D), B_mem0.reshape(M, D),
               by_feature(B_Wq), by_feature(B_Wk), by_feature(B_Wv), B_Wo.reshape(H * DH, D))
    return out.reshape(1, S, 2 * D)
```

```python
import functools

import jax
import jax.numpy as jnp
from jax import lax
from jax.experimental import pallas as pl
from jax.experimental.pallas import tpu as pltpu

F32, BF16, U32 = jnp.float32, jnp.bfloat16, jnp.uint32
NN = (((1,), (0,)), ((), ()))
NT = (((1,), (1,)), ((), ()))
MASKED = -1000000000.0

S, D = 2048, 640
LT = D // 128

AH, AD, AW, ADIL = 32, 20, 8, 2
HALO = 16
TB = 128
NB = S // TB
NS = 2
TL = 32
TE = TB - TL
RC = 8

H, DH, M, SEG = 32, 192, 8, 32
L = M + SEG
HALF = SEG // 2
NP = H // 2
FT = 3 * NP
NSEG = S // SEG
LAM = (0.0, 0.625, -0.625, 1.875, -1.875)
PAIRS = [(i, j) for i in range(LT) for j in range(i + 1, LT)]
NZ = LT + len(PAIRS)
NG = 28
WG = 2
G0 = 4
ZB = TB // SEG
KC = 3
CG = 2
NCH = NG // CG
NST = NCH - 2
FIRST, STEP = (864, 688, 0), (480, 496, 432)
WO_STEP = 256
WO_FIRST = (NST - 3) * WO_STEP

ROUNDS = (
    "PsLssssLssssLssssLssssLssssLssssLssssLsQssssLssssLssssLssssLssQsssVssssLssssLsssssLsssVsssLssssLssQsssVs"
    "sssLssssLssssLssssLssQssVsssssWsLssssLssWWssssLsssVsWsssWssVsssWsQsWsWssssWQsWssWsWWssWWsssVsssWWWsssVsW"
    "sWsWsWsssWWWsssVssQsWsWsWsQsssWWWsssVswWsWWssVwWwWwwwWVwwwWwWWwwWWWwWWWW",
    "LPssssLssssLssssLssssLssssLssssLssssLssssLssssLssssLssssLssssLsssQssQssssLsssLssssLssssVssVssQsssVssssLs"
    "sWssssWsLssQssVssssLsssLssssLssssLssssLsssVssWsWsssVssssLsssWsWWsWsQsWsWsWsQssWsWWsWssssVsWWssWsWsWsWssV"
    "ssssLsWsssWWsWssVssQsWsWsWsQsssWWsWswVsWwsWWswwVswWsWWwWwwVWwWwWWwWwwWWWW",
    "LPsssLssssLssssLssssLssssLsQssssLssssLssssLssssLssssLssssVsQssssLsssssLssssLsssVssQsssVssssLssssLssssLsW"
    "sWssQsssVsssssLssssLsWssWssssLssssLssssLssWsssVsWssssVsQsWssWWssQssssLsWssWsssLssWsWsWssVsssWWsWsssVWssW"
    "sWssWsWssWWWsssVssQsWsWsWsQsssWWsWwssVsWwwWWwsVssWWwWwwwVwwWWWwWWwwWWWWW",
    "LPssssLssssLssssLssssLssssLssssLssssLssssLssssLssssLsssQssQsssssLsssLssssLssssLssssVssVsQssssVssLsssWsWs"
    "sLssQsssVssssLssssLsWssssLssssLssssLssssLssssLssssVsWssWssVsssWWsQsWsWsWsWsQssWsWWssssVsWsWWsssWsWWWsssV"
    "ssssLsssWsWWsWssVssQssWWssWsQssWsWWswVswWssWWwwVwsWWswWWWwwVwWwwWWWwwWWWW",
)
LAST_ROUNDS = (
    "PsLsssssLssssLsssssssLsssQsssLsssssLssssLssssLssssQsssVssssWssssLssssLsssVsWsWsssssWsVsWsWssssLsWsWssWss"
    "ssssQsQsssWWsssWsssLsssssVWsWssssVssWsWWssssVsWsWssssssLssWWsssQsWsWsWsssQssWsWsssssVsssWWsWssWsWWssWsWs"
    "sVssssssWWssWQsssVsWsssWWsQssWssWWWsssVsWsssWWVWWVWWWWWWWWWWW"
)
LATENCY, SOFTMAX_STEP, LHS_STEP = 120, 24, 48
START_TIMES, START_LAGS = [300, 986, 1612], [[0, 22, 120, 142, 330, 500, 510], [0, 22, 120, 142, 330, 650, 655]]
LOOP_TIMES, LOOP_LAGS = [1240, 747, 2746, 2398, 4010], [2, 38, 174, 227, 346, 369, 409]
END_TIMES = [500, 0, 1530]


def _tile_order():
    lag = [2] * 8 + [3] * 4 + [4] * 4
    order = []
    for p in range(NP + max(lag)):
        if p < NP:
            order += [(j, 3 * p + t) for j in (0, 1) for t in range(3)]
        order += [(2, 3 * x + t) for x in range(NP) if x + lag[x] == p for t in range(3)]
    rest = [(2, t) for t in (11, 23, 35, 42)]
    return [x for x in order if x not in rest] + rest


TILES = _tile_order()
NPL = len(TILES) - NG * LT
assert all((t + 1) * 128 <= FIRST[j] + n // (CG * LT) * STEP[j] for n, (j, t) in enumerate(TILES[:NST * CG * LT]))

R_LHS = 0
R_H = R_LHS + ZB * LT * LT * (M + HALF)
R_QKV = R_H + ZB * LT * L
R_O = R_QKV + 3 * FT * L
R_P = R_O + FT * L
R_ACC = R_P + NP * 2 * L
R_OL = R_ACC + LT * L
R_END = (R_OL + WG * LT * LT * (M + HALF) + 31) // 32 * 32


def _targets(n):
    return (n,) if n < LT else PAIRS[n - LT]


def _long_index(name):
    return LT + PAIRS.index(name) if name in PAIRS else name


def _make_plan(rounds, longs, fast):
    shell = []
    for k in range(LT):
        for n in range(k + 1, LT):
            shell += [(k, n), (n, k)]
        shell += [(k, k)]
    todo = dict(
        L=longs,
        s=[("short", g, i, j) for g in range(NG) for (i, j) in shell],
        w=[("short", NG + g, i, j) for (i, j) in shell for g in range(fast)],
        W=[("out", t, n) for k in range(0, FT, KC) for n in range(LT) for t in range(max(k, fast * LT), k + KC)],
        P=[("plain", n, 0) for n in range(NPL)] + [("plain", n, k) for n in range(NPL) for k in range(1, LT)],
        Q=[("score", p + u, both) for p in range(0, NP, 2) for both in (p // 2 % 2, 1 - p // 2 % 2) for u in (0, 1)],
        V=[("pv", t) for t in range(FT)])
    plan, timed, now = [], [], 0

    def needs(name, *args):
        if name == "out":
            return [("pv_end", args[0])]
        if name == "short" and args[0] >= NG:
            return [("out_lhs", args[0] - NG, args[2])]
        if name == "long" and args[0] >= NG:
            return [("out_lhs", args[0] - NG, j) for j in range(LT)]
        if name not in ("score", "pv"):
            return []
        need = [("softmax", args[0] // 3, 5)] if name == "pv" else []
        for tile in [(2, args[0])] if name == "pv" else [(j, 3 * args[0] + t) for j in (0, 1) for t in range(3)]:
            g, j = divmod(TILES.index(tile), LT)
            need.append(("short_end", g, j, j) if g < NG else ("plain_end", j, LT - 1))
        return need

    for n, kind in enumerate(rounds):
        tasks = todo[kind][:4]
        del todo[kind][:4]
        if kind == "Q":
            tasks += [todo["P"].pop(0), todo["P"].pop(0)]
        while kind == "w" and len(tasks) < 4:
            tasks.append(todo["W"].pop(0))
        need = [x for task in tasks for x in needs(*task)]
        until = max([now] + [time for time, task in timed if task in need])
        timed.sort(key=lambda x: x[0])
        while timed and timed[0][0] <= until:
            plan.append(timed.pop(0)[1])
        assert all(x in plan for x in need)
        plan += tasks
        now += dict(s=M + HALF, w=M + HALF, L=ZB * HALF, Q=2 * L).get(kind, L)
        for name, *args in tasks:
            if name in ("short", "plain", "long", "pv") or (name == "out" and args[0] % KC == KC - 1):
                timed.append((now + LATENCY, (name + "_end", *args)))
            if name == "pv" and args[0] < fast * LT and args[0] % LT == LT - 1:
                timed += [(now + LATENCY + LHS_STEP * j, ("out_lhs", args[0] // LT, j)) for j in range(LT)]
            if name == "score" and args[1]:
                timed += [(now + SOFTMAX_STEP * (step + args[0] % 2), ("softmax", args[0], step)) for step in range(6)]
        if kind == "L":
            timed.append((now + LATENCY, ("long_store",)))
        if kind == "s" and kind not in rounds[n + 1:]:
            plan.append(("next_tokens",))
        if kind == "L" and fast and not longs:
            timed += [(now + LATENCY + 32 * k, ("finish", k % LT, k // LT)) for k in range(LT * (ZB - 1))]
            timed.append((now + 2 * LATENCY + 32 * LT * ZB, ("finished",)))
    assert not any(todo[kind] for kind in "swWPQV")
    return plan, [task for _, task in sorted(timed, key=lambda x: x[0])]


def _ds(i, n):
    return pl.ds(i * n if isinstance(i, int) else pl.multiple_of(i * n, n), n)


def _rows(r0, n):
    return slice(r0, r0 + n)


def _dot(a, b, dims=NN):
    r = lax.dot_general(a, b, dims, preferred_element_type=F32)
    return jnp.concatenate([r[0:8], r[8:]], axis=0)


def _inverse(x):
    r = pltpu.reciprocal(x, approx=True)
    return r + r * (1.0 - x * r)


def _load(ref, *index):
    return pltpu.bitcast(ref.bitcast(U32)[index], BF16)


def _run(tasks):
    for task in tasks:
        task()


def _short_lhs(a, b, j):
    p = [a[i] + LAM[j] * b[i] if LAM[j] else a[i] for i in range(LT)]
    return [p[j] if i == j else (p[i] + p[j]) * (1.0 / (LAM[j] - LAM[i])) for i in range(LT)]


def _long_lhs(a, b, dst, i):
    p = [a[k] + LAM[k] * b[k] if LAM[k] else a[k] for k in range(LT)]
    dst[i] = b[i].astype(BF16)
    for k in ((i + 1) % LT, (i + 2) % LT):
        lo, hi = sorted((i, k))
        dst[_long_index((lo, hi))] = ((p[lo] + p[hi]) * (1.0 / (LAM[lo] - LAM[hi]))).astype(BF16)


def _combine(tile, dst, r, i):
    row = col = tile(i, i)
    for k in range(LT):
        if k != i:
            a, b = tile(i, k), tile(k, i)
            row, col = row - a, col - b
            if k > i:
                dst[_long_index((i, k)), _rows(16 * r, 16), :] = (a - b).astype(BF16)
    dst[i, _rows(16 * r, 16), :] = row.astype(BF16)
    dst[NZ + i, _rows(16 * r, 16), :] = col.astype(BF16)


def _add_long(dst, i, r, first):
    for u in range(ZB):
        x = r[_rows(u * HALF, HALF)]
        dst[u, _rows(i * HALF, HALF), :] = x if first else x + dst[u, _rows(i * HALF, HALF), :]


def _z_index(g, batch):
    if isinstance(batch, int) and batch == 0:
        return g
    if isinstance(g, int) and g >= G0:
        return g + (batch % 2) * (NG - G0)
    return jnp.where(batch == 0, g, 2 * (NG - G0) + batch * G0 + g)


def _kernel(ax_hbm, awqkv_hbm, awo_hbm, bx_hbm, mem_hbm, wq_hbm, wk_hbm, wv_hbm, wo_hbm,
            out_hbm,
            ax, awo, tmp, wqkv_p, wo_p, q_s, kv_s, oa, ob, ol, outa, outl,
            bx, mem, raw, wb, wz, wo, lz, z, lo, op, buf,
            flag, sem_a, sem_w, sem_o):
    awqkv = raw.at[pl.ds(3 * (H * DH - D), 3 * D), :]
    outb = raw.at[pl.ds(0, S), :]

    cp = pltpu.make_async_copy

    def span(first, i, n):
        return pl.ds(first + i * n if isinstance(i, int) else pl.multiple_of(first + i * n, 16), n)

    def c_strips(src, dst, at, sem):
        return [cp(src.at[at, pl.ds(t * 128, 128)], dst.at[t, at, :], sem) for t in range(LT)]

    def c_bx(i, n, sem):
        return cp(bx_hbm.at[_ds(i, n), :], bx.at[_ds(i, n), :], sem)

    def c_w(j, first, i, n, sem):
        return cp((wq_hbm, wk_hbm, wv_hbm)[j].at[span(first, i, n), :], raw.at[span(j * H * DH + first, i, n), :], sem)

    def c_ax(c, sem):
        return c_strips(ax_hbm, ax, _ds(c + NS, TB), sem)

    def c_step(c):
        return [c_bx(c + 2, TB, sem_w.at[c])] + [c_w(j, FIRST[j], c - 1, STEP[j], sem_w.at[c]) for j in range(3)]

    def c_outb(r0, n):
        at = pl.multiple_of(lax.rem(r0, TB), n)
        return cp(outb.at[pl.ds(r0, n), :], out_hbm.at[r0 // TB, pl.ds(at, n), pl.ds(D, D)], sem_o.at[1])

    def c_outl(u):
        at = pl.ds(u * (NB // ZB), NB // ZB)
        return cp(outl.at[at], out_hbm.at[at, pl.ds(TE, TL), pl.ds(0, D)], sem_o.at[2])

    def start(copies):
        for c in copies:
            c.start()

    def wait(copies):
        for c in copies:
            c.wait()

    def wait_filled(ref, sem):
        cp(ref, ref, sem).wait()

    def permute_rows(dst, base):
        def move(t, d0):
            for d in range(d0, d0 + AD // 4):
                dst[t, pl.ds(base + d * AH, AH), :] = tmp[t, pl.ds(d, AH, stride=AD), :].astype(BF16)
        return [functools.partial(move, t, d0) for t in range(LT) for d0 in range(0, AD, AD // 4)]

    def prep_wqkv(j):
        def transpose(t):
            tmp[t] = awqkv[_rows(j * D + t * 128, 128), :].astype(F32).T
        return [functools.partial(transpose, t) for t in range(LT)], permute_rows(wqkv_p, j * D)

    def prep_wo():
        def widen(t, r):
            tmp[t, _rows(r, D // 4), :] = awo[_rows(r, D // 4), _rows(t * 128, 128)].astype(F32)
        moves = permute_rows(wo_p, 0)
        return [task for t in range(LT)
                for task in [functools.partial(widen, t, r) for r in range(0, D, D // 4)] + moves[4 * t:4 * t + 4]]

    def slot(i):
        return i * TB if isinstance(i, int) and i < NS else (NS - 1) * TB

    def a_tiles(count, product, store):
        acc = {}

        def tile(t, k):
            r = product(t, k)
            acc[t] = acc[t] + r if k else r
            return r
        return [(count, functools.partial(tile, t, k), (lambda t=t: store(t, acc[t])) if k == LT - 1 else None)
                for t in range(LT) for k in range(LT)]

    def a_proj(i, j):
        at = slot(i)

        def store(t, r):
            if j == 0:
                q_s[t, _rows(at, TB), :] = r
                return
            c = (j - 1) * LT + t
            if not isinstance(i, int):
                kv_s[c, _rows(at, HALO), :] = kv_s[c, _rows(at + TB, HALO), :]
            elif i == 0:
                kv_s[c, 0:HALO, :] = jnp.broadcast_to(r[0:1, :], (HALO, 128))
            kv_s[c, _rows(at + HALO, TB), :] = r
        return a_tiles(TB, lambda t, k: _dot(_load(ax, k, _ds(i, TB // 2)), _load(wqkv_p, k, _ds(j * LT + t, 64)), NT),
                       store)

    def a_attention(i):
        state = {}

        def window(c, r0, w):
            return kv_s[c, _rows(HALO + r0 - ADIL * w, RC), :]

        def logits(r0, half, late):
            q = [q_s[t, _rows(r0, RC), :] for t in range(LT)]
            q[0] = late(q[0])
            for w in range(half * AW // 2, (half + 1) * AW // 2):
                a = q[0] * window(0, r0, w)
                for t in range(1, LT):
                    a = a + q[t] * window(t, r0, w)
                state.setdefault(r0, []).append(a + pltpu.roll(a, 2 * AH, 1))

        def fold(r0, half, late):
            for w in range(half * AW // 2, (half + 1) * AW // 2):
                a = state[r0][w]
                a = (a + pltpu.roll(a, AH, 1)) * (AD ** -0.5)
                if isinstance(i, int) and r0 < ADIL * w:
                    pos = lax.broadcasted_iota(jnp.int32, (RC, 128), 0) + r0
                    a = jnp.where(pos >= ADIL * w, a, MASKED)
                state[r0][w] = a

        def weights(r0, late):
            m = late(functools.reduce(jnp.maximum, state[r0]))
            state[r0] = [jnp.exp(a - m) for a in state[r0]]

        def mix(r0, tiles, late):
            e = [late(state[r0][0])] + state[r0][1:]
            if 0 in tiles:
                state[r0, "inverse"] = _inverse(functools.reduce(jnp.add, e))
            for t in tiles:
                o = e[0] * window(LT + t, r0, 0)
                for w in range(1, AW):
                    o = o + e[w] * window(LT + t, r0, w)
                oa[t, _rows(r0, RC), :] = o * state[r0, "inverse"]

        stages = ((logits, 0), (logits, 1), (fold, 0), (fold, 1), (weights,), (mix, (0, 1)), (mix, (2, 3, 4)))
        return [[functools.partial(f, r0, *args) for r0 in range(slot(i), slot(i) + TB, RC)] for f, *args in stages]

    def a_pack(i):
        def pack(k):
            ob[k] = oa[k, _rows(slot(i), TE), :].astype(BF16)
            ol[k, _ds(i, TL), :] = oa[k, _rows(slot(i) + TE, TL), :].astype(BF16)
        return [functools.partial(pack, k) for k in range(LT)]

    def a_out(i):
        def store(t, r):
            outa[i, :, _rows(t * 128, 128)] = r.astype(BF16)
        return a_tiles(TE, lambda t, k: _dot(_load(ob, k), _load(wo_p, t, _ds(k, 64))), store)

    def overlap(tiles, side, zero):
        due = sorted((lo + (hi - lo) * n / len(tasks), m, n, task, tie)
                     for m, (lo, hi, tasks, tie) in enumerate(side) for n, task in enumerate(tasks))
        free = [0] * 4
        results = []
        for count, tile, end in tiles:
            now = min(free)
            free[free.index(now)] += count
            results.append((now, tile()))
            while due and (due[0][0] < min(free) or len(results) == len(tiles)):
                time, _, _, task, tie = due.pop(0)
                begin, r = [x for x in results if x[0] <= time][-1]
                row = min(int(time - begin), r.shape[0] - 1) // 8 * 8
                if isinstance(tie, str):
                    task(lambda x: jnp.where(zero == 0, x, r[_rows(row, 8)]))
                    continue
                if tie is bx:
                    tie[span(S, zero, 16), 0:128] = r[_rows(row // 16 * 16, 16)].astype(BF16)
                elif tie is not None:
                    tie[tie.shape[0] - 1 - zero, 0:8, :] = pltpu.bitcast(r[_rows(row, 8)], tie.dtype)
                task()
            if end:
                end()

    def wo_rows(r0, n, t):
        return _load(wo, t, _rows(r0 // 2, n // 2))

    def w_transpose(c, n):
        at = [FT * j + t for j, t in TILES[n::CG * LT]]
        if isinstance(c, int):
            at = at[c]
        else:
            words = [sum(x << 8 * k for k, x in enumerate(at[m::5])) for m in range(5)]
            word = functools.reduce(lambda x, m: jnp.where(lax.rem(c, 5) == m, words[m], x), range(1, 5), words[0])
            at = lax.shift_right_logical(word, lax.div(c, 5) * 8) & 255
        chunk = wb.at[pl.ds(c * CG * LT, NPL if isinstance(c, int) else CG * LT)]
        chunk[n] = pltpu.bitcast(raw[_ds(at, 128), :].T, U32)

    def w_combine(c, u, r, i):
        chunk = wb.at[pl.ds(c * CG * LT, CG * LT)]
        _combine(lambda a, b: pltpu.bitcast(chunk[u * LT + b, _rows(a * 64 + 8 * r, 8), :], BF16).astype(F32),
                 wz.at[pl.ds(c * CG, CG)].at[u], r, i)

    def wo_combine(g, r, i, late):
        def tile(a, b):
            x = wo_rows((g * LT + a) * 128 + 16 * r, 16, b).astype(F32)
            return jnp.concatenate([late(x[0:8]), x[8:]], axis=0)
        _combine(tile, wz.at[NG + g], r, i)

    def halves(batch, u):
        at = batch * TB if isinstance(batch, int) else pl.multiple_of(batch * TB, TB)
        x = bx.at[pl.ds(at, TB + SEG), :][_ds(u, SEG), :].astype(F32)
        return [[x[_rows(r, HALF), _rows(i * 128, 128)] for i in range(LT)] for r in (0, HALF)]

    def z_lhs(batch):
        def task(u, i):
            _long_lhs(*halves(batch, u), lz.at[:, _ds(batch * ZB + u, HALF), :], i)
        return [functools.partial(task, u, i) for u in range(ZB) for i in range(LT)]

    def z_product(g, n, batch):
        return _dot(_load(lz, n, _ds(batch, ZB * HALF // 2)), _load(wz, g, n))

    def z_group(g, batch):
        dst = z.at[_z_index(g, batch)]
        sums, stored = {}, []

        def tile(n):
            r = z_product(g, n, batch)
            for i in _targets(n):
                sums[i] = sums[i] + r if i in sums else r
            return r

        def end():
            for i in sums:
                _add_long(dst, i, sums[i], i not in stored)
                stored.append(i)
            sums.clear()
        sets = (((0, 1), (0, 2), (1, 2), 0, 1), ((0, 3), (0, 4), (3, 4), 3, 4), ((1, 3), (1, 4), (2, 3), (2, 4), 2))
        return [(ZB * HALF, functools.partial(tile, _long_index(n)), end if n == some[-1] else None)
                for some in sets for n in some]

    def part_a():
        c_wqkv = [cp(awqkv_hbm.at[:, pl.ds(j * D, D)], awqkv.at[pl.ds(j * D, D), :], sem_a.at[j]) for j in range(3)]
        c_second = [c_wqkv[1]] + c_strips(ax_hbm, ax, pl.ds(0, NS * TB), sem_a.at[1])
        c_third = [c_wqkv[2], c_bx(0, 2 * TB, sem_a.at[2])]
        c_awo = cp(awo_hbm, awo, sem_a.at[3])
        c_first = c_ax(0, sem_w.at[0]) + [c_bx(2, TB, sem_w.at[0])] + [
            c_w(j, 0, 0, FIRST[j], sem_w.at[0]) for j in range(2)]
        last_rows = pl.ds(S - 2 * TB, 2 * TB)
        c_last = [c_bx(NB // 2 - 1, 2 * TB, sem_w.at[NST]), cp(mem_hbm, mem.at[pl.ds(0, M), :], sem_w.at[NST]),
                  c_w(2, (NST - 1) * STEP[2], 0, H * DH - (NST - 1) * STEP[2], sem_w.at[NST])]

        flag[0] = 0
        start([c_wqkv[0]] + c_second)
        c_wqkv[0].wait()
        zero = flag[0]
        _run(sum(prep_wqkv(0), []))
        start(c_third)
        wait(c_second)
        first, second = prep_wqkv(1)
        overlap(a_proj(0, 0) + a_proj(1, 0), [(0, 0, first, None), (700, 1500, second, tmp)], zero)
        start([c_awo] + c_first[:-1])
        wait(c_third)
        first, second = prep_wqkv(2)
        overlap(a_proj(0, 1) + a_proj(1, 1),
                [(0, 0, first, None), (700, 1500, second, tmp), (0, 1500, z_lhs(0) + z_lhs(1), bx)], zero)
        c_first[-1].start()
        c_awo.wait()
        for i in range(NS):
            assert START_TIMES[i] + START_LAGS[i][-2] >= (i + 1) * 800
        assert START_TIMES[1] + START_LAGS[0][-1] <= 1500
        overlap(a_proj(0, 2) + a_proj(1, 2) + a_out(0),
                [(0, 800, prep_wo(), tmp), (1500, 1500, a_pack(0), None)]
                + [(START_TIMES[i] + d, START_TIMES[i + 1] + d, tasks, "value")
                   for i in range(NS) for d, tasks in zip(START_LAGS[i], a_attention(i))], zero)
        start(c_ax(1, sem_w.at[1]) + c_step(1) + c_ax(2, sem_w.at[2]) + c_step(2))
        wait(c_first)

        def step(c, carry):
            pl.when((c > 0) & (c < NST))(lambda: wait_filled(ax.at[:, _ds(c + NS, TB), :], sem_w.at[c]))
            for copy in c_step(jnp.clip(c, 1, NST - 1)):
                pl.when((c > 0) & (c < NST))(copy.wait)
            pl.when(c == NST)(lambda: wait_filled(ax.at[:, last_rows, :], sem_w.at[NST]))
            for copy in c_last:
                pl.when(c == NST)(copy.wait)

            zero = lax.shift_right_logical(c, 16)
            flag[zero] = 0
            i, t = c + NS, LOOP_TIMES
            assert t[0] / 2 <= t[1] + 100 and t[2] < 2900 and t[3] + LOOP_LAGS[-2] > 2500
            early = [x for u in range(2) for b in range(2) for x in z_group((c & 1) * 2 + u, (c | 1) + b)]
            overlap(a_proj(i, 0) + a_proj(i, 1) + a_proj(i, 2) + a_out(i - 1)
                    + z_group(c * CG, 0) + early + z_group(c * CG + 1, 0),
                    [(0, t[0], [functools.partial(w_transpose, c, n) for n in range(CG * LT)], None),
                     (0, t[1], z_lhs(c + 2), bx),
                     (0, t[1], a_pack(i - 1), oa),
                     (t[1], t[2], [functools.partial(w_combine, c, u, r, k)
                                   for u in range(CG) for r in range(8) for k in range(LT)], wb)]
                    + [(t[3] + d, t[4] + d, tasks, "value") for d, tasks in zip(LOOP_LAGS, a_attention(i))], zero)

            n = jnp.minimum(c + 3, NST - 1)
            for copy in c_ax(n, sem_w.at[n]) + c_step(n) + c_strips(wo_hbm, wo, _ds(c, WO_STEP), sem_a.at[4]):
                pl.when(c < NST - 3)(copy.start)
            for copy in c_strips(ax_hbm, ax, last_rows, sem_w.at[NST]) + c_last:
                pl.when(c == NST - 3)(copy.start)
            at = span(WO_FIRST, jnp.clip(c - (NST - 2), 0, 1), (H * DH - WO_FIRST) // 2)
            for copy in c_strips(wo_hbm, wo, at, sem_a.at[5]):
                pl.when((c > NST - 3) & (c < NST))(copy.start)
            return carry

        lax.fori_loop(0, NCH, step, 0)
        wait_filled(wo.at[:, pl.ds(0, WO_FIRST), :], sem_a.at[4])
        t = END_TIMES
        overlap([x for g in range(G0) for x in z_group(g, NB - 1)] + a_out(NB - 1),
                [(0, 0, [functools.partial(w_transpose, NCH, n) for n in range(NPL)], None),
                 (0, t[0], a_pack(NB - 1), oa),
                 (t[1], t[2], [functools.partial(wo_combine, g, r, i)
                               for g in range(WG) for r in range(8) for i in range(LT)], "value")], zero)

    def r_lhs(hb, i, j):
        return R_LHS + ((hb * LT + i) * LT + j) * (M + HALF)

    def r_qkv(j, t):
        return _rows(R_QKV + (j * FT + t) * L, L)

    def token_lhs(batch, u, hb):
        a, b = halves(batch, u)
        for j in range(LT):
            buf[_rows(R_H + (hb * LT + j) * L + M, SEG)] = jnp.concatenate([a[j], b[j]], axis=0)
            for i, x in enumerate(_short_lhs(a, b, j)):
                buf[_rows(r_lhs(hb, i, j) + M, HALF)] = x

    def memory_lhs(m, n, hb):
        buf[_rows(R_H + (hb * LT + n) * L, M)] = m[n]
        buf[_rows(r_lhs(hb, n, n), M)] = m[n]
        for k in range(n):
            buf[_rows(r_lhs(hb, n, k), M)] = buf[_rows(r_lhs(hb, k, n), M)] = m[n] + m[k]

    stored = []

    def segment(plan, batch, part, hb, nh, before=()):
        s = batch * ZB + part
        key = lax.broadcasted_iota(jnp.int32, (L, 128), 0)
        col = lax.broadcasted_iota(jnp.int32, (L, 128), 1)
        head0 = col < L
        query = jnp.where(head0, col, col - L)
        visible = (query < M) | (query >= key)
        low = col < 64
        zo = z.at[z.shape[0] - 1 - batch % 2]
        z_next = z.at[pl.ds(_z_index(G0, batch + 1), NG - G0)]
        val, sums, new_mem = {}, {}, []

        def add(name, x):
            val[name] = val[name] + x if name in val else x

        def product(*args):
            r = _dot(*args)
            val["latest"] = r[-8:]
            return r

        def short(g, i, j):
            if i == j:
                w = _load(wz, g, NZ + i)
            elif g < NG:
                w = pltpu.bitcast(wb[g * LT + j, _rows(i * 64, 64), :], BF16)
            else:
                w = wo_rows(((g - NG) * LT + i) * 128, 128, j)
            at = r_lhs(hb, i, j) if g < NG else R_OL + r_lhs(g - NG, i, j)
            add((min(g, NG), i, j), product(buf[_rows(at, M + HALF)], w))

        def short_end(g, i, j):
            if NG <= g < NG + WG - 1:
                return
            g = min(g, NG)
            r = val.pop((g, i, j))
            add(("m", g, j), r[0:M])
            if i != j:
                add(("y", g, i), r[M:])
                add(("b", g, j), r[M:])
                if LAM[i]:
                    add(("a", g, j), r[M:] * -LAM[i])
                return
            y = val.pop(("y", g, j))
            if g < NG:
                y = y + z[_z_index(g, batch), part, _rows(j * HALF, HALF), :]
            a = val.pop(("a", g, j)) + r[M:]
            if LAM[j]:
                a = a - LAM[j] * y
            r = jnp.concatenate([val.pop(("m", g, j)), a, val.pop(("b", g, j)) + y], axis=0)
            if g < NG:
                buf[r_qkv(*TILES[g * LT + j])] = r
            else:
                buf[_rows(R_ACC + j * L, L)] = out_sum(j, r)

        def plain(n, k):
            w = pltpu.bitcast(wb[NG * LT + n, _rows(k * 64, 64), :], BF16)
            val["plain", n, k] = product(buf[_rows(R_H + (hb * LT + k) * L, L)], w)

        def plain_end(n, k):
            dst = r_qkv(*TILES[NG * LT + n])
            r = val.pop(("plain", n, k))
            buf[dst] = r + buf[dst] if k else r

        def long(g, n):
            r = z_product(g, n, batch + 1) if g < NG else _dot(_load(lo, g - NG, n), _load(wz, g, n))
            val["long", g, n], val["latest"] = r, r[24:32]

        def long_end(g, n):
            r = val.pop(("long", g, n))
            g = min(g, NG)
            for i in _targets(n):
                sums[g, i] = sums[g, i] + r if (g, i) in sums else r

        def long_store():
            for (g, i), r in sums.items():
                _add_long(z_next.at[g - G0] if g < NG else zo, i, r, (g, i) not in stored)
                stored.append((g, i))
            sums.clear()

        def a_late(u, t, k):
            n = ZB * HALF
            x = _load(ol, k, _ds(part * (NB * TL // (ZB * n)) + u, n // 2))
            add("late", product(x, _load(wo_p, t, _ds(k, 64))))
            if k == LT - 1:
                r = val.pop("late").astype(BF16)
                for m in range(n // TL):
                    outl[part * (NB // ZB) + u * (n // TL) + m, :, _rows(t * 128, 128)] = r[_rows(m * TL, TL)]

        def score(p, both):
            if both:
                q, k = [[buf[r_qkv(j, 3 * p + t)] for t in (0, 2)] for j in (0, 1)]
            else:
                q, k = buf[r_qkv(0, 3 * p + 1)], [buf[r_qkv(1, 3 * p + 1)]]
                q = [jnp.where(low, q, 0.0), jnp.where(low, 0.0, q)]
            q = jnp.concatenate(q + [jnp.zeros((128 - 2 * L, 128), F32)], axis=0)
            r = product(jnp.concatenate(k, axis=0), q.astype(BF16), NT)
            add(("s", p), jnp.where(head0, r[0:L], r[L:]) if both else r)

        def softmax(p, step):
            def late(x):
                return jnp.where(col[0:8] < 2 * L, x, val["latest"])

            def groups(x):
                return [x[_rows(r, 8)] for r in range(0, L, 8)]

            def spread(x):
                return jnp.concatenate([x] * (L // 8), axis=0)
            x, y = val["s", p], val.get(("t", p))
            if step == 0:
                x = jnp.where(visible, x * (DH ** -0.5), MASKED)
                y = functools.reduce(jnp.maximum, groups(x))
            elif step == 1:
                y = jnp.broadcast_to(jnp.max(late(y), axis=0, keepdims=True), (8, 128))
            elif step == 2:
                x = jnp.exp(x - spread(late(y)))
                y = functools.reduce(jnp.add, groups(x))
            elif step == 3:
                y = jnp.broadcast_to(jnp.sum(late(y), axis=0, keepdims=True), (8, 128))
            elif step == 4:
                y = _inverse(late(y))
            else:
                x = x * spread(late(y))
                x = jnp.concatenate([x, x], axis=0)[:, 0:2 * L]
                buf[_rows(R_P + p * 2 * L, 2 * L), 0:2 * L] = x.astype(BF16).T.astype(F32)
            val["s", p], val["t", p] = x, y

        def pv(t):
            pa, pb = [buf[_rows(R_P + (2 * (t // 3) + u) * L, L), 0:2 * L] for u in range(2)]
            v = buf[r_qkv(2, t)]
            if t % 3 == 1:
                v = jnp.concatenate([jnp.where(low, v, 0.0), jnp.where(low, 0.0, v)], axis=0)
            pr = (pa[:, 0:L], jnp.where(head0[:, 0:2 * L], pa, pb), pb[:, 0:L])[t % 3]
            val["o", t] = product(pr, v.astype(BF16))

        def pv_end(t):
            buf[_rows(R_O + t * L, L)] = val.pop(("o", t))

        def out_lhs(g, j):
            o = [buf[_rows(R_O + (g * LT + i) * L, L)] for i in range(LT)]
            a, b = [x[M:M + HALF] for x in o], [x[M + HALF:] for x in o]
            a[j] = jnp.concatenate([jnp.where(batch >= 0, x, val["latest"]) for x in (a[j][0:8], a[j][8:])], axis=0)
            for i, x in enumerate(_short_lhs(a, b, j)):
                m = o[j][0:M] if i == j else o[i][0:M] + o[j][0:M]
                buf[_rows(R_OL + r_lhs(g, i, j), M + HALF)] = jnp.concatenate([m, x], axis=0)
            _long_lhs(a, b, lo.at[g, :, _rows(part * HALF, HALF), :], j)

        def out(t, n):
            x = buf[_rows(R_O + t * L, L)]
            if "stored" in val:
                x = jnp.concatenate([x[0:L - 8], jnp.where(batch >= 0, x[L - 8:], val.pop("stored"))], axis=0)
            add(("out", t // KC, n), product(x, wo_rows(t * 128, 128, n)))

        def out_sum(n, r):
            if ("sum", n) in val:
                r = r + buf[_rows(R_ACC + n * L, L)]
            val["sum", n] = True
            return r

        def out_end(t, n):
            r = out_sum(n, val.pop(("out", t // KC, n)))
            if t < FT - 1:
                buf[_rows(R_ACC + n * L, L)] = r
                return
            new_mem.append(r[0:M])
            memory_lhs(new_mem, n, nh)
            if not isinstance(part, int):
                outb[_ds(s, SEG), _rows(n * 128, 128)] = r[M:L].astype(BF16)
            elif part < ZB - 1:
                op[part, n] = r[M:L]
            else:
                finish(n, part, r[M:L])

        def finish(n, u, r=None):
            y = zo[u, _rows(n * HALF, HALF), :]
            if r is None:
                r = op[u, n]
                y = jnp.concatenate([jnp.where(batch >= 0, x, val["latest"]) for x in (y[0:8], y[8:])], axis=0)
            y = jnp.concatenate([-LAM[n] * y, y], axis=0)
            outb[_ds(batch * ZB + u, SEG), _rows(n * 128, 128)] = (r + y).astype(BF16)

        def finished():
            val["stored"] = outb[_ds(jnp.maximum(batch, 0) * (TB // 8), 8), 0:128].astype(F32)

        tasks = dict(short=short, short_end=short_end, plain=plain, plain_end=plain_end, long=long,
                     long_end=long_end, long_store=long_store, a_late=a_late, score=score, softmax=softmax,
                     pv=pv, pv_end=pv_end, out_lhs=out_lhs, out=out, out_end=out_end, finish=finish, finished=finished,
                     next_tokens=lambda: token_lhs(
                         batch, part + 1 if isinstance(part, int) else jnp.minimum(part + 1, ZB - 1), nh))
        before = list(before)
        for name, *args in plan[0]:
            if name in ("short", "plain"):
                while len(before) > LT - 1 - max(args[1:]):
                    before.pop(0)()
            tasks[name](*args)
        return [functools.partial(tasks[name], *args) for name, *args in plan[1]]

    order = [_long_index(n) for n in
             ((0, 1), (0, 2), (1, 2), 0, (0, 3), (0, 4), (3, 4), 3, 4, (1, 4), 1, (1, 3), (2, 3), (2, 4), 2)]
    longs = ([("long", g, n) for g in range(G0, NG) for n in order]
             + [("long", NG + g, n) for n in order for g in range(WG)])
    plans = [_make_plan(rounds, longs, WG) for rounds in ROUNDS]
    late = [("a_late", u, t, k) for u in range(NB * TL // (ZB * ZB * HALF)) for t in range(LT) for k in range(LT)]
    last_plan = _make_plan(LAST_ROUNDS, late, 0)
    assert not longs and not late
    tasks = plans[-1][0]
    assert ("long", NG, order[0]) in tasks and ("finished",) in tasks
    assert ("long_store",) not in tasks[tasks.index(("finish", 0, 0)):]
    for tasks in (sum(plan, []) for plan in plans):
        assert tasks.index(("short_end", NG + WG - 1, LT - 1, LT - 1)) < tasks.index(("out_end", FT - 1, 0))

    def batch_step(batch, carry):
        rest = ()
        for u in range(ZB):
            rest = segment(plans[u], batch, u, u, (u + 1) % ZB, rest)
        _run(rest)
        c_outb(pl.multiple_of(batch * TB, TB), TB).start()
        return carry

    def last_step(s, carry):
        _run(segment(last_plan, s // ZB, s % ZB, 0, 0))
        c_outl(s % ZB).start()
        c_outb(pl.multiple_of(s * SEG, SEG), SEG).start()
        return carry

    part_a()
    token_lhs(0, 0, 0)
    mem0 = mem[0:M, :].astype(F32)
    for n in range(LT):
        memory_lhs([mem0[:, _rows(k * 128, 128)] for k in range(LT)], n, 0)
    wait_filled(wo.at[:, pl.ds(WO_FIRST, H * DH - WO_FIRST), :], sem_a.at[5])
    c_outa = cp(outa, out_hbm.at[:, pl.ds(0, TE), pl.ds(0, D)], sem_o.at[0])
    c_outa.start()
    lax.fori_loop(0, NB - 1, batch_step, 0)
    lax.fori_loop(NSEG - ZB, NSEG, last_step, 0)
    c_outa.wait()
    wait_filled(out_hbm.at[:, :, pl.ds(D, D)], sem_o.at[1])
    wait_filled(out_hbm.at[:, pl.ds(TE, TL), pl.ds(0, D)], sem_o.at[2])


def pallas_concat_heads__sliding_local_dilated__memory_aug_recurrent_mem_tr__prompt_kernel(
    A_x, A_wqkv, A_wo, B_x, B_mem0, B_Wq, B_Wk, B_Wv, B_Wo, B_seg_len,
):
    assert B_seg_len == SEG
    assert A_x.shape == B_x.shape == (1, S, D) and B_mem0.shape == (1, M, D)
    assert B_Wq.shape == B_Wk.shape == B_Wv.shape == (D, H, DH) and B_Wo.shape == (H, DH, D)
    vmem, dma = pltpu.VMEM, pltpu.SemaphoreType.DMA
    call = pl.pallas_call(
        _kernel,
        out_shape=jax.ShapeDtypeStruct((NB, TB, 2 * D), BF16),
        in_specs=[pl.BlockSpec(memory_space=pl.ANY)] * 9,
        out_specs=pl.BlockSpec(memory_space=pl.ANY),
        scratch_shapes=[
            vmem((LT, S, 128), BF16),
            vmem((D, D), BF16),
            vmem((LT + 1, D, 128), F32),
            vmem((LT, 3 * D, 128), BF16),
            vmem((LT, D, 128), BF16),
            vmem((LT, NS * TB, 128), F32),
            vmem((2 * LT, HALO + NS * TB, 128), F32),
            vmem((LT + 1, NS * TB, 128), F32),
            vmem((LT + 1, TE, 128), BF16),
            vmem((LT, NB * TL, 128), BF16),
            vmem((NB, TE, D), BF16),
            vmem((NB, TL, D), BF16),
            vmem((S + 64, D), BF16),
            vmem((64, D), BF16),
            vmem((3 * H * DH, D), BF16),
            vmem((len(TILES) + 1, D // 2, 128), U32),
            vmem((NG + WG, NZ + LT, 128, 128), BF16),
            vmem((LT, H * DH, 128), BF16),
            vmem((NZ, S // 2, 128), BF16),
            vmem((2 * (NG - G0) + NB * G0 + 2, ZB, (LT + 1) * HALF, 128), F32),
            vmem((WG, NZ, ZB * HALF, 128), BF16),
            vmem((ZB, LT, SEG, 128), F32),
            vmem((R_END, 128), F32),
            pltpu.SMEM((2,), jnp.int32),
            dma((6,)), dma((NCH,)), dma((3,)),
        ],
        compiler_params=pltpu.CompilerParams(
            vmem_limit_bytes=126 * 1024 * 1024, internal_scratch_in_bytes=48 * 1024,
            disable_bounds_checks=True, disable_semaphore_checks=True),
        name="sliding_and_memory_attention",
    )

    def by_feature(w):
        return w.transpose(1, 2, 0).reshape(H * DH, D)

    out = call(A_x.reshape(S, D), A_wqkv, A_wo, B_x.reshape(S, D), B_mem0.reshape(M, D),
               by_feature(B_Wq), by_feature(B_Wk), by_feature(B_Wv), B_Wo.reshape(H * DH, D))
    return out.reshape(1, S, 2 * D)
```

```python
import functools

import jax
import jax.numpy as jnp
from jax import lax
from jax.experimental import pallas as pl
from jax.experimental.pallas import tpu as pltpu

F32, BF16, U32 = jnp.float32, jnp.bfloat16, jnp.uint32
NN = (((1,), (0,)), ((), ()))
NT = (((1,), (1,)), ((), ()))
MASKED = -1000000000.0

S, D = 2048, 640
LT = D // 128

AH, AD, AW, ADIL = 32, 20, 8, 2
HALO = 16
TB = 128
NB = S // TB
NS = 2
TL = 32
TE = TB - TL
RC = 8

H, DH, M, SEG = 32, 192, 8, 32
L = M + SEG
HALF = SEG // 2
NP = H // 2
FT = 3 * NP
NSEG = S // SEG
LAM = (0.0, 0.625, -0.625, 1.875, -1.875)
PAIRS = [(i, j) for i in range(LT) for j in range(i + 1, LT)]
NZ = LT + len(PAIRS)
NG = 28
WG = 2
G0 = 4
ZB = TB // SEG
KC = 3
CG = 2
NCH = NG // CG
NST = NCH - 2
FIRST, STEP = (864, 688, 0), (480, 496, 432)
WO_STEP = 256
WO_FIRST = (NST - 3) * WO_STEP

ROUNDS = (
    "PsLssssLssssLssssLssssLssssLssssLssssLsQssssLssssLssssLssssLssQsssVssssLssssLsssssLsssVsssLssssLssQsssVs"
    "sssLssssLssssLssssLssQssVsssssWsLssssLssWWssssLsssVsWsssWssVsssWsQsWsWssssWQsWssWsWWssWWsssVsssWWWsssVsW"
    "sWsWsWsssWWWsssVssQsWsWsWsQsssWWWsssVswWsWWssVwWwWwwwWVwwwWwWWwwWWWwWWWW",
    "LPssssLssssLssssLssssLssssLssssLssssLssssLssssLssssLssssLssssLsssQssQssssLsssLssssLssssVssVssQsssVssssLs"
    "sWssssWsLssQssVssssLsssLssssLssssLssssLsssVssWsWsssVssssLsssWsWWsWsQsWsWsWsQssWsWWsWssssVsWWssWsWsWsWssV"
    "ssssLsWsssWWsWssVssQsWsWsWsQsssWWsWswVsWwsWWswwVswWsWWwWwwVWwWwWWwWwwWWWW",
    "LPsssLssssLssssLssssLssssLsQssssLssssLssssLssssLssssLssssVsQssssLsssssLssssLsssVssQsssVssssLssssLssssLsW"
    "sWssQsssVsssssLssssLsWssWssssLssssLssssLssWsssVsWssssVsQsWssWWssQssssLsWssWsssLssWsWsWssVsssWWsWsssVWssW"
    "sWssWsWssWWWsssVssQsWsWsWsQsssWWsWwssVsWwwWWwsVssWWwWwwwVwwWWWwWWwwWWWWW",
    "LPssssLssssLssssLssssLssssLssssLssssLssssLssssLssssLsssQssQsssssLsssLssssLssssLssssVssVsQssssVssLsssWsWs"
    "sLssQsssVssssLssssLsWssssLssssLssssLssssLssssLssssVsWssWssVsssWWsQsWsWsWsWsQssWsWWssssVsWsWWsssWsWWWsssV"
    "ssssLsssWsWWsWssVssQssWWssWsQssWsWWswVswWssWWwwVwsWWswWWWwwVwWwwWWWwwWWWW",
)
LAST_ROUNDS = (
    "PsLsssssLssssLsssssssLsssQsssLsssssLssssLssssLssssQsssVssssWssssLssssLsssVsWsWsssssWsVsWsWssssLsWsWssWss"
    "ssssQsQsssWWsssWsssLsssssVWsWssssVssWsWWssssVsWsWssssssLssWWsssQsWsWsWsssQssWsWsssssVsssWWsWssWsWWssWsWs"
    "sVssssssWWssWQsssVsWsssWWsQssWssWWWsssVsWsssWWVWWVWWWWWWWWWWW"
)
LATENCY, SOFTMAX_STEP, LHS_STEP = 120, 24, 48
START_TIMES, START_LAGS = [300, 986, 1612], [[0, 22, 120, 142, 330, 500, 510], [0, 22, 120, 142, 330, 650, 655]]
LOOP_TIMES, LOOP_LAGS = [1240, 747, 2746, 2398, 4010], [2, 38, 174, 227, 346, 369, 409]
END_TIMES = [500, 0, 1530]


def _tile_order():
    lag = [2] * 8 + [3] * 4 + [4] * 4
    order = []
    for p in range(NP + max(lag)):
        if p < NP:
            order += [(j, 3 * p + t) for j in (0, 1) for t in range(3)]
        order += [(2, 3 * x + t) for x in range(NP) if x + lag[x] == p for t in range(3)]
    rest = [(2, t) for t in (11, 23, 35, 42)]
    return [x for x in order if x not in rest] + rest


TILES = _tile_order()
NPL = len(TILES) - NG * LT
assert all((t + 1) * 128 <= FIRST[j] + n // (CG * LT) * STEP[j] for n, (j, t) in enumerate(TILES[:NST * CG * LT]))

R_LHS = 0
R_H = R_LHS + ZB * LT * LT * (M + HALF)
R_QKV = R_H + ZB * LT * L
R_O = R_QKV + 3 * FT * L
R_P = R_O + FT * L
R_ACC = R_P + NP * 2 * L
R_OL = R_ACC + LT * L
R_END = (R_OL + WG * LT * LT * (M + HALF) + 31) // 32 * 32


def _targets(n):
    return (n,) if n < LT else PAIRS[n - LT]


def _long_index(name):
    return LT + PAIRS.index(name) if name in PAIRS else name


def _make_plan(rounds, longs, fast):
    shell = []
    for k in range(LT):
        for n in range(k + 1, LT):
            shell += [(k, n), (n, k)]
        shell += [(k, k)]
    todo = dict(
        L=longs,
        s=[("short", g, i, j) for g in range(NG) for (i, j) in shell],
        w=[("short", NG + g, i, j) for (i, j) in shell for g in range(fast)],
        W=[("out", t, n) for k in range(0, FT, KC) for n in range(LT) for t in range(max(k, fast * LT), k + KC)],
        P=[("plain", n, 0) for n in range(NPL)] + [("plain", n, k) for n in range(NPL) for k in range(1, LT)],
        Q=[("score", p + u, both) for p in range(0, NP, 2) for both in (p // 2 % 2, 1 - p // 2 % 2) for u in (0, 1)],
        V=[("pv", t) for t in range(FT)])
    plan, timed, now = [], [], 0

    def needs(name, *args):
        if name == "out":
            return [("pv_end", args[0])]
        if name == "short" and args[0] >= NG:
            return [("out_lhs", args[0] - NG, args[2])]
        if name == "long" and args[0] >= NG:
            return [("out_lhs", args[0] - NG, j) for j in range(LT)]
        if name not in ("score", "pv"):
            return []
        need = [("softmax", args[0] // 3, 5)] if name == "pv" else []
        for tile in [(2, args[0])] if name == "pv" else [(j, 3 * args[0] + t) for j in (0, 1) for t in range(3)]:
            g, j = divmod(TILES.index(tile), LT)
            need.append(("short_end", g, j, j) if g < NG else ("plain_end", j, LT - 1))
        return need

    for n, kind in enumerate(rounds):
        tasks = todo[kind][:4]
        del todo[kind][:4]
        if kind == "Q":
            tasks += [todo["P"].pop(0), todo["P"].pop(0)]
        while kind == "w" and len(tasks) < 4:
            tasks.append(todo["W"].pop(0))
        need = [x for task in tasks for x in needs(*task)]
        until = max([now] + [time for time, task in timed if task in need])
        timed.sort(key=lambda x: x[0])
        while timed and timed[0][0] <= until:
            plan.append(timed.pop(0)[1])
        assert all(x in plan for x in need)
        plan += tasks
        now += dict(s=M + HALF, w=M + HALF, L=ZB * HALF, Q=2 * L).get(kind, L)
        for name, *args in tasks:
            if name in ("short", "plain", "long", "pv") or (name == "out" and args[0] % KC == KC - 1):
                timed.append((now + LATENCY, (name + "_end", *args)))
            if name == "pv" and args[0] < fast * LT and args[0] % LT == LT - 1:
                timed += [(now + LATENCY + LHS_STEP * j, ("out_lhs", args[0] // LT, j)) for j in range(LT)]
            if name == "score" and args[1]:
                timed += [(now + SOFTMAX_STEP * (step + args[0] % 2), ("softmax", args[0], step)) for step in range(6)]
        if kind == "L":
            timed.append((now + LATENCY, ("long_store",)))
        if kind == "s" and kind not in rounds[n + 1:]:
            plan.append(("next_tokens",))
        if kind == "L" and fast and not longs:
            timed += [(now + LATENCY + 32 * k, ("finish", k % LT, k // LT)) for k in range(LT * (ZB - 1))]
            timed.append((now + 2 * LATENCY + 32 * LT * ZB, ("finished",)))
    assert not any(todo[kind] for kind in "swWPQV")
    return plan, [task for _, task in sorted(timed, key=lambda x: x[0])]


def _ds(i, n):
    return pl.ds(i * n if isinstance(i, int) else pl.multiple_of(i * n, n), n)


def _rows(r0, n):
    return slice(r0, r0 + n)


def _dot(a, b, dims=NN):
    r = lax.dot_general(a, b, dims, preferred_element_type=F32)
    return jnp.concatenate([r[0:8], r[8:]], axis=0)


def _inverse(x):
    r = pltpu.reciprocal(x, approx=True)
    return r + r * (1.0 - x * r)


def _load(ref, *index):
    return pltpu.bitcast(ref.bitcast(U32)[index], BF16)


def _run(tasks):
    for task in tasks:
        task()


def _short_lhs(a, b, j):
    p = [a[i] + LAM[j] * b[i] if LAM[j] else a[i] for i in range(LT)]
    return [p[j] if i == j else (p[i] + p[j]) * (1.0 / (LAM[j] - LAM[i])) for i in range(LT)]


def _long_lhs(a, b, dst, i):
    p = [a[k] + LAM[k] * b[k] if LAM[k] else a[k] for k in range(LT)]
    dst[i] = b[i].astype(BF16)
    for k in ((i + 1) % LT, (i + 2) % LT):
        lo, hi = sorted((i, k))
        dst[_long_index((lo, hi))] = ((p[lo] + p[hi]) * (1.0 / (LAM[lo] - LAM[hi]))).astype(BF16)


def _combine(tile, dst, r, i):
    row = col = tile(i, i)
    for k in range(LT):
        if k != i:
            a, b = tile(i, k), tile(k, i)
            row, col = row - a, col - b
            if k > i:
                dst[_long_index((i, k)), _rows(16 * r, 16), :] = (a - b).astype(BF16)
    dst[i, _rows(16 * r, 16), :] = row.astype(BF16)
    dst[NZ + i, _rows(16 * r, 16), :] = col.astype(BF16)


def _add_long(dst, i, r, first):
    for u in range(ZB):
        x = r[_rows(u * HALF, HALF)]
        dst[u, _rows(i * HALF, HALF), :] = x if first else x + dst[u, _rows(i * HALF, HALF), :]


def _z_index(g, batch):
    if isinstance(batch, int) and batch == 0:
        return g
    if isinstance(g, int) and g >= G0:
        return g + (batch % 2) * (NG - G0)
    return jnp.where(batch == 0, g, 2 * (NG - G0) + batch * G0 + g)


def _kernel(ax_hbm, awqkv_hbm, awo_hbm, bx_hbm, mem_hbm, wq_hbm, wk_hbm, wv_hbm, wo_hbm,
            out_hbm,
            ax, awo, tmp, wqkv_p, wo_p, q_s, kv_s, oa, ob, ol, outa, outl,
            bx, mem, raw, wb, wz, wo, lz, z, lo, op, buf,
            flag, sem_a, sem_w, sem_o):
    awqkv = raw.at[pl.ds(3 * (H * DH - D), 3 * D), :]
    outb = raw.at[pl.ds(0, S), :]

    cp = pltpu.make_async_copy

    def span(first, i, n):
        return pl.ds(first + i * n if isinstance(i, int) else pl.multiple_of(first + i * n, 16), n)

    def c_strips(src, dst, at, sem):
        return [cp(src.at[at, pl.ds(t * 128, 128)], dst.at[t, at, :], sem) for t in range(LT)]

    def c_bx(i, n, sem):
        return cp(bx_hbm.at[_ds(i, n), :], bx.at[_ds(i, n), :], sem)

    def c_w(j, first, i, n, sem):
        return cp((wq_hbm, wk_hbm, wv_hbm)[j].at[span(first, i, n), :], raw.at[span(j * H * DH + first, i, n), :], sem)

    def c_ax(c, sem):
        return c_strips(ax_hbm, ax, _ds(c + NS, TB), sem)

    def c_step(c):
        return [c_bx(c + 2, TB, sem_w.at[c])] + [c_w(j, FIRST[j], c - 1, STEP[j], sem_w.at[c]) for j in range(3)]

    def c_outb(r0, n):
        at = pl.multiple_of(lax.rem(r0, TB), n)
        return cp(outb.at[pl.ds(r0, n), :], out_hbm.at[r0 // TB, pl.ds(at, n), pl.ds(D, D)], sem_o.at[1])

    def c_outl(u):
        at = pl.ds(u * (NB // ZB), NB // ZB)
        return cp(outl.at[at], out_hbm.at[at, pl.ds(TE, TL), pl.ds(0, D)], sem_o.at[2])

    def start(copies):
        for c in copies:
            c.start()

    def wait(copies):
        for c in copies:
            c.wait()

    def wait_filled(ref, sem):
        cp(ref, ref, sem).wait()

    def permute_rows(dst, base):
        def move(t, d0):
            for d in range(d0, d0 + AD // 4):
                dst[t, pl.ds(base + d * AH, AH), :] = tmp[t, pl.ds(d, AH, stride=AD), :].astype(BF16)
        return [functools.partial(move, t, d0) for t in range(LT) for d0 in range(0, AD, AD // 4)]

    def prep_wqkv(j):
        def transpose(t):
            tmp[t] = awqkv[_rows(j * D + t * 128, 128), :].astype(F32).T
        return [functools.partial(transpose, t) for t in range(LT)], permute_rows(wqkv_p, j * D)

    def prep_wo():
        def widen(t, r):
            tmp[t, _rows(r, D // 4), :] = awo[_rows(r, D // 4), _rows(t * 128, 128)].astype(F32)
        moves = permute_rows(wo_p, 0)
        return [task for t in range(LT)
                for task in [functools.partial(widen, t, r) for r in range(0, D, D // 4)] + moves[4 * t:4 * t + 4]]

    def slot(i):
        return i * TB if isinstance(i, int) and i < NS else (NS - 1) * TB

    def a_tiles(count, product, store):
        acc = {}

        def tile(t, k):
            r = product(t, k)
            acc[t] = acc[t] + r if k else r
            return r
        return [(count, functools.partial(tile, t, k), (lambda t=t: store(t, acc[t])) if k == LT - 1 else None)
                for t in range(LT) for k in range(LT)]

    def a_proj(i, j):
        at = slot(i)

        def store(t, r):
            if j == 0:
                q_s[t, _rows(at, TB), :] = r
                return
            c = (j - 1) * LT + t
            if not isinstance(i, int):
                kv_s[c, _rows(at, HALO), :] = kv_s[c, _rows(at + TB, HALO), :]
            elif i == 0:
                kv_s[c, 0:HALO, :] = jnp.broadcast_to(r[0:1, :], (HALO, 128))
            kv_s[c, _rows(at + HALO, TB), :] = r
        return a_tiles(TB, lambda t, k: _dot(_load(ax, k, _ds(i, TB // 2)), _load(wqkv_p, k, _ds(j * LT + t, 64)), NT),
                       store)

    def a_attention(i):
        state = {}

        def window(c, r0, w):
            return kv_s[c, _rows(HALO + r0 - ADIL * w, RC), :]

        def logits(r0, half, late):
            q = [q_s[t, _rows(r0, RC), :] for t in range(LT)]
            q[0] = late(q[0])
            for w in range(half * AW // 2, (half + 1) * AW // 2):
                a = q[0] * window(0, r0, w)
                for t in range(1, LT):
                    a = a + q[t] * window(t, r0, w)
                state.setdefault(r0, []).append(a + pltpu.roll(a, 2 * AH, 1))

        def fold(r0, half, late):
            for w in range(half * AW // 2, (half + 1) * AW // 2):
                a = state[r0][w]
                a = (a + pltpu.roll(a, AH, 1)) * (AD ** -0.5)
                if isinstance(i, int) and r0 < ADIL * w:
                    pos = lax.broadcasted_iota(jnp.int32, (RC, 128), 0) + r0
                    a = jnp.where(pos >= ADIL * w, a, MASKED)
                state[r0][w] = a

        def weights(r0, late):
            m = late(functools.reduce(jnp.maximum, state[r0]))
            state[r0] = [jnp.exp(a - m) for a in state[r0]]

        def mix(r0, tiles, late):
            e = [late(state[r0][0])] + state[r0][1:]
            if 0 in tiles:
                state[r0, "inverse"] = _inverse(functools.reduce(jnp.add, e))
            for t in tiles:
                o = e[0] * window(LT + t, r0, 0)
                for w in range(1, AW):
                    o = o + e[w] * window(LT + t, r0, w)
                oa[t, _rows(r0, RC), :] = o * state[r0, "inverse"]

        stages = ((logits, 0), (logits, 1), (fold, 0), (fold, 1), (weights,), (mix, (0, 1)), (mix, (2, 3, 4)))
        return [[functools.partial(f, r0, *args) for r0 in range(slot(i), slot(i) + TB, RC)] for f, *args in stages]

    def a_pack(i):
        def pack(k):
            ob[k] = oa[k, _rows(slot(i), TE), :].astype(BF16)
            ol[k, _ds(i, TL), :] = oa[k, _rows(slot(i) + TE, TL), :].astype(BF16)
        return [functools.partial(pack, k) for k in range(LT)]

    def a_out(i):
        def store(t, r):
            outa[i, :, _rows(t * 128, 128)] = r.astype(BF16)
        return a_tiles(TE, lambda t, k: _dot(_load(ob, k), _load(wo_p, t, _ds(k, 64))), store)

    def overlap(tiles, side, zero):
        due = sorted((lo + (hi - lo) * n / len(tasks), m, n, task, tie)
                     for m, (lo, hi, tasks, tie) in enumerate(side) for n, task in enumerate(tasks))
        free = [0] * 4
        results = []
        for count, tile, end in tiles:
            now = min(free)
            free[free.index(now)] += count
            results.append((now, tile()))
            while due and (due[0][0] < min(free) or len(results) == len(tiles)):
                time, _, _, task, tie = due.pop(0)
                begin, r = [x for x in results if x[0] <= time][-1]
                row = min(int(time - begin), r.shape[0] - 1) // 8 * 8
                if isinstance(tie, str):
                    task(lambda x: jnp.where(zero == 0, x, r[_rows(row, 8)]))
                    continue
                if tie is bx:
                    tie[span(S, zero, 16), 0:128] = r[_rows(row // 16 * 16, 16)].astype(BF16)
                elif tie is not None:
                    tie[tie.shape[0] - 1 - zero, 0:8, :] = pltpu.bitcast(r[_rows(row, 8)], tie.dtype)
                task()
            if end:
                end()

    def wo_rows(r0, n, t):
        return _load(wo, t, _rows(r0 // 2, n // 2))

    def w_transpose(c, n):
        at = [FT * j + t for j, t in TILES[n::CG * LT]]
        if isinstance(c, int):
            at = at[c]
        else:
            words = [sum(x << 8 * k for k, x in enumerate(at[m::5])) for m in range(5)]
            word = functools.reduce(lambda x, m: jnp.where(lax.rem(c, 5) == m, words[m], x), range(1, 5), words[0])
            at = lax.shift_right_logical(word, lax.div(c, 5) * 8) & 255
        chunk = wb.at[pl.ds(c * CG * LT, NPL if isinstance(c, int) else CG * LT)]
        chunk[n] = pltpu.bitcast(raw[_ds(at, 128), :].T, U32)

    def w_combine(c, u, r, i):
        chunk = wb.at[pl.ds(c * CG * LT, CG * LT)]
        _combine(lambda a, b: pltpu.bitcast(chunk[u * LT + b, _rows(a * 64 + 8 * r, 8), :], BF16).astype(F32),
                 wz.at[pl.ds(c * CG, CG)].at[u], r, i)

    def wo_combine(g, r, i, late):
        def tile(a, b):
            x = wo_rows((g * LT + a) * 128 + 16 * r, 16, b).astype(F32)
            return jnp.concatenate([late(x[0:8]), x[8:]], axis=0)
        _combine(tile, wz.at[NG + g], r, i)

    def halves(batch, u):
        at = batch * TB if isinstance(batch, int) else pl.multiple_of(batch * TB, TB)
        x = bx.at[pl.ds(at, TB + SEG), :][_ds(u, SEG), :].astype(F32)
        return [[x[_rows(r, HALF), _rows(i * 128, 128)] for i in range(LT)] for r in (0, HALF)]

    def z_lhs(batch):
        def task(u, i):
            _long_lhs(*halves(batch, u), lz.at[:, _ds(batch * ZB + u, HALF), :], i)
        return [functools.partial(task, u, i) for u in range(ZB) for i in range(LT)]

    def z_product(g, n, batch):
        return _dot(_load(lz, n, _ds(batch, ZB * HALF // 2)), _load(wz, g, n))

    def z_group(g, batch):
        dst = z.at[_z_index(g, batch)]
        sums, stored = {}, []

        def tile(n):
            r = z_product(g, n, batch)
            for i in _targets(n):
                sums[i] = sums[i] + r if i in sums else r
            return r

        def end():
            for i in sums:
                _add_long(dst, i, sums[i], i not in stored)
                stored.append(i)
            sums.clear()
        sets = (((0, 1), (0, 2), (1, 2), 0, 1), ((0, 3), (0, 4), (3, 4), 3, 4), ((1, 3), (1, 4), (2, 3), (2, 4), 2))
        return [(ZB * HALF, functools.partial(tile, _long_index(n)), end if n == some[-1] else None)
                for some in sets for n in some]

    def part_a():
        c_wqkv = [cp(awqkv_hbm.at[:, pl.ds(j * D, D)], awqkv.at[pl.ds(j * D, D), :], sem_a.at[j]) for j in range(3)]
        c_second = [c_wqkv[1]] + c_strips(ax_hbm, ax, pl.ds(0, NS * TB), sem_a.at[1])
        c_third = [c_wqkv[2], c_bx(0, 2 * TB, sem_a.at[2])]
        c_awo = cp(awo_hbm, awo, sem_a.at[3])
        c_first = c_ax(0, sem_w.at[0]) + [c_bx(2, TB, sem_w.at[0])] + [
            c_w(j, 0, 0, FIRST[j], sem_w.at[0]) for j in range(2)]
        last_rows = pl.ds(S - 2 * TB, 2 * TB)
        c_last = [c_bx(NB // 2 - 1, 2 * TB, sem_w.at[NST]), cp(mem_hbm, mem.at[pl.ds(0, M), :], sem_w.at[NST]),
                  c_w(2, (NST - 1) * STEP[2], 0, H * DH - (NST - 1) * STEP[2], sem_w.at[NST])]

        flag[0] = 0
        start([c_wqkv[0]] + c_second)
        c_wqkv[0].wait()
        zero = flag[0]
        _run(sum(prep_wqkv(0), []))
        start(c_third)
        wait(c_second)
        first, second = prep_wqkv(1)
        overlap(a_proj(0, 0) + a_proj(1, 0), [(0, 0, first, None), (700, 1500, second, tmp)], zero)
        start([c_awo] + c_first[:-1])
        wait(c_third)
        first, second = prep_wqkv(2)
        overlap(a_proj(0, 1) + a_proj(1, 1),
                [(0, 0, first, None), (700, 1500, second, tmp), (0, 1500, z_lhs(0) + z_lhs(1), bx)], zero)
        c_first[-1].start()
        c_awo.wait()
        for i in range(NS):
            assert START_TIMES[i] + START_LAGS[i][-2] >= (i + 1) * 800
        assert START_TIMES[1] + START_LAGS[0][-1] <= 1500
        overlap(a_proj(0, 2) + a_proj(1, 2) + a_out(0),
                [(0, 800, prep_wo(), tmp), (1500, 1500, a_pack(0), None)]
                + [(START_TIMES[i] + d, START_TIMES[i + 1] + d, tasks, "value")
                   for i in range(NS) for d, tasks in zip(START_LAGS[i], a_attention(i))], zero)
        start(c_ax(1, sem_w.at[1]) + c_step(1) + c_ax(2, sem_w.at[2]) + c_step(2))
        wait(c_first)

        def step(c, carry):
            @pl.when((c > 0) & (c < NST))
            def _():
                wait_filled(ax.at[:, _ds(c + NS, TB), :], sem_w.at[c])
                wait(c_step(c))

            @pl.when(c == NST)
            def _():
                wait_filled(ax.at[:, last_rows, :], sem_w.at[NST])
                wait(c_last)

            zero = lax.shift_right_logical(c, 16)
            flag[zero] = 0
            i, t = c + NS, LOOP_TIMES
            assert t[0] / 2 <= t[1] + 100 and t[2] < 2900 and t[3] + LOOP_LAGS[-2] > 2500
            early = [x for u in range(2) for b in range(2) for x in z_group((c & 1) * 2 + u, (c | 1) + b)]
            overlap(a_proj(i, 0) + a_proj(i, 1) + a_proj(i, 2) + a_out(i - 1)
                    + z_group(c * CG, 0) + early + z_group(c * CG + 1, 0),
                    [(0, t[0], [functools.partial(w_transpose, c, n) for n in range(CG * LT)], None),
                     (0, t[1], z_lhs(c + 2), bx),
                     (0, t[1], a_pack(i - 1), oa),
                     (t[1], t[2], [functools.partial(w_combine, c, u, r, k)
                                   for u in range(CG) for r in range(8) for k in range(LT)], wb)]
                    + [(t[3] + d, t[4] + d, tasks, "value") for d, tasks in zip(LOOP_LAGS, a_attention(i))], zero)

            n = jnp.minimum(c + 3, NST - 1)
            for copy in c_ax(n, sem_w.at[n]) + c_step(n) + c_strips(wo_hbm, wo, _ds(c, WO_STEP), sem_a.at[4]):
                pl.when(c < NST - 3)(copy.start)
            for copy in c_strips(ax_hbm, ax, last_rows, sem_w.at[NST]) + c_last:
                pl.when(c == NST - 3)(copy.start)
            at = span(WO_FIRST, jnp.clip(c - (NST - 2), 0, 1), (H * DH - WO_FIRST) // 2)
            for copy in c_strips(wo_hbm, wo, at, sem_a.at[5]):
                pl.when((c > NST - 3) & (c < NST))(copy.start)
            return carry

        lax.fori_loop(0, NCH, step, 0)
        wait_filled(wo.at[:, pl.ds(0, WO_FIRST), :], sem_a.at[4])
        t = END_TIMES
        overlap([x for g in range(G0) for x in z_group(g, NB - 1)] + a_out(NB - 1),
                [(0, 0, [functools.partial(w_transpose, NCH, n) for n in range(NPL)], None),
                 (0, t[0], a_pack(NB - 1), oa),
                 (t[1], t[2], [functools.partial(wo_combine, g, r, i)
                               for g in range(WG) for r in range(8) for i in range(LT)], "value")], zero)

    def r_lhs(hb, i, j):
        return R_LHS + ((hb * LT + i) * LT + j) * (M + HALF)

    def r_qkv(j, t):
        return _rows(R_QKV + (j * FT + t) * L, L)

    def token_lhs(batch, u, hb):
        a, b = halves(batch, u)
        for j in range(LT):
            buf[_rows(R_H + (hb * LT + j) * L + M, SEG)] = jnp.concatenate([a[j], b[j]], axis=0)
            for i, x in enumerate(_short_lhs(a, b, j)):
                buf[_rows(r_lhs(hb, i, j) + M, HALF)] = x

    def memory_lhs(m, n, hb):
        buf[_rows(R_H + (hb * LT + n) * L, M)] = m[n]
        buf[_rows(r_lhs(hb, n, n), M)] = m[n]
        for k in range(n):
            buf[_rows(r_lhs(hb, n, k), M)] = buf[_rows(r_lhs(hb, k, n), M)] = m[n] + m[k]

    stored = []

    def segment(plan, batch, part, hb, nh, before=()):
        s = batch * ZB + part
        key = lax.broadcasted_iota(jnp.int32, (L, 128), 0)
        col = lax.broadcasted_iota(jnp.int32, (L, 128), 1)
        head0 = col < L
        query = jnp.where(head0, col, col - L)
        visible = (query < M) | (query >= key)
        low = col < 64
        zo = z.at[z.shape[0] - 1 - batch % 2]
        z_next = z.at[pl.ds(_z_index(G0, batch + 1), NG - G0)]
        val, sums, new_mem = {}, {}, []

        def add(name, x):
            val[name] = val[name] + x if name in val else x

        def product(*args):
            r = _dot(*args)
            val["latest"] = r[-8:]
            return r

        def short(g, i, j):
            if i == j:
                w = _load(wz, g, NZ + i)
            elif g < NG:
                w = pltpu.bitcast(wb[g * LT + j, _rows(i * 64, 64), :], BF16)
            else:
                w = wo_rows(((g - NG) * LT + i) * 128, 128, j)
            at = r_lhs(hb, i, j) if g < NG else R_OL + r_lhs(g - NG, i, j)
            add((min(g, NG), i, j), product(buf[_rows(at, M + HALF)], w))

        def short_end(g, i, j):
            if NG <= g < NG + WG - 1:
                return
            g = min(g, NG)
            r = val.pop((g, i, j))
            add(("m", g, j), r[0:M])
            if i != j:
                add(("y", g, i), r[M:])
                add(("b", g, j), r[M:])
                if LAM[i]:
                    add(("a", g, j), r[M:] * -LAM[i])
                return
            y = val.pop(("y", g, j))
            if g < NG:
                y = y + z[_z_index(g, batch), part, _rows(j * HALF, HALF), :]
            a = val.pop(("a", g, j)) + r[M:]
            if LAM[j]:
                a = a - LAM[j] * y
            r = jnp.concatenate([val.pop(("m", g, j)), a, val.pop(("b", g, j)) + y], axis=0)
            if g < NG:
                buf[r_qkv(*TILES[g * LT + j])] = r
            else:
                buf[_rows(R_ACC + j * L, L)] = out_sum(j, r)

        def plain(n, k):
            w = pltpu.bitcast(wb[NG * LT + n, _rows(k * 64, 64), :], BF16)
            val["plain", n, k] = product(buf[_rows(R_H + (hb * LT + k) * L, L)], w)

        def plain_end(n, k):
            dst = r_qkv(*TILES[NG * LT + n])
            r = val.pop(("plain", n, k))
            buf[dst] = r + buf[dst] if k else r

        def long(g, n):
            r = z_product(g, n, batch + 1) if g < NG else _dot(_load(lo, g - NG, n), _load(wz, g, n))
            val["long", g, n], val["latest"] = r, r[24:32]

        def long_end(g, n):
            r = val.pop(("long", g, n))
            g = min(g, NG)
            for i in _targets(n):
                sums[g, i] = sums[g, i] + r if (g, i) in sums else r

        def long_store():
            for (g, i), r in sums.items():
                _add_long(z_next.at[g - G0] if g < NG else zo, i, r, (g, i) not in stored)
                stored.append((g, i))
            sums.clear()

        def a_late(u, t, k):
            n = ZB * HALF
            x = _load(ol, k, _ds(part * (NB * TL // (ZB * n)) + u, n // 2))
            add("late", product(x, _load(wo_p, t, _ds(k, 64))))
            if k == LT - 1:
                r = val.pop("late").astype(BF16)
                for m in range(n // TL):
                    outl[part * (NB // ZB) + u * (n // TL) + m, :, _rows(t * 128, 128)] = r[_rows(m * TL, TL)]

        def score(p, both):
            if both:
                q, k = [[buf[r_qkv(j, 3 * p + t)] for t in (0, 2)] for j in (0, 1)]
            else:
                q, k = buf[r_qkv(0, 3 * p + 1)], [buf[r_qkv(1, 3 * p + 1)]]
                q = [jnp.where(low, q, 0.0), jnp.where(low, 0.0, q)]
            q = jnp.concatenate(q + [jnp.zeros((128 - 2 * L, 128), F32)], axis=0)
            r = product(jnp.concatenate(k, axis=0), q.astype(BF16), NT)
            add(("s", p), jnp.where(head0, r[0:L], r[L:]) if both else r)

        def softmax(p, step):
            def late(x):
                return jnp.where(col[0:8] < 2 * L, x, val["latest"])

            def groups(x):
                return [x[_rows(r, 8)] for r in range(0, L, 8)]

            def spread(x):
                return jnp.concatenate([x] * (L // 8), axis=0)
            x, y = val["s", p], val.get(("t", p))
            if step == 0:
                x = jnp.where(visible, x * (DH ** -0.5), MASKED)
                y = functools.reduce(jnp.maximum, groups(x))
            elif step == 1:
                y = jnp.broadcast_to(jnp.max(late(y), axis=0, keepdims=True), (8, 128))
            elif step == 2:
                x = jnp.exp(x - spread(late(y)))
                y = functools.reduce(jnp.add, groups(x))
            elif step == 3:
                y = jnp.broadcast_to(jnp.sum(late(y), axis=0, keepdims=True), (8, 128))
            elif step == 4:
                y = _inverse(late(y))
            else:
                x = x * spread(late(y))
                x = jnp.concatenate([x, x], axis=0)[:, 0:2 * L]
                buf[_rows(R_P + p * 2 * L, 2 * L), 0:2 * L] = x.astype(BF16).T.astype(F32)
            val["s", p], val["t", p] = x, y

        def pv(t):
            pa, pb = [buf[_rows(R_P + (2 * (t // 3) + u) * L, L), 0:2 * L] for u in range(2)]
            v = buf[r_qkv(2, t)]
            if t % 3 == 1:
                v = jnp.concatenate([jnp.where(low, v, 0.0), jnp.where(low, 0.0, v)], axis=0)
            pr = (pa[:, 0:L], jnp.where(head0[:, 0:2 * L], pa, pb), pb[:, 0:L])[t % 3]
            val["o", t] = product(pr, v.astype(BF16))

        def pv_end(t):
            buf[_rows(R_O + t * L, L)] = val.pop(("o", t))

        def out_lhs(g, j):
            o = [buf[_rows(R_O + (g * LT + i) * L, L)] for i in range(LT)]
            a, b = [x[M:M + HALF] for x in o], [x[M + HALF:] for x in o]
            a[j] = jnp.concatenate([jnp.where(batch >= 0, x, val["latest"]) for x in (a[j][0:8], a[j][8:])], axis=0)
            for i, x in enumerate(_short_lhs(a, b, j)):
                m = o[j][0:M] if i == j else o[i][0:M] + o[j][0:M]
                buf[_rows(R_OL + r_lhs(g, i, j), M + HALF)] = jnp.concatenate([m, x], axis=0)
            _long_lhs(a, b, lo.at[g, :, _rows(part * HALF, HALF), :], j)

        def out(t, n):
            x = buf[_rows(R_O + t * L, L)]
            if "stored" in val:
                x = jnp.concatenate([x[0:L - 8], jnp.where(batch >= 0, x[L - 8:], val.pop("stored"))], axis=0)
            add(("out", t // KC, n), product(x, wo_rows(t * 128, 128, n)))

        def out_sum(n, r):
            if ("sum", n) in val:
                r = r + buf[_rows(R_ACC + n * L, L)]
            val["sum", n] = True
            return r

        def out_end(t, n):
            r = out_sum(n, val.pop(("out", t // KC, n)))
            if t < FT - 1:
                buf[_rows(R_ACC + n * L, L)] = r
                return
            new_mem.append(r[0:M])
            memory_lhs(new_mem, n, nh)
            if not isinstance(part, int):
                outb[_ds(s, SEG), _rows(n * 128, 128)] = r[M:L].astype(BF16)
            elif part < ZB - 1:
                op[part, n] = r[M:L]
            else:
                finish(n, part, r[M:L])

        def finish(n, u, r=None):
            y = zo[u, _rows(n * HALF, HALF), :]
            if r is None:
                r = op[u, n]
                y = jnp.concatenate([jnp.where(batch >= 0, x, val["latest"]) for x in (y[0:8], y[8:])], axis=0)
            y = jnp.concatenate([-LAM[n] * y, y], axis=0)
            outb[_ds(batch * ZB + u, SEG), _rows(n * 128, 128)] = (r + y).astype(BF16)

        def finished():
            val["stored"] = outb[_ds(jnp.maximum(batch, 0) * (TB // 8), 8), 0:128].astype(F32)

        tasks = dict(short=short, short_end=short_end, plain=plain, plain_end=plain_end, long=long,
                     long_end=long_end, long_store=long_store, a_late=a_late, score=score, softmax=softmax,
                     pv=pv, pv_end=pv_end, out_lhs=out_lhs, out=out, out_end=out_end, finish=finish, finished=finished,
                     next_tokens=lambda: token_lhs(
                         batch, part + 1 if isinstance(part, int) else jnp.minimum(part + 1, ZB - 1), nh))
        before = list(before)
        for name, *args in plan[0]:
            if name in ("short", "plain"):
                while len(before) > LT - 1 - max(args[1:]):
                    before.pop(0)()
            tasks[name](*args)
        return [functools.partial(tasks[name], *args) for name, *args in plan[1]]

    order = [_long_index(n) for n in
             ((0, 1), (0, 2), (1, 2), 0, (0, 3), (0, 4), (3, 4), 3, 4, (1, 4), 1, (1, 3), (2, 3), (2, 4), 2)]
    longs = ([("long", g, n) for g in range(G0, NG) for n in order]
             + [("long", NG + g, n) for n in order for g in range(WG)])
    plans = [_make_plan(rounds, longs, WG) for rounds in ROUNDS]
    late = [("a_late", u, t, k) for u in range(NB * TL // (ZB * ZB * HALF)) for t in range(LT) for k in range(LT)]
    last_plan = _make_plan(LAST_ROUNDS, late, 0)
    assert not longs and not late
    tasks = plans[-1][0]
    assert ("long", NG, order[0]) in tasks and ("finished",) in tasks
    assert ("long_store",) not in tasks[tasks.index(("finish", 0, 0)):]
    for tasks in (sum(plan, []) for plan in plans):
        assert tasks.index(("short_end", NG + WG - 1, LT - 1, LT - 1)) < tasks.index(("out_end", FT - 1, 0))

    def batch_step(batch, carry):
        rest = ()
        for u in range(ZB):
            rest = segment(plans[u], batch, u, u, (u + 1) % ZB, rest)
        _run(rest)
        c_outb(pl.multiple_of(batch * TB, TB), TB).start()
        return carry

    def last_step(s, carry):
        _run(segment(last_plan, s // ZB, s % ZB, 0, 0))
        c_outl(s % ZB).start()
        c_outb(pl.multiple_of(s * SEG, SEG), SEG).start()
        return carry

    part_a()
    token_lhs(0, 0, 0)
    mem0 = mem[0:M, :].astype(F32)
    for n in range(LT):
        memory_lhs([mem0[:, _rows(k * 128, 128)] for k in range(LT)], n, 0)
    wait_filled(wo.at[:, pl.ds(WO_FIRST, H * DH - WO_FIRST), :], sem_a.at[5])
    c_outa = cp(outa, out_hbm.at[:, pl.ds(0, TE), pl.ds(0, D)], sem_o.at[0])
    c_outa.start()
    lax.fori_loop(0, NB - 1, batch_step, 0)
    lax.fori_loop(NSEG - ZB, NSEG, last_step, 0)
    c_outa.wait()
    wait_filled(out_hbm.at[:, :, pl.ds(D, D)], sem_o.at[1])
    wait_filled(out_hbm.at[:, pl.ds(TE, TL), pl.ds(0, D)], sem_o.at[2])


def pallas_concat_heads__sliding_local_dilated__memory_aug_recurrent_mem_tr__prompt_kernel(
    A_x, A_wqkv, A_wo, B_x, B_mem0, B_Wq, B_Wk, B_Wv, B_Wo, B_seg_len,
):
    assert B_seg_len == SEG
    assert A_x.shape == B_x.shape == (1, S, D) and B_mem0.shape == (1, M, D)
    assert B_Wq.shape == B_Wk.shape == B_Wv.shape == (D, H, DH) and B_Wo.shape == (H, DH, D)
    vmem, dma = pltpu.VMEM, pltpu.SemaphoreType.DMA
    call = pl.pallas_call(
        _kernel,
        out_shape=jax.ShapeDtypeStruct((NB, TB, 2 * D), BF16),
        in_specs=[pl.BlockSpec(memory_space=pl.ANY)] * 9,
        out_specs=pl.BlockSpec(memory_space=pl.ANY),
        scratch_shapes=[
            vmem((LT, S, 128), BF16),
            vmem((D, D), BF16),
            vmem((LT + 1, D, 128), F32),
            vmem((LT, 3 * D, 128), BF16),
            vmem((LT, D, 128), BF16),
            vmem((LT, NS * TB, 128), F32),
            vmem((2 * LT, HALO + NS * TB, 128), F32),
            vmem((LT + 1, NS * TB, 128), F32),
            vmem((LT + 1, TE, 128), BF16),
            vmem((LT, NB * TL, 128), BF16),
            vmem((NB, TE, D), BF16),
            vmem((NB, TL, D), BF16),
            vmem((S + 64, D), BF16),
            vmem((64, D), BF16),
            vmem((3 * H * DH, D), BF16),
            vmem((len(TILES) + 1, D // 2, 128), U32),
            vmem((NG + WG, NZ + LT, 128, 128), BF16),
            vmem((LT, H * DH, 128), BF16),
            vmem((NZ, S // 2, 128), BF16),
            vmem((2 * (NG - G0) + NB * G0 + 2, ZB, (LT + 1) * HALF, 128), F32),
            vmem((WG, NZ, ZB * HALF, 128), BF16),
            vmem((ZB, LT, SEG, 128), F32),
            vmem((R_END, 128), F32),
            pltpu.SMEM((2,), jnp.int32),
            dma((6,)), dma((NCH,)), dma((3,)),
        ],
        compiler_params=pltpu.CompilerParams(
            vmem_limit_bytes=126 * 1024 * 1024, internal_scratch_in_bytes=48 * 1024,
            disable_bounds_checks=True, disable_semaphore_checks=True),
        name="sliding_and_memory_attention",
    )

    def by_feature(w):
        return w.transpose(1, 2, 0).reshape(H * DH, D)

    out = call(A_x.reshape(S, D), A_wqkv, A_wo, B_x.reshape(S, D), B_mem0.reshape(M, D),
               by_feature(B_Wq), by_feature(B_Wk), by_feature(B_Wv), B_Wo.reshape(H * DH, D))
    return out.reshape(1, S, 2 * D)
```
